```python
import jax
import jax.numpy as jnp

def _softmax(x, axis=-1):
    return jax.nn.softmax(x, axis=axis)

def _gelu(x):
    return jax.nn.gelu(x, approximate=True)

def _silu(x):
    return jax.nn.silu(x)

def _sigmoid(x):
    return jax.nn.sigmoid(x)

def _layernorm(x, axis=-1, eps=1e-05):
    m = jnp.mean(x, axis=axis, keepdims=True)
    v = jnp.var(x, axis=axis, keepdims=True)
    return (x - m) / jnp.sqrt(v + eps)

def _scatter_add(tgt, idx, src, axis=0):
    return tgt.at[idx].add(src)

def _segment_sum(src, seg, n):
    return jax.ops.segment_sum(src, seg, n)

class _Rng:

    def __init__(self, key):
        self._k = key

    def _next(self):
        self._k, sub = jax.random.split(self._k)
        return sub

    def normal(self, shape):
        return jax.random.normal(self._next(), shape, dtype=jnp.bfloat16)

    def randint(self, lo, hi, shape):
        return jax.random.randint(self._next(), shape, lo, hi, dtype=jnp.int32)

    def uniform(self, shape, lo=0.0, hi=1.0):
        return jax.random.uniform(self._next(), shape, jnp.bfloat16, lo, hi)

    def permutation(self, n):
        return jax.random.permutation(self._next(), n)
kernel_name = 'adaLN_cond__memory_aug_recurrent_mem_tr__mixer_s_mlp__prompt'

def setup_inputs():
    _rng = _Rng(jax.random.key(int.from_bytes(__import__("os").urandom(4), "little")))
    _w = lambda a: (lambda t: t.astype(jnp.bfloat16) if jnp.issubdtype(t.dtype, jnp.floating) else t)(jnp.asarray(a))

    def _A_setup():
        B, S, Dm = (1, 2048, 1024)
        H, Dh = (32, 128)
        M, seg = (8, 32)
        seg = min(seg, S)
        S = S // seg * seg
        return {'x': _w((lambda *s: _rng.normal(s) * 0.05)(B, S, Dm)), 'mem0': _w((lambda *s: _rng.normal(s) * 0.05)(B, M, Dm)), 'Wq': _w((lambda *s: _rng.normal(s) * 0.05)(Dm, H, Dh) * Dm ** (-0.5)), 'Wk': _w((lambda *s: _rng.normal(s) * 0.05)(Dm, H, Dh) * Dm ** (-0.5)), 'Wv': _w((lambda *s: _rng.normal(s) * 0.05)(Dm, H, Dh) * Dm ** (-0.5)), 'Wo': _w((lambda *s: _rng.normal(s) * 0.05)(H, Dh, Dm) * (H * Dh) ** (-0.5)), 'seg_len': seg}
    _A_in = _A_setup()

    def _B_setup():
        B, S, D, F = (1, 2048, 1024, 3584)
        return {'x': _w((lambda *s: _rng.normal(s) * 0.05)(B, S, D)), 'w1': _w((lambda *s: _rng.normal(s) * 0.05)(D, D) * D ** (-0.5)), 'w2': _w((lambda *s: _rng.normal(s) * 0.05)(D, D) * D ** (-0.5)), 'w3': _w((lambda *s: _rng.normal(s) * 0.05)(D, F) * D ** (-0.5)), 'w4': _w((lambda *s: _rng.normal(s) * 0.05)(F, D) * F ** (-0.5))}
    _B_in = _B_setup()
    return {'A_x': _A_in['x'], 'A_mem0': _A_in['mem0'], 'A_Wq': _A_in['Wq'], 'A_Wk': _A_in['Wk'], 'A_Wv': _A_in['Wv'], 'A_Wo': _A_in['Wo'], 'A_seg_len': _A_in['seg_len'], 'B_x': _B_in['x'], 'B_w1': _B_in['w1'], 'B_w2': _B_in['w2'], 'B_w3': _B_in['w3'], 'B_w4': _B_in['w4'], 'c': _w((lambda *s: _rng.normal(s) * 0.05)(1, 1024)), 'w_mod': _w((lambda *s: _rng.normal(s) * 0.05)(1024, 6 * 1024) * 1024 ** (-0.5))}

def reference(A_x, A_mem0, A_Wq, A_Wk, A_Wv, A_Wo, A_seg_len, B_x, B_w1, B_w2, B_w3, B_w4, c, w_mod):

    def _A_ref(x, mem0, Wq, Wk, Wv, Wo, seg_len):
        B, S, Dm = x.shape
        H, Dh = (Wq.shape[1], Wq.shape[2])
        M = mem0.shape[1]
        scale = Dh ** (-0.5)
        n_seg = S // seg_len
        L = M + seg_len
        idx = jnp.arange(L)
        mask = (idx[:, None] < M) | (idx[:, None] >= idx[None, :])
        mem = mem0
        outs = []
        for s in range(n_seg):
            xs = x[:, s * seg_len:(s + 1) * seg_len, :].copy()
            h = jnp.concatenate([mem, xs], axis=1)
            q = jnp.einsum('btd,dhe->bhte', h, Wq)
            k = jnp.einsum('btd,dhe->bhte', h, Wk)
            v = jnp.einsum('btd,dhe->bhte', h, Wv)
            scores = jnp.einsum('bhqe,bhke->bhqk', q, k) * scale
            scores = jnp.where(mask[None, None], scores, -1000000000.0)
            p = _softmax(scores, axis=-1)
            o = jnp.einsum('bhqk,bhke->bhqe', p, v)
            o = jnp.einsum('bhte,hed->btd', o, Wo)
            mem = o[:, :M, :].copy()
            outs.append(o[:, M:, :])
        return jnp.concatenate(outs, axis=1)

    def _B_ref(x, w1, w2, w3, w4):
        B, S, D = x.shape
        h = _gelu(_layernorm(x, axis=-1) @ w1)
        c = D // 4
        g0 = jnp.pad(h[:, :, 0 * c:1 * c], ((0, 0), (1, 0), (0, 0)))[:, :S, :]
        g1 = jnp.pad(h[:, :, 1 * c:2 * c], ((0, 0), (0, 1), (0, 0)))[:, 1:, :]
        g2 = jnp.pad(h[:, :, 2 * c:3 * c], ((0, 0), (2, 0), (0, 0)))[:, :S, :]
        g3 = jnp.pad(h[:, :, 3 * c:], ((0, 0), (0, 2), (0, 0)))[:, 2:, :]
        hs = jnp.concatenate([g0, g1, g2, g3], axis=-1) @ w2
        x1 = x + hs
        h2 = _gelu(_layernorm(x1, axis=-1) @ w3) @ w4
        return x1 + h2
    x = A_x
    mod = (_silu(c) @ w_mod).reshape(c.shape[0], 6, 1, -1)
    sa, ca, ga, sb, cb, gb = (mod[:, 0].copy(), mod[:, 1].copy(), mod[:, 2].copy(), mod[:, 3].copy(), mod[:, 4].copy(), mod[:, 5].copy())
    h = _layernorm(x, axis=-1) * (1 + ca) + sa
    x = x + ga * _A_ref(h, A_mem0, A_Wq, A_Wk, A_Wv, A_Wo, A_seg_len)
    h = _layernorm(x, axis=-1) * (1 + cb) + sb
    x = x + gb * _B_ref(h, B_w1, B_w2, B_w3, B_w4)
    return x
```

```python
import functools
import math

import jax
import jax.numpy as jnp
from jax import lax
import jax.experimental.pallas as pl
import jax.experimental.pallas.tpu as pltpu

_F32 = jnp.float32
_BF16 = jnp.bfloat16
_U32 = jnp.uint32
_LANE = 128
_EPS = 1e-05
_TM = 256
_FC = 512
_DC = 128
_HALO = 8


def _dot(a, b):
    return lax.dot_general(a, b, (((1,), (0,)), ((), ())), preferred_element_type=_F32)


def _dot_nt(a, b):
    return lax.dot_general(a, b, (((1,), (1,)), ((), ())), preferred_element_type=_F32)


def _layernorm(x):
    m = jnp.mean(x, axis=-1, keepdims=True)
    d = x - m
    v = jnp.mean(d * d, axis=-1, keepdims=True)
    return d * lax.rsqrt(v + _EPS)


def _gelu(x):
    c = math.sqrt(2.0 / math.pi)
    inner = x * (c + (c * 0.044715) * (x * x))
    hx = 0.5 * x
    return hx + hx * jnp.tanh(inner)


def _cat_slabs(ref, lo, hi, rows=slice(None)):
    return jnp.concatenate([ref[j, rows, :] for j in range(lo, hi)], axis=1)


def _kernel(mem0_ref, c_ref, x_hbm, wq_hbm, wk_hbm, wv_hbm, wo_hbm, w1_hbm, w2_hbm, w3_hbm,
            w4_hbm, wmod_hbm, out_hbm,
            x_v, wqkv, stage, wo_s, w1_s, w2_s, w3_s, w4_s, wmod_s, mod_s, lhs_s, o_s, a_s, g_s,
            hb_s, x1_s, n1_s, out_s, sems, out_sems, *, seg_len):
    S, D = x_v.shape
    M = mem0_ref.shape[0]
    H = wqkv.shape[0] // 3
    L = M + seg_len
    n_seg = S // seg_len
    ND = D // _LANE
    NF = w3_s.shape[0]
    scale = float(_LANE) ** -0.5

    sem_count = [0]

    def copy(src, dst):
        i = sem_count[0]
        sem_count[0] += 1
        return pltpu.make_async_copy(src, dst, sems.at[i])

    def slab_copies(src, dst, col0, n):
        return [copy(src.at[:, pl.ds(col0 + j * _LANE, _LANE)], dst.at[j]) for j in range(n)]

    def start(cps):
        for cp in cps:
            cp.start()

    def wait(cps):
        for cp in cps:
            cp.wait()

    cp_mod_a = slab_copies(wmod_hbm, wmod_s, 0, 2 * ND)
    cp_x = [copy(x_hbm, x_v)]
    cp_wq = [copy(wq_hbm, stage.at[0])]
    cp_wk = [copy(wk_hbm, stage.at[1])]
    cp_wv = [copy(wv_hbm, stage.at[0])]
    cp_wo = slab_copies(wo_hbm, wo_s, 0, ND)
    cp_mod_b = slab_copies(wmod_hbm, wmod_s, 2 * D, 4 * ND)
    cp_b = (slab_copies(w1_hbm, w1_s, 0, ND) + slab_copies(w2_hbm, w2_s, 0, ND)
            + slab_copies(w3_hbm, w3_s, 0, NF) + slab_copies(w4_hbm, w4_s, 0, ND))

    def relayout(slot, base):
        hp_n = H // 2
        words = stage.at[slot].bitcast(_U32)

        def body(i, carry):
            src = words.at[pl.ds(pl.multiple_of(i * (_DC * hp_n), _DC * hp_n), _DC * hp_n), :]
            dst = pl.ds(pl.multiple_of(i * (_DC // 2), _DC // 2), _DC // 2)
            for hp in range(hp_n):
                w = src[pl.ds(hp, _DC, stride=hp_n), :]
                lo = pltpu.bitcast(w << 16, _F32).astype(_BF16)
                hi = pltpu.bitcast(w & jnp.uint32(0xFFFF0000), _F32).astype(_BF16)
                wqkv[base + 2 * hp, dst, :] = pltpu.bitcast(lo, _U32)
                wqkv[base + 2 * hp + 1, dst, :] = pltpu.bitcast(hi, _U32)
            return carry

        lax.fori_loop(0, D // _DC, body, 0)

    start(cp_mod_a + cp_x + cp_wq)
    cf = c_ref[...].astype(_F32)
    silu_c = jnp.broadcast_to(cf * jax.nn.sigmoid(cf), (8, D))
    with jax.named_scope('sc_wait_mod'):
        wait(cp_mod_a)
    start(cp_wk)
    for r in range(2):
        mod_s[r] = _dot(silu_c, _cat_slabs(wmod_s, r * ND, (r + 1) * ND))
    with jax.named_scope('sc_wait_q'):
        wait(cp_wq)
    relayout(0, 0)
    start(cp_wv)
    with jax.named_scope('sc_wait_k'):
        wait(cp_wk)
    start(cp_wo)
    relayout(1, H)
    with jax.named_scope('sc_wait_v'):
        wait(cp_wv)
    relayout(0, 2 * H)
    with jax.named_scope('sc_wait_wo'):
        wait(cp_x + cp_wo)
    start(cp_mod_b + cp_b)

    def seg_input(s):
        xs = x_v[pl.ds(pl.multiple_of(s * seg_len, seg_len), seg_len), :].astype(_F32)
        return _layernorm(xs) * (1.0 + mod_s[1, 0:1, :]) + mod_s[0, 0:1, :]

    lhs_s[0:M, :] = mem0_ref[...].astype(_F32)
    lhs_s[M:L, :] = seg_input(0)

    row = lax.broadcasted_iota(jnp.int32, (L, L), 0)
    col = lax.broadcasted_iota(jnp.int32, (L, L), 1)
    mask = (row < M) | (row >= col)

    G = 4
    NG = H // G

    def seg_step(s, carry):
        lhs = lhs_s[...]

        def proj(base, g):
            w = jnp.concatenate([pltpu.bitcast(wqkv[base + g * G + j], _BF16) for j in range(G)], axis=1)
            return _dot(lhs, w)

        def head(t, j):
            return t[:, j * _LANE:(j + 1) * _LANE]

        def probs(q, k):
            out = []
            for j in range(G):
                sc = _dot_nt(head(q, j), head(k, j)) * scale
                sc = jnp.where(mask, sc, -1000000000.0)
                e = jnp.exp(sc - jnp.max(sc, axis=-1, keepdims=True))
                out.append(e / jnp.sum(e, axis=-1, keepdims=True))
            return out

        def mix(g, p, v):
            for j in range(G):
                h = g * G + j
                o_s[:, h * _LANE:(h + 1) * _LANE] = _dot(p[j], head(v, j))

        def out_proj(h0, h1):
            ks = slice(h0 * _LANE, h1 * _LANE)
            return _dot(o_s[:, ks], _cat_slabs(wo_s, 0, ND, ks))

        pend = None
        for g in range(NG):
            q = proj(0, g)
            k = proj(H, g).astype(_BF16)
            if pend is not None:
                mix(*pend)
            v = proj(2 * H, g).astype(_BF16)
            pend = (g, probs(q, k), v)
        nxt = seg_input(jnp.minimum(s + 1, n_seg - 1))
        y = out_proj(0, 8)
        mix(*pend)
        y = y + out_proj(8, H)
        rows = pl.ds(pl.multiple_of(s * seg_len, seg_len), seg_len)
        lhs_s[0:M, :] = y[0:M]
        a_s[rows, :] = y[M:L]
        lhs_s[M:L, :] = nxt
        return carry

    with jax.named_scope('sc_attn'):
        lax.fori_loop(0, n_seg, seg_step, 0)

    with jax.named_scope('sc_wait_b'):
        wait(cp_mod_b + cp_b)
    for r in range(4):
        mod_s[2 + r] = _dot(silu_c, _cat_slabs(wmod_s, r * ND, (r + 1) * ND))
    g_s[0:_HALO, :] = jnp.zeros((_HALO, D), _F32)
    g_s[_HALO + S:_HALO + S + _HALO, :] = jnp.zeros((_HALO, D), _F32)
    n_blk = S // _TM
    cq = D // 4

    def stage1(i):
        rows = pl.ds(pl.multiple_of(i * _TM, _TM), _TM)
        xm = x_v[rows, :].astype(_F32) + mod_s[2, 0:1, :] * a_s[rows, :]
        a_s[rows, :] = xm
        hb = _layernorm(xm) * (1.0 + mod_s[4, 0:1, :]) + mod_s[3, 0:1, :]
        hb_s[rows, :] = hb
        g = _gelu(_dot(_layernorm(hb).astype(_BF16), _cat_slabs(w1_s, 0, ND)))
        g_s[pl.ds(pl.multiple_of(i * _TM + _HALO, 8), _TM), :] = g

    def stage2(i):
        rows = pl.ds(pl.multiple_of(i * _TM, _TM), _TM)
        win = g_s.at[pl.ds(pl.multiple_of(i * _TM, _TM), _TM + 2 * _HALO), :]
        parts = [win[_HALO + off:_HALO + off + _TM, j * cq:(j + 1) * cq]
                 for j, off in enumerate((-1, 1, -2, 2))]
        shifted = jnp.concatenate(parts, axis=1).astype(_BF16)
        x1 = hb_s[rows, :] + _dot(shifted, _cat_slabs(w2_s, 0, ND))
        x1_s[rows, :] = x1
        n1_s[rows, :] = _layernorm(x1).astype(_BF16)

    def out_copy(i, slot):
        return pltpu.make_async_copy(
            out_s.at[slot], out_hbm.at[pl.ds(pl.multiple_of(i * _TM, _TM), _TM), :],
            out_sems.at[slot])

    def stage3(i):
        rows = pl.ds(pl.multiple_of(i * _TM, _TM), _TM)
        n1 = n1_s[rows, :]
        acc = x1_s[rows, :]
        per = _FC // _LANE
        for f in range(NF // per):
            u = _gelu(_dot(n1, _cat_slabs(w3_s, f * per, (f + 1) * per))).astype(_BF16)
            acc = acc + _dot(u, _cat_slabs(w4_s, 0, ND, slice(f * _FC, (f + 1) * _FC)))
        res = a_s[rows, :] + mod_s[5, 0:1, :] * acc
        slot = i % 2

        @pl.when(i >= 2)
        def _():
            out_copy(jnp.maximum(i - 2, 0), slot).wait()

        out_s[slot] = res.astype(out_s.dtype)
        out_copy(i, slot).start()

    def loop(fn):
        def body(i, carry):
            fn(i)
            return carry
        lax.fori_loop(0, n_blk, body, 0)

    with jax.named_scope('sc_s1'):
        loop(stage1)
    with jax.named_scope('sc_s2'):
        loop(stage2)
    with jax.named_scope('sc_s3'):
        loop(stage3)
    for i in (n_blk - 2, n_blk - 1):
        out_copy(i, i % 2).wait()


@functools.partial(jax.jit, static_argnames=("A_seg_len",))
def pallas_adaLN_cond__memory_aug_recurrent_mem_tr__mixer_s_mlp__prompt_kernel(
    A_x: jax.Array,
    A_mem0: jax.Array,
    A_Wq: jax.Array,
    A_Wk: jax.Array,
    A_Wv: jax.Array,
    A_Wo: jax.Array,
    A_seg_len: int,
    B_x: jax.Array,
    B_w1: jax.Array,
    B_w2: jax.Array,
    B_w3: jax.Array,
    B_w4: jax.Array,
    c: jax.Array,
    w_mod: jax.Array,
):
    del B_x
    batch, S, D = A_x.shape
    _, H, Dh = A_Wq.shape
    M = A_mem0.shape[1]
    F = B_w3.shape[1]
    seg_len = int(A_seg_len)
    L = M + seg_len
    assert batch == 1 and Dh == _LANE and S % seg_len == 0 and S % _TM == 0 and F % _FC == 0
    ND, NF = D // _LANE, F // _LANE
    n_sems = 6 * ND + 4 + ND + 3 * ND + NF

    vmem = pl.BlockSpec(memory_space=pltpu.VMEM)
    hbm = pl.BlockSpec(memory_space=pl.ANY)
    out = pl.pallas_call(
        functools.partial(_kernel, seg_len=seg_len),
        out_shape=jax.ShapeDtypeStruct((S, D), A_x.dtype),
        in_specs=[vmem, vmem] + [hbm] * 10,
        out_specs=hbm,
        scratch_shapes=[
            pltpu.VMEM((S, D), _BF16),
            pltpu.VMEM((3 * H, D // 2, Dh), _U32),
            pltpu.VMEM((2, D * H, Dh), _BF16),
            pltpu.VMEM((ND, H * Dh, _LANE), _BF16),
            pltpu.VMEM((ND, D, _LANE), _BF16),
            pltpu.VMEM((ND, D, _LANE), _BF16),
            pltpu.VMEM((NF, D, _LANE), _BF16),
            pltpu.VMEM((ND, F, _LANE), _BF16),
            pltpu.VMEM((4 * ND, D, _LANE), _BF16),
            pltpu.VMEM((6, 8, D), _F32),
            pltpu.VMEM((L, D), _F32),
            pltpu.VMEM((L, H * Dh), _F32),
            pltpu.VMEM((S, D), _F32),
            pltpu.VMEM((S + 2 * _HALO, D), _F32),
            pltpu.VMEM((S, D), _F32),
            pltpu.VMEM((S, D), _F32),
            pltpu.VMEM((S, D), _BF16),
            pltpu.VMEM((2, _TM, D), _BF16),
            pltpu.SemaphoreType.DMA((n_sems,)),
            pltpu.SemaphoreType.DMA((2,)),
        ],
        compiler_params=pltpu.CompilerParams(vmem_limit_bytes=126 * 1024 * 1024),
        name="adaln_rmt_mixer",
    )(
        A_mem0.reshape(M, D), c, A_x.reshape(S, D),
        A_Wq.reshape(D * H, Dh), A_Wk.reshape(D * H, Dh), A_Wv.reshape(D * H, Dh),
        A_Wo.reshape(H * Dh, D), B_w1, B_w2, B_w3, B_w4, w_mod,
    )
    return out.reshape(batch, S, D)
```

```python
import functools
import math

import jax
import jax.numpy as jnp
from jax import lax
import jax.experimental.pallas as pl
import jax.experimental.pallas.tpu as pltpu

_F32 = jnp.float32
_BF16 = jnp.bfloat16
_U32 = jnp.uint32
_LANE = 128
_EPS = 1e-05
_TM = 256
_FC = 512
_HALO = 8
_PRE = 8
_N_PRE = 72
_G = 4


def _dot(a, b):
    return lax.dot_general(a, b, (((1,), (0,)), ((), ())), preferred_element_type=_F32)


def _dot_nt(a, b):
    return lax.dot_general(a, b, (((1,), (1,)), ((), ())), preferred_element_type=_F32)


def _layernorm(x):
    m = jnp.mean(x, axis=-1, keepdims=True)
    d = x - m
    v = jnp.mean(d * d, axis=-1, keepdims=True)
    return d * lax.rsqrt(v + _EPS)


def _gelu(x):
    c = math.sqrt(2.0 / math.pi)
    inner = x * (c + (c * 0.044715) * (x * x))
    hx = 0.5 * x
    return hx + hx * jnp.tanh(inner)


def _aligned(start, size):
    return pl.ds(pl.multiple_of(start, size), size)


def _loop(lo, hi, fn):
    def body(i, carry):
        fn(i)
        return carry
    lax.fori_loop(lo, hi, body, 0)


def _start(cps):
    for cp in cps:
        cp.start()


def _wait(cps):
    for cp in cps:
        cp.wait()


def _kernel(mem0_ref, c_ref, x_hbm, wq_hbm, wk_hbm, wv_hbm, wo_hbm, w1_hbm, w2_hbm, w3_hbm,
            w4_hbm, wmod_hbm, out_hbm,
            x_v, a_s, w1_v, w2_v, w3_v, w4_v, wmodb_v, mod_s, sems):
    n_seg, seg_len, D = x_v.shape
    S = n_seg * seg_len
    M = mem0_ref.shape[0]
    H = wo_hbm.shape[0] // _LANE
    F = w3_hbm.shape[1]
    L = M + seg_len
    ND = D // _LANE
    scale = float(_LANE) ** -0.5
    copy = pltpu.make_async_copy

    cf = c_ref[...].astype(_F32)
    silu_c = jnp.broadcast_to(cf * jax.nn.sigmoid(cf), (8, D))

    n_pre = _N_PRE
    x_head = 8
    cp_x_head = copy(x_hbm.at[pl.ds(0, x_head)], x_v.at[pl.ds(0, x_head)], sems.at[0])
    cp_x_tail = copy(x_hbm.at[pl.ds(x_head, n_seg - x_head)], x_v.at[pl.ds(x_head, n_seg - x_head)],
                     sems.at[6])
    cp_late = [cp_x_tail, copy(wmod_hbm.at[:, pl.ds(2 * D, 4 * D)], wmodb_v, sems.at[1]),
               copy(w1_hbm, w1_v, sems.at[2]), copy(w2_hbm, w2_v, sems.at[3]),
               copy(w3_hbm, w3_v, sems.at[4]), copy(w4_hbm, w4_v, sems.at[5])]

    def attention(wqkv, wo_s, pre_s, moda_s, lhs_s, o_s):

        def load_weights(stage, xq_v, nq_s, hq_s, wmoda_v, w_sems, m_sems, o_sems):
            rows_c = _LANE * H
            words = stage.bitcast(_U32)
            w_hbm = (wq_hbm, wk_hbm, wv_hbm)

            def w_copy(t, j):
                slot = (t % 2) * ND + j
                return copy(w_hbm[t].at[_aligned(j * rows_c, rows_c), :],
                            stage.at[_aligned(slot * rows_c, rows_c), :], w_sems.at[slot])

            def m_copy(j):
                return [copy(wmod_hbm.at[:, _aligned((r * ND + j) * _LANE, _LANE)],
                             wmoda_v.at[r * ND + j], m_sems.at[r * ND + j]) for r in range(2)]

            def modulate(j):
                shift = _dot(silu_c, wmoda_v[j])
                gain = 1.0 + _dot(silu_c, wmoda_v[ND + j])
                moda_s[0, j] = shift
                moda_s[1, j] = gain
                hj = (nq_s[j] * gain[0:1] + shift[0:1]).astype(_BF16)
                hq_s[j] = hj
                return hj

            def absorb(t, j, hj):
                slot = (t % 2) * ND + j
                src = words.at[_aligned(slot * (rows_c // 2), rows_c // 2), :]
                dst = _aligned(j * (_LANE // 2), _LANE // 2)
                for h in range(0, H, _G):
                    tiles = []
                    for hp in range(h // 2, (h + _G) // 2):
                        w = src[pl.ds(hp, _LANE, stride=H // 2), :]
                        tiles.append(pltpu.bitcast(w << 16, _F32).astype(_BF16))
                        tiles.append(pltpu.bitcast(w & jnp.uint32(0xFFFF0000), _F32).astype(_BF16))
                    for i in range(_G):
                        wqkv[t * H + h + i, dst, :] = pltpu.bitcast(tiles[i], _U32)
                    if t * H + h < n_pre:
                        y = _dot(hj, jnp.concatenate(tiles, axis=1))
                        for i in range(_G):
                            pre_s[t * H + h + i] += y[:, i * _LANE:(i + 1) * _LANE]

            cp_xq = copy(x_hbm.at[:, pl.ds(seg_len - _PRE, _PRE), :], xq_v, o_sems.at[ND])
            cp_wo = [copy(wo_hbm.at[:, pl.ds(n * _LANE, _LANE)], wo_s.at[n], o_sems.at[n])
                     for n in range(ND)]

            q_unit = [m_copy(j) + [w_copy(0, j)] for j in range(ND)]
            k_unit = [[w_copy(1, j)] for j in range(ND)]
            v_unit = [[w_copy(2, j)] for j in range(ND)]
            o_unit = [[cp] for cp in cp_wo]
            plan = [q_unit[2] + q_unit[3], q_unit[4], q_unit[5] + q_unit[6], q_unit[7] + k_unit[0],
                    k_unit[1] + k_unit[2], k_unit[3] + k_unit[4], k_unit[5] + k_unit[6],
                    k_unit[7] + v_unit[0],
                    v_unit[1] + v_unit[2] + o_unit[0], v_unit[3] + v_unit[4],
                    v_unit[5] + v_unit[6], v_unit[7] + o_unit[1], o_unit[2] + o_unit[3],
                    o_unit[4] + o_unit[5], o_unit[6] + o_unit[7] + [cp_x_head], cp_late]

            def issue(j, first):
                for i in range(ND):
                    pl.when(j == i)(functools.partial(_start, plan[first + i]))

            with jax.named_scope('sc_first'):
                _start([cp_xq] + q_unit[0])

                def clear(h):
                    pre_s[h] = jnp.zeros(pre_s.shape[1:], _F32)
                _loop(0, n_pre, clear)
                _start(q_unit[1])

                cp_xq.wait()
                nq = _layernorm(xq_v[...].astype(_F32).reshape(n_seg * _PRE, D))
                for j in range(ND):
                    nq_s[j] = nq[:, j * _LANE:(j + 1) * _LANE]

            def q_step(j):
                issue(j, 0)
                _wait(m_copy(j))
                w_copy(0, j).wait()
                absorb(0, j, modulate(j))
            with jax.named_scope('sc_q'):
                _loop(0, ND, q_step)

            def k_step(j):
                issue(j, ND)
                w_copy(1, j).wait()
                absorb(1, j, hq_s[j])
            with jax.named_scope('sc_k'):
                _loop(0, ND, k_step)

            def v_step(j):
                w_copy(2, j).wait()
                absorb(2, j, hq_s[j])
            with jax.named_scope('sc_v'):
                _loop(0, ND, v_step)
            with jax.named_scope('sc_wo'):
                _wait(cp_wo + [cp_x_head])

        pl.run_scoped(
            load_weights,
            pltpu.VMEM((2 * D * H, _LANE), _BF16),
            pltpu.VMEM((n_seg, _PRE, D), _BF16),
            pltpu.VMEM((ND, n_seg * _PRE, _LANE), _F32),
            pltpu.VMEM((ND, n_seg * _PRE, _LANE), _BF16),
            pltpu.VMEM((2 * ND, D, _LANE), _BF16),
            pltpu.SemaphoreType.DMA((2 * ND,)),
            pltpu.SemaphoreType.DMA((2 * ND,)),
            pltpu.SemaphoreType.DMA((ND + 1,)),
        )
        for r in range(2):
            mod_s[r] = jnp.concatenate([moda_s[r, j] for j in range(ND)], axis=1)

        def seg_input(s):
            return _layernorm(x_v[s].astype(_F32)) * mod_s[1, 0:1, :] + mod_s[0, 0:1, :]

        lhs_s[0:M, :] = mem0_ref[...].astype(_F32)
        lhs_s[M:L, :] = seg_input(0)

        row = lax.broadcasted_iota(jnp.int32, (L, L), 0)
        col = lax.broadcasted_iota(jnp.int32, (L, L), 1)
        mask = (row < M) | (row >= col)

        def seg_step(s):
            pl.when(s == x_head - 1)(cp_x_tail.wait)
            lhs = lhs_s[...]
            lhs_short = lhs[0:L - _PRE].astype(_BF16)
            pre_rows = _aligned(s * _PRE, _PRE)

            def proj_rows(a, first):
                w = jnp.concatenate([pltpu.bitcast(wqkv[first + i], _BF16) for i in range(_G)],
                                    axis=1)
                y = _dot(a, w)
                return [y[:, i * _LANE:(i + 1) * _LANE] for i in range(_G)]

            def proj(first):
                if first >= n_pre:
                    return proj_rows(lhs, first)
                return [jnp.concatenate([t, pre_s[first + i, pre_rows, :]], axis=0)
                        for i, t in enumerate(proj_rows(lhs_short, first))]

            def weights(q, k):
                sc = jnp.where(mask, _dot_nt(q, k.astype(_BF16)) * scale, -1000000000.0)
                e = jnp.exp(sc - jnp.max(sc, axis=-1, keepdims=True))
                return e, jnp.sum(e, axis=-1, keepdims=True)

            def mix(h0, ws, vs):
                for i, ((e, den), v) in enumerate(zip(ws, vs)):
                    o_s[:, (h0 + i) * _LANE:(h0 + i + 1) * _LANE] = _dot(e, v.astype(_BF16)) / den

            def out_proj(h0, h1):
                ks = slice(h0 * _LANE, h1 * _LANE)
                return _dot(o_s[:, ks], jnp.concatenate([wo_s[n, ks, :] for n in range(ND)], axis=1))

            pend = None
            for h in range(0, H, _G):
                qs = proj(h)
                ks = proj(H + h)
                if pend is not None:
                    mix(*pend)
                vs = proj(2 * H + h)
                pend = (h, [weights(q, k) for q, k in zip(qs, ks)], vs)
            nxt = seg_input(jnp.minimum(s + 1, n_seg - 1))
            y = out_proj(0, 2 * _G)
            mix(*pend)
            y = out_proj(2 * _G, H) + y
            lhs_s[0:M, :] = y[0:M]
            a_s[_aligned(s * seg_len, seg_len), :] = y[M:L]
            lhs_s[M:L, :] = nxt

        with jax.named_scope('sc_attn'):
            _loop(0, n_seg, seg_step)

    pl.run_scoped(
        attention,
        pltpu.VMEM((3 * H, D // 2, _LANE), _U32),
        pltpu.VMEM((ND, H * _LANE, _LANE), _BF16),
        pltpu.VMEM((n_pre, n_seg * _PRE, _LANE), _F32),
        pltpu.VMEM((2, ND, 8, _LANE), _F32),
        pltpu.VMEM((L, D), _F32),
        pltpu.VMEM((L, H * _LANE), _F32),
    )

    def mixer(g_s, hb_s, n1_s, out_s, out_sems):
        _wait(cp_late[1:])
        for r in range(4):
            mod_s[2 + r] = _dot(silu_c, wmodb_v[:, r * D:(r + 1) * D])
        g_s[0:_HALO, :] = jnp.zeros((_HALO, D), _F32)
        g_s[_HALO + S:_HALO + S + _HALO, :] = jnp.zeros((_HALO, D), _F32)
        n_blk = S // _TM
        seg_blk = _TM // seg_len
        cq = D // 4

        def stage1(i):
            rows = _aligned(i * _TM, _TM)
            x = x_v[pl.ds(i * seg_blk, seg_blk)].astype(_F32).reshape(_TM, D)
            xm = x + mod_s[2, 0:1, :] * a_s[rows, :]
            a_s[rows, :] = xm
            hb = _layernorm(xm) * (1.0 + mod_s[4, 0:1, :]) + mod_s[3, 0:1, :]
            hb_s[rows, :] = hb
            g = _gelu(_dot(_layernorm(hb).astype(_BF16), w1_v[...]))
            g_s[pl.ds(pl.multiple_of(i * _TM + _HALO, 8), _TM), :] = g

        def stage2(i):
            rows = _aligned(i * _TM, _TM)
            win = g_s.at[pl.ds(pl.multiple_of(i * _TM, _TM), _TM + 2 * _HALO), :]
            parts = [win[_HALO + off:_HALO + off + _TM, j * cq:(j + 1) * cq]
                     for j, off in enumerate((-1, 1, -2, 2))]
            shifted = jnp.concatenate(parts, axis=1).astype(_BF16)
            x1 = hb_s[rows, :] + _dot(shifted, w2_v[...])
            return rows, x1

        def stage2_store(rows, x1):
            hb_s[rows, :] = x1
            n1_s[rows, :] = _layernorm(x1).astype(_BF16)

        def stage12(i):
            done = stage2(i)
            stage1(i + 2)
            stage2_store(*done)

        def out_copy(i, slot):
            return copy(out_s.at[slot], out_hbm.at[_aligned(i * _TM, _TM), :], out_sems.at[slot])

        def stage3(i):
            slot = i % 2

            @pl.when(i >= 2)
            def _():
                out_copy(jnp.maximum(i - 2, 0), slot).wait()

            rows = _aligned(i * _TM, _TM)
            n1 = n1_s[rows, :]
            acc = hb_s[rows, :]
            for f in range(0, F, _FC):
                u = _gelu(_dot(n1, w3_v[:, f:f + _FC])).astype(_BF16)
                acc = acc + _dot(u, w4_v[f:f + _FC, :])
            out_s[slot] = (a_s[rows, :] + mod_s[5, 0:1, :] * acc).astype(out_s.dtype)
            out_copy(i, slot).start()

        with jax.named_scope('sc_s1'):
            stage1(0)
            stage1(1)
        with jax.named_scope('sc_s12'):
            _loop(0, n_blk - 2, stage12)
        with jax.named_scope('sc_s2'):
            last = [stage2(i) for i in (n_blk - 2, n_blk - 1)]
            for done in last:
                stage2_store(*done)
        with jax.named_scope('sc_s3'):
            _loop(0, n_blk, stage3)
        for i in (n_blk - 2, n_blk - 1):
            out_copy(i, i % 2).wait()

    pl.run_scoped(
        mixer,
        pltpu.VMEM((S + 2 * _HALO, D), _F32),
        pltpu.VMEM((S, D), _F32),
        pltpu.VMEM((S, D), _BF16),
        pltpu.VMEM((2, _TM, D), _BF16),
        pltpu.SemaphoreType.DMA((2,)),
    )


@functools.partial(jax.jit, static_argnames=("A_seg_len",))
def pallas_adaLN_cond__memory_aug_recurrent_mem_tr__mixer_s_mlp__prompt_kernel(
    A_x: jax.Array,
    A_mem0: jax.Array,
    A_Wq: jax.Array,
    A_Wk: jax.Array,
    A_Wv: jax.Array,
    A_Wo: jax.Array,
    A_seg_len: int,
    B_x: jax.Array,
    B_w1: jax.Array,
    B_w2: jax.Array,
    B_w3: jax.Array,
    B_w4: jax.Array,
    c: jax.Array,
    w_mod: jax.Array,
):
    del B_x
    batch, S, D = A_x.shape
    _, H, Dh = A_Wq.shape
    M = A_mem0.shape[1]
    F = B_w3.shape[1]
    seg_len = int(A_seg_len)
    assert batch == 1 and Dh == _LANE and S % _TM == 0 and _TM % seg_len == 0 and F % _FC == 0
    n_seg = S // seg_len

    vmem = pl.BlockSpec(memory_space=pltpu.VMEM)
    hbm = pl.BlockSpec(memory_space=pl.ANY)
    out = pl.pallas_call(
        _kernel,
        out_shape=jax.ShapeDtypeStruct((S, D), A_x.dtype),
        in_specs=[vmem, vmem] + [hbm] * 10,
        out_specs=hbm,
        scratch_shapes=[
            pltpu.VMEM((n_seg, seg_len, D), _BF16),
            pltpu.VMEM((S, D), _F32),
            pltpu.VMEM((D, D), _BF16),
            pltpu.VMEM((D, D), _BF16),
            pltpu.VMEM((D, F), _BF16),
            pltpu.VMEM((F, D), _BF16),
            pltpu.VMEM((D, 4 * D), _BF16),
            pltpu.VMEM((6, 8, D), _F32),
            pltpu.SemaphoreType.DMA((7,)),
        ],
        compiler_params=pltpu.CompilerParams(vmem_limit_bytes=126 * 1024 * 1024),
        name="adaln_rmt_mixer",
    )(
        A_mem0.reshape(M, D), c, A_x.reshape(n_seg, seg_len, D),
        A_Wq.reshape(D * H, Dh), A_Wk.reshape(D * H, Dh), A_Wv.reshape(D * H, Dh),
        A_Wo.reshape(H * Dh, D), B_w1, B_w2, B_w3, B_w4, w_mod,
    )
    return out.reshape(batch, S, D)
```

```python
import functools
import math

import jax
import jax.numpy as jnp
from jax import lax
import jax.experimental.pallas as pl
import jax.experimental.pallas.tpu as pltpu

_F32 = jnp.float32
_BF16 = jnp.bfloat16
_U32 = jnp.uint32
_LANE = 128
_EPS = 1e-05
_TM = 256
_LEVEL = 2
_UNROLL = 2
_HALO = 8
_PRE = 8
_N_PRE = 64
_G = 4


def _dot(a, b):
    return lax.dot_general(a, b, (((1,), (0,)), ((), ())), preferred_element_type=_F32)


def _dot_nt(a, b):
    return lax.dot_general(a, b, (((1,), (1,)), ((), ())), preferred_element_type=_F32)


def _layernorm(x):
    m = jnp.mean(x, axis=-1, keepdims=True)
    d = x - m
    v = jnp.mean(d * d, axis=-1, keepdims=True)
    return d * lax.rsqrt(v + _EPS)


def _gelu(x):
    c = math.sqrt(2.0 / math.pi)
    inner = x * (c + (c * 0.044715) * (x * x))
    hx = 0.5 * x
    return hx + hx * jnp.tanh(inner)


def _pack(x):
    return pltpu.bitcast(x.astype(_BF16), _U32)


def _unpacked(x):
    return pltpu.bitcast(x, _BF16)


def _quads(g):
    n = len(g) // 2
    return [[row[j * n:(j + 1) * n] for row in g[i * n:(i + 1) * n]]
            for i in range(2) for j in range(2)]


def _add(a, b):
    return [[x + y for x, y in zip(r, t)] for r, t in zip(a, b)]


def _sub(a, b):
    return [[x - y for x, y in zip(r, t)] for r, t in zip(a, b)]


def _lhs_terms(g):
    if len(g) == 1:
        return [g[0][0]]
    a11, a12, a21, a22 = _quads(g)
    terms = (_sub(a11, a22), _sub(a21, a22), a22, _sub(a21, a11), _sub(a22, a12), a11,
             _sub(a11, a12))
    return [v for t in terms for v in _lhs_terms(t)]


def _rhs_terms(g):
    if len(g) == 1:
        return [g[0][0]]
    b11, b12, b21, b22 = _quads(g)
    terms = (_sub(b11, b22), b11, _add(b21, b11), _add(b11, b12), _add(b21, b22), _add(b12, b22),
             b22)
    return [v for t in terms for v in _rhs_terms(t)]


def _combine(level, product, base=0):
    if level == 0:
        return [[product(base)]]

    def m(i):
        return _combine(level - 1, product, base + i * 7 ** (level - 1))

    m0, m1 = m(0), m(1)
    c22 = _sub(m0, m1)
    m2 = m(2)
    c21, c11 = _add(m1, m2), _add(m0, m2)
    c22 = _add(m(3), c22)
    c11 = _sub(c11, m(4))
    m5 = m(5)
    c22 = _add(c22, m5)
    m6 = m(6)
    c12, c11 = _sub(m5, m6), _add(c11, m6)
    return [x + y for x, y in zip(c11, c12)] + [x + y for x, y in zip(c21, c22)]


def _aligned(start, size):
    return pl.ds(pl.multiple_of(start, size), size)


def _loop(lo, hi, fn):
    def body(i, carry):
        fn(i)
        return carry
    lax.fori_loop(lo, hi, body, 0)


def _start(cps):
    for cp in cps:
        cp.start()


def _wait(cps):
    for cp in cps:
        cp.wait()


def _kernel(mem0_ref, c_ref, x_hbm, wq_hbm, wk_hbm, wv_hbm, wo_hbm, w1_hbm, w2_hbm, w3_hbm,
            w4_hbm, wmod_hbm, out_hbm,
            x_v, a_s, w1_v, w2_v, w3_v, w4_v, wmodb_v, mod_s, sems):
    n_seg, seg_len, D = x_v.shape
    S = n_seg * seg_len
    M = mem0_ref.shape[0]
    H = wo_hbm.shape[0] // _LANE
    F = w3_hbm.shape[1]
    L = M + seg_len
    ND = D // _LANE
    scale = float(_LANE) ** -0.5
    copy = pltpu.make_async_copy

    cf = c_ref[...].astype(_F32)
    silu_c = jnp.broadcast_to(cf * jax.nn.sigmoid(cf), (8, D))

    n_pre = _N_PRE
    x_head = 8
    cp_x_head = copy(x_hbm.at[pl.ds(0, x_head)], x_v.at[pl.ds(0, x_head)], sems.at[0])
    cp_x_tail = copy(x_hbm.at[pl.ds(x_head, n_seg - x_head)], x_v.at[pl.ds(x_head, n_seg - x_head)],
                     sems.at[6])
    cp_late = [cp_x_tail, copy(wmod_hbm.at[:, pl.ds(2 * D, 4 * D)], wmodb_v, sems.at[1]),
               copy(w1_hbm, w1_v, sems.at[2]), copy(w2_hbm, w2_v, sems.at[3]),
               copy(w3_hbm, w3_v, sems.at[4]), copy(w4_hbm, w4_v, sems.at[5])]

    def attention(wqkv, wo_s, pre_s, moda_s, lhs_s, o_s):

        def load_weights(stage, xq_v, nq_s, hq_s, wmoda_v, w_sems, m_sems, o_sems):
            rows_c = _LANE * H
            words = stage.bitcast(_U32)
            w_hbm = (wq_hbm, wk_hbm, wv_hbm)

            def w_copy(t, j):
                slot = (t % 2) * ND + j
                return copy(w_hbm[t].at[_aligned(j * rows_c, rows_c), :],
                            stage.at[_aligned(slot * rows_c, rows_c), :], w_sems.at[slot])

            def m_copy(j):
                return [copy(wmod_hbm.at[:, _aligned((r * ND + j) * _LANE, _LANE)],
                             wmoda_v.at[r * ND + j], m_sems.at[r * ND + j]) for r in range(2)]

            def modulate(j):
                shift = _dot(silu_c, wmoda_v[j])
                gain = 1.0 + _dot(silu_c, wmoda_v[ND + j])
                moda_s[0, j] = shift
                moda_s[1, j] = gain
                hj = (nq_s[j] * gain[0:1] + shift[0:1]).astype(_BF16)
                hq_s[j] = hj
                return hj

            def absorb(t, j, hj):
                slot = (t % 2) * ND + j
                src = words.at[_aligned(slot * (rows_c // 2), rows_c // 2), :]
                dst = _aligned(j * (_LANE // 2), _LANE // 2)
                for h in range(0, H, _G):
                    tiles = []
                    for hp in range(h // 2, (h + _G) // 2):
                        w = src[pl.ds(hp, _LANE, stride=H // 2), :]
                        tiles.append(pltpu.bitcast(w << 16, _F32).astype(_BF16))
                        tiles.append(pltpu.bitcast(w & jnp.uint32(0xFFFF0000), _F32).astype(_BF16))
                    for i in range(_G):
                        wqkv[t * H + h + i, dst, :] = pltpu.bitcast(tiles[i], _U32)
                    if t * H + h < n_pre:
                        y = _dot(hj, jnp.concatenate(tiles, axis=1))
                        for i in range(_G):
                            pre_s[t * H + h + i] += y[:, i * _LANE:(i + 1) * _LANE]

            cp_xq = copy(x_hbm.at[:, pl.ds(seg_len - _PRE, _PRE), :], xq_v, o_sems.at[ND])
            cp_wo = [copy(wo_hbm.at[:, pl.ds(n * _LANE, _LANE)], wo_s.at[n], o_sems.at[n])
                     for n in range(ND)]

            q_unit = [m_copy(j) + [w_copy(0, j)] for j in range(ND)]
            k_unit = [[w_copy(1, j)] for j in range(ND)]
            v_unit = [[w_copy(2, j)] for j in range(ND)]
            o_unit = [[cp] for cp in cp_wo]
            plan = [q_unit[2] + q_unit[3], q_unit[4], q_unit[5] + q_unit[6], q_unit[7] + k_unit[0],
                    k_unit[1] + k_unit[2], k_unit[3] + k_unit[4], k_unit[5] + k_unit[6],
                    k_unit[7] + v_unit[0],
                    v_unit[1] + v_unit[2] + o_unit[0], v_unit[3] + v_unit[4],
                    v_unit[5] + v_unit[6], v_unit[7] + o_unit[1], o_unit[2] + o_unit[3],
                    o_unit[4] + o_unit[5], o_unit[6] + o_unit[7] + [cp_x_head], cp_late]

            def issue(j, first):
                for i in range(ND):
                    pl.when(j == i)(functools.partial(_start, plan[first + i]))

            with jax.named_scope('sc_first'):
                _start([cp_xq] + q_unit[0])

                def clear(h):
                    pre_s[h] = jnp.zeros(pre_s.shape[1:], _F32)
                _loop(0, n_pre, clear)
                _start(q_unit[1])

                cp_xq.wait()
                nq = _layernorm(xq_v[...].astype(_F32).reshape(n_seg * _PRE, D))
                for j in range(ND):
                    nq_s[j] = nq[:, j * _LANE:(j + 1) * _LANE]

            def q_step(j):
                issue(j, 0)
                _wait(m_copy(j))
                w_copy(0, j).wait()
                absorb(0, j, modulate(j))
            with jax.named_scope('sc_q'):
                _loop(0, ND, q_step)

            def k_step(j):
                issue(j, ND)
                w_copy(1, j).wait()
                absorb(1, j, hq_s[j])
            with jax.named_scope('sc_k'):
                _loop(0, ND, k_step)

            def v_step(j):
                w_copy(2, j).wait()
                absorb(2, j, hq_s[j])
            with jax.named_scope('sc_v'):
                _loop(0, ND, v_step)
            with jax.named_scope('sc_wo'):
                _wait(cp_wo + [cp_x_head])

        pl.run_scoped(
            load_weights,
            pltpu.VMEM((2 * D * H, _LANE), _BF16),
            pltpu.VMEM((n_seg, _PRE, D), _BF16),
            pltpu.VMEM((ND, n_seg * _PRE, _LANE), _F32),
            pltpu.VMEM((ND, n_seg * _PRE, _LANE), _BF16),
            pltpu.VMEM((2 * ND, D, _LANE), _BF16),
            pltpu.SemaphoreType.DMA((2 * ND,)),
            pltpu.SemaphoreType.DMA((2 * ND,)),
            pltpu.SemaphoreType.DMA((ND + 1,)),
        )
        for r in range(2):
            mod_s[r] = jnp.concatenate([moda_s[r, j] for j in range(ND)], axis=1)

        def seg_input(s):
            return _layernorm(x_v[s].astype(_F32)) * mod_s[1, 0:1, :] + mod_s[0, 0:1, :]

        lhs_s[0:M, :] = mem0_ref[...].astype(_F32)
        lhs_s[M:L, :] = seg_input(0)

        row = lax.broadcasted_iota(jnp.int32, (L, L), 0)
        col = lax.broadcasted_iota(jnp.int32, (L, L), 1)
        mask = (row < M) | (row >= col)

        def seg_step(s, mem, seg):
            half = D // 2
            lhs = [jnp.concatenate([mem[i], seg[:, i * half:(i + 1) * half]], axis=0)
                   for i in range(2)]
            lhs_short = [t[0:L - _PRE].astype(_BF16) for t in lhs]
            pre_rows = _aligned(s * _PRE, _PRE)

            def proj_part(first, parts):
                rows = slice(parts[0] * half // 2, (parts[-1] + 1) * half // 2)
                src = lhs_short if first < n_pre else lhs
                a = jnp.concatenate([src[i] for i in parts], axis=1)
                w = jnp.concatenate([_unpacked(wqkv[first + i, rows, :]) for i in range(_G)], axis=1)
                return _dot(a, w)

            def heads(first, y):
                ts = [y[:, i * _LANE:(i + 1) * _LANE] for i in range(_G)]
                if first >= n_pre:
                    return ts
                return [jnp.concatenate([t, pre_s[first + i, pre_rows, :]], axis=0)
                        for i, t in enumerate(ts)]

            def proj(first):
                return heads(first, proj_part(first, (0, 1)))

            def weights(q, k):
                sc = jnp.where(mask, _dot_nt(q, k.astype(_BF16)) * scale, -1000000000.0)
                e = jnp.exp(sc - jnp.max(sc, axis=-1, keepdims=True))
                return e, jnp.sum(e, axis=-1, keepdims=True)

            def mix(h0, ws, vs):
                for i, ((e, den), v) in enumerate(zip(ws, vs)):
                    o_s[:, (h0 + i) * _LANE:(h0 + i + 1) * _LANE] = _dot(e, v.astype(_BF16)) / den

            def out_proj(h0, h1, part):
                ks = slice(h0 * _LANE, h1 * _LANE)
                cols = range(part * ND // 2, (part + 1) * ND // 2)
                return _dot(o_s[:, ks], jnp.concatenate([wo_s[n, ks, :] for n in cols], axis=1))

            pend = None
            for h in range(0, H, _G):
                if pend is None:
                    q0, k0 = proj_part(h, (0,)), proj_part(H + h, (0,))
                    qs = heads(h, proj_part(h, (1,)) + q0)
                    ks = heads(H + h, proj_part(H + h, (1,)) + k0)
                else:
                    qs, ks = proj(h), proj(H + h)
                    mix(*pend)
                vs = proj(2 * H + h)
                pend = (h, [weights(q, k) for q, k in zip(qs, ks)], vs)
            nxt = seg_input(jnp.minimum(s + 1, n_seg - 1))
            y0 = out_proj(0, 6 * _G, 0)
            mix(*pend)
            y1 = out_proj(0, 2 * _G, 1)
            y0 = out_proj(6 * _G, H, 0) + y0
            y1 = out_proj(2 * _G, H, 1) + y1
            for i, y in enumerate((y0, y1)):
                a_s[_aligned(s * seg_len, seg_len), i * half:(i + 1) * half] = y[M:L]
            return (y0[0:M], y1[0:M]), nxt

        def seg_steps(i):
            pl.when(i == x_head // _UNROLL - 1)(cp_x_tail.wait)
            mem, seg = (lhs_s[0:M, 0:D // 2], lhs_s[0:M, D // 2:D]), lhs_s[M:L, :]
            for u in range(_UNROLL):
                mem, seg = seg_step(i * _UNROLL + u, mem, seg)
            lhs_s[0:M, 0:D // 2] = mem[0]
            lhs_s[0:M, D // 2:D] = mem[1]
            lhs_s[M:L, :] = seg

        with jax.named_scope('sc_attn'):
            _loop(0, n_seg // _UNROLL, seg_steps)

    pl.run_scoped(
        attention,
        pltpu.VMEM((3 * H, D // 2, _LANE), _U32),
        pltpu.VMEM((ND, H * _LANE, _LANE), _BF16),
        pltpu.VMEM((n_pre, n_seg * _PRE, _LANE), _F32),
        pltpu.VMEM((2, ND, 8, _LANE), _F32),
        pltpu.VMEM((L, D), _F32),
        pltpu.VMEM((L, H * _LANE), _F32),
    )

    P = 2 ** _LEVEL
    T = 7 ** _LEVEL
    mq, dq, fq = _TM // P, D // P, F // P

    def mixer(g_s, hb_s, t3_s, t4_s, a1_s, a2_s, out_s, out_sems):
        _wait(cp_late[1:])
        for r in range(4):
            mod_s[2 + r] = _dot(silu_c, wmodb_v[:, r * D:(r + 1) * D])
        g_s[0:_HALO, :] = jnp.zeros((_HALO, D), _F32)
        g_s[_HALO + S:_HALO + S + _HALO, :] = jnp.zeros((_HALO, D), _F32)
        n_blk = S // _TM
        seg_blk = _TM // seg_len
        cq = D // 4

        def norm_in(i):
            out = []
            for t in range(i * seg_blk, (i + 1) * seg_blk):
                rows = slice(t * seg_len, (t + 1) * seg_len)
                xm = x_v[t].astype(_F32) + mod_s[2, 0:1, :] * a_s[rows, :]
                a_s[rows, :] = xm
                hb = _layernorm(xm) * (1.0 + mod_s[4, 0:1, :]) + mod_s[3, 0:1, :]
                hb_s[rows, :] = hb
                out.append(_layernorm(hb).astype(_BF16))
            return jnp.concatenate(out, axis=0)

        def gate(i, n0):
            g_s[_HALO + i * _TM:_HALO + (i + 1) * _TM, :] = _gelu(_dot(n0, w1_v[...]))

        def shift_mix(i):
            parts = [g_s[_HALO + i * _TM + off:_HALO + (i + 1) * _TM + off, j * cq:(j + 1) * cq]
                     for j, off in enumerate((-1, 1, -2, 2))]
            shifted = jnp.concatenate(parts, axis=1).astype(_BF16)
            rows = slice(i * _TM, (i + 1) * _TM)
            hb_s[rows, :] = _dot(shifted, w2_v[...]) + hb_s[rows, :]

        def weight_terms(src, dst, r, col):
            nr, nc = src.shape[0] // P, src.shape[1] // P
            g = [[src[a * nr + r:a * nr + r + 16, b * nc + col:b * nc + col + _LANE].astype(_F32)
                  for b in range(P)] for a in range(P)]
            for t, v in enumerate(_rhs_terms(g)):
                dst[t, r // 2:r // 2 + 8, col:col + _LANE] = _pack(v)

        jobs = [(w3_v, t3_s, r, col) for col in range(0, fq, _LANE) for r in range(0, dq, 16)]
        jobs += [(w4_v, t4_s, r, col) for col in range(0, dq, _LANE) for r in range(0, fq, 16)]
        per_blk = -(-len(jobs) // n_blk)

        def mlp_terms(i):
            for r in range(0, mq, 16):
                n1 = [_layernorm(hb_s[_aligned(i * _TM + a * mq + r, 16), :]) for a in range(P)]
                for col in range(0, dq, _LANE):
                    g = [[n[:, b * dq + col:b * dq + col + _LANE] for b in range(P)] for n in n1]
                    for t, v in enumerate(_lhs_terms(g)):
                        a1_s[t, r // 2:r // 2 + 8, col:col + _LANE] = _pack(v)

        def out_copy(i, slot):
            return copy(out_s.at[slot], out_hbm.at[_aligned(i * _TM, _TM), :], out_sems.at[slot])

        def mlp(i):
            slot = i % 2

            @pl.when(i >= 2)
            def _():
                out_copy(jnp.maximum(i - 2, 0), slot).wait()

            for col in range(0, fq, _LANE):
                cols = slice(col, col + _LANE)
                g = _combine(_LEVEL, lambda t: _dot(_unpacked(a1_s[t]), _unpacked(t3_s[t, :, cols])))
                for t, v in enumerate(_lhs_terms([[_gelu(y) for y in r] for r in g])):
                    a2_s[t, :, cols] = _pack(v)
            mlp_terms(jnp.minimum(i + 1, n_blk - 1))
            for col in range(0, dq, _LANE):
                cols = slice(col, col + _LANE)
                g = _combine(_LEVEL, lambda t: _dot(_unpacked(a2_s[t]), _unpacked(t4_s[t, :, cols])))
                for a in range(P):
                    rows = _aligned(i * _TM + a * mq, mq)
                    for b in range(P):
                        oc = slice(b * dq + col, b * dq + col + _LANE)
                        y = a_s[rows, oc] + mod_s[5, 0:1, oc] * (hb_s[rows, oc] + g[a][b])
                        out_s[slot, a * mq:(a + 1) * mq, oc] = y.astype(out_s.dtype)
            out_copy(i, slot).start()

        with jax.named_scope('sc_s12'):
            n0 = norm_in(0)
            for i in range(n_blk + 2):
                if i < n_blk:
                    gate(i, n0)
                if i + 1 < n_blk:
                    n0 = norm_in(i + 1)
                if i >= 2:
                    shift_mix(i - 2)
                    for job in jobs[(i - 2) * per_blk:(i - 1) * per_blk]:
                        weight_terms(*job)
                if i == n_blk:
                    mlp_terms(0)
        with jax.named_scope('sc_s3'):
            _loop(0, n_blk, mlp)
        for i in (n_blk - 2, n_blk - 1):
            out_copy(i, i % 2).wait()

    pl.run_scoped(
        mixer,
        pltpu.VMEM((S + 2 * _HALO, D), _F32),
        pltpu.VMEM((S, D), _F32),
        pltpu.VMEM((T, dq // 2, fq), _U32),
        pltpu.VMEM((T, fq // 2, dq), _U32),
        pltpu.VMEM((T, mq // 2, dq), _U32),
        pltpu.VMEM((T, mq // 2, fq), _U32),
        pltpu.VMEM((2, _TM, D), _BF16),
        pltpu.SemaphoreType.DMA((2,)),
    )


@functools.partial(jax.jit, static_argnames=("A_seg_len",))
def pallas_adaLN_cond__memory_aug_recurrent_mem_tr__mixer_s_mlp__prompt_kernel(
    A_x: jax.Array,
    A_mem0: jax.Array,
    A_Wq: jax.Array,
    A_Wk: jax.Array,
    A_Wv: jax.Array,
    A_Wo: jax.Array,
    A_seg_len: int,
    B_x: jax.Array,
    B_w1: jax.Array,
    B_w2: jax.Array,
    B_w3: jax.Array,
    B_w4: jax.Array,
    c: jax.Array,
    w_mod: jax.Array,
):
    del B_x
    batch, S, D = A_x.shape
    _, H, Dh = A_Wq.shape
    M = A_mem0.shape[1]
    F = B_w3.shape[1]
    seg_len = int(A_seg_len)
    assert batch == 1 and Dh == _LANE and S % _TM == 0 and _TM % seg_len == 0
    n_seg = S // seg_len

    vmem = pl.BlockSpec(memory_space=pltpu.VMEM)
    hbm = pl.BlockSpec(memory_space=pl.ANY)
    out = pl.pallas_call(
        _kernel,
        out_shape=jax.ShapeDtypeStruct((S, D), A_x.dtype),
        in_specs=[vmem, vmem] + [hbm] * 10,
        out_specs=hbm,
        scratch_shapes=[
            pltpu.VMEM((n_seg, seg_len, D), _BF16),
            pltpu.VMEM((S, D), _F32),
            pltpu.VMEM((D, D), _BF16),
            pltpu.VMEM((D, D), _BF16),
            pltpu.VMEM((D, F), _BF16),
            pltpu.VMEM((F, D), _BF16),
            pltpu.VMEM((D, 4 * D), _BF16),
            pltpu.VMEM((6, 8, D), _F32),
            pltpu.SemaphoreType.DMA((7,)),
        ],
        compiler_params=pltpu.CompilerParams(vmem_limit_bytes=126 * 1024 * 1024),
        name="adaln_rmt_mixer",
    )(
        A_mem0.reshape(M, D), c, A_x.reshape(n_seg, seg_len, D),
        A_Wq.reshape(D * H, Dh), A_Wk.reshape(D * H, Dh), A_Wv.reshape(D * H, Dh),
        A_Wo.reshape(H * Dh, D), B_w1, B_w2, B_w3, B_w4, w_mod,
    )
    return out.reshape(batch, S, D)
```

```python
import functools
import math

import jax
import jax.numpy as jnp
from jax import lax
import jax.experimental.pallas as pl
import jax.experimental.pallas.tpu as pltpu

_F32 = jnp.float32
_BF16 = jnp.bfloat16
_U32 = jnp.uint32
_LANE = 128
_EPS = 1e-05
_TM = 256
_LEVEL = 2
_UNROLL = 1
_HALO = 8
_PRE = 8
_G = 4


def _dot(a, b):
    return lax.dot_general(a, b, (((1,), (0,)), ((), ())), preferred_element_type=_F32)


def _dot_nt(a, b):
    return lax.dot_general(a, b, (((1,), (1,)), ((), ())), preferred_element_type=_F32)


def _layernorm(x):
    m = jnp.mean(x, axis=-1, keepdims=True)
    d = x - m
    v = jnp.mean(d * d, axis=-1, keepdims=True)
    return d * lax.rsqrt(v + _EPS)


def _gelu(x):
    c = math.sqrt(2.0 / math.pi)
    inner = x * (c + (c * 0.044715) * (x * x))
    hx = 0.5 * x
    return hx + hx * jnp.tanh(inner)


def _pack(x):
    return pltpu.bitcast(x.astype(_BF16), _U32)


def _unpacked(x):
    return pltpu.bitcast(x, _BF16)


def _low_half(w):
    return pltpu.bitcast(w << 16, _F32)


def _high_half(w):
    return pltpu.bitcast(w & jnp.uint32(0xFFFF0000), _F32)


def _quads(g):
    n = len(g) // 2
    return [[row[j * n:(j + 1) * n] for row in g[i * n:(i + 1) * n]]
            for i in range(2) for j in range(2)]


def _add(a, b):
    return [[x + y for x, y in zip(r, t)] for r, t in zip(a, b)]


def _sub(a, b):
    return [[x - y for x, y in zip(r, t)] for r, t in zip(a, b)]


def _lhs_terms(g):
    if len(g) == 1:
        return [g[0][0]]
    a11, a12, a21, a22 = _quads(g)
    terms = (_sub(a11, a22), _sub(a21, a22), a22, _sub(a21, a11), _sub(a22, a12), a11,
             _sub(a11, a12))
    return [v for t in terms for v in _lhs_terms(t)]


def _rhs_terms(g):
    if len(g) == 1:
        return [g[0][0]]
    b11, b12, b21, b22 = _quads(g)
    terms = (_sub(b11, b22), b11, _add(b21, b11), _add(b11, b12), _add(b21, b22), _add(b12, b22),
             b22)
    return [v for t in terms for v in _rhs_terms(t)]


def _combine(level, product, base=0, emit=None):
    if level == 0:
        return [[product(base)]]

    def m(i):
        return _combine(level - 1, product, base + i * 7 ** (level - 1))

    def done(qi, qj, g):
        if emit is None:
            return g
        n = len(g)
        return [[emit(qi * n + a, qj * n + b, g[a][b]) for b in range(n)] for a in range(n)]

    m0, m1 = m(0), m(1)
    c22 = _sub(m0, m1)
    m2 = m(2)
    c11 = _add(m0, m2)
    c21 = done(1, 0, _add(m1, m2))
    m5 = m(5)
    c22 = _add(c22, m5)
    m6 = m(6)
    c11 = _add(c11, m6)
    c12 = done(0, 1, _sub(m5, m6))
    c22 = done(1, 1, _add(m(3), c22))
    c11 = done(0, 0, _sub(c11, m(4)))
    return [x + y for x, y in zip(c11, c12)] + [x + y for x, y in zip(c21, c22)]


def _aligned(start, size):
    return pl.ds(pl.multiple_of(start, size), size)


def _cols(j, n=_LANE):
    return slice(j * n, (j + 1) * n)


def _loop(lo, hi, fn):
    def body(i, carry):
        fn(i)
        return carry
    lax.fori_loop(lo, hi, body, 0)


def _start(cps):
    for cp in cps:
        cp.start()


def _wait(cps):
    for cp in cps:
        cp.wait()


def _kernel(mem0_ref, c_ref, x_hbm, wq_hbm, wk_hbm, wv_hbm, wo_hbm, w1_hbm, w2_hbm, w3_hbm,
            w4_hbm, wmod_hbm, out_hbm, x_v, a_s, mod_s, zero_s, sems):
    n_seg, seg_len, D = x_v.shape
    S = n_seg * seg_len
    M = mem0_ref.shape[0]
    H = wo_hbm.shape[0] // _LANE
    F = w3_hbm.shape[1]
    L = M + seg_len
    ND = D // _LANE
    P = 2 ** _LEVEL
    T = 7 ** _LEVEL
    mq, dq, fq = _TM // P, D // P, F // P
    scale = float(_LANE) ** -0.5
    copy = pltpu.make_async_copy

    def mod(r, cols=slice(None)):
        return mod_s[r, 0:1, cols]

    zero_s[...] = jnp.zeros(zero_s.shape, _U32)

    def paced(w, jobs):
        step = w.shape[0] // (_LANE // 2) // max(len(jobs), 1) * (_LANE // 2)
        parts = []
        for n, job in enumerate(jobs):
            tiles = [pltpu.bitcast(v, _U32)[r:r + 8, c:c + _LANE] for v in job()
                     for r in range(0, v.shape[0], 8) for c in range(0, v.shape[1], _LANE)]
            done = functools.reduce(jnp.bitwise_or, tiles) & zero_s[...]
            parts += [w[n * step:n * step + 8] | done, w[n * step + 8:(n + 1) * step]]
        if len(jobs) * step < w.shape[0]:
            parts.append(w[len(jobs) * step:])
        return _unpacked(jnp.concatenate(parts, axis=0))

    def load_weights(wqkv, wo_s, pre_s, stage, xq_v, nq_s, hq_s, wmod_v, moda_s, w_sems, m_sems,
                     o_sems):
        cf = c_ref[...].astype(_F32)
        silu_c = jnp.broadcast_to(cf * jax.nn.sigmoid(cf), (8, D))
        rows_c = _LANE * H
        words = stage.bitcast(_U32)
        w_hbm = (wq_hbm, wk_hbm, wv_hbm)

        def w_copy(t, j):
            return copy(w_hbm[t].at[_aligned(j * rows_c, rows_c), :],
                        stage.at[_aligned(j * rows_c, rows_c), :], w_sems.at[j])

        def m_copy(r, j):
            n = r * ND + j
            return copy(wmod_hbm.at[:, _aligned(n * _LANE, _LANE)], wmod_v.at[n], m_sems.at[n])

        def modulate(j):
            shift = _dot(silu_c, wmod_v[j])
            gain = 1.0 + _dot(silu_c, wmod_v[ND + j])
            moda_s[0, j] = shift
            moda_s[1, j] = gain
            hq_s[j] = _pack(nq_s[j] * gain[0:1] + shift[0:1])

        def absorb(t, j, n, a, after_first=None):
            size = n * rows_c // 2
            src = words.at[_aligned(j * size, size), :]
            dst = wqkv.at[pl.ds(t * H, H), _aligned(j * n * (_LANE // 2), n * (_LANE // 2)), :]
            acc = pre_s.at[pl.ds(t * H, H)]
            for h in range(0, H, _G):
                tiles = []
                for hp in range(h // 2, (h + _G) // 2):
                    w = src[pl.ds(hp, n * _LANE, stride=H // 2), :]
                    tiles += [_low_half(w).astype(_BF16), _high_half(w).astype(_BF16)]
                for i in range(_G):
                    dst[h + i] = pltpu.bitcast(tiles[i], _U32)
                if h == 0 and after_first is not None:
                    after_first()
                y = _dot(a, jnp.concatenate(tiles, axis=1))
                for i in range(_G):
                    acc[h + i] = y[:, _cols(i)] + jnp.where(j == 0, 0.0, acc[h + i])

        cp_xq = copy(x_hbm.at[:, pl.ds(seg_len - _PRE, _PRE), :], xq_v, o_sems.at[ND])
        cp_x = copy(x_hbm, x_v, o_sems.at[ND + 1])
        cp_wo = [copy(wo_hbm.at[:, pl.ds(n * _LANE, _LANE)], wo_s.at[n], o_sems.at[n])
                 for n in range(ND)]
        cp_mb = [m_copy(r, j) for r in range(2, 6) for j in range(ND)]

        mu = [[m_copy(0, j), m_copy(1, j)] for j in range(ND)]
        qu, ku, vu = ([[w_copy(t, j)] for j in range(ND)] for t in range(3))
        q_plan = [mu[3] + qu[2], mu[4] + qu[3] + mu[5], qu[4] + mu[6] + qu[5],
                  mu[7] + qu[6] + qu[7], ku[0] + ku[1], ku[2] + ku[3], ku[4] + ku[5], cp_wo[:2]]
        kv_plan = [ku[6] + ku[7] + cp_wo[2:4], vu[0] + vu[1] + cp_wo[4:6],
                   vu[2] + vu[3] + cp_wo[6:], vu[4] + vu[5] + cp_mb[:ND],
                   vu[6] + vu[7] + [cp_x], cp_mb[ND:3 * ND], cp_mb[3 * ND:]]

        def issue(j, plan):
            for i, cps in enumerate(plan):
                pl.when(j == i)(functools.partial(_start, cps))

        with jax.named_scope('sc_first'):
            _start([cp_xq] + mu[0] + qu[0])
            cp_xq.wait()
            _start(mu[1] + mu[2] + qu[1])
            nq = _layernorm(xq_v[...].astype(_F32).reshape(n_seg * _PRE, D))
            for j in range(ND):
                nq_s[j] = nq[:, _cols(j)]
            _wait(mu[0])
            modulate(0)

        def q_step(j):
            issue(j, q_plan)
            nxt = jnp.minimum(j + 1, ND - 1)
            pl.when(j + 1 < ND)(functools.partial(_wait, [m_copy(0, nxt), m_copy(1, nxt)]))
            w_copy(0, j).wait()
            absorb(0, j, 1, _unpacked(hq_s[j]), functools.partial(modulate, nxt))
        with jax.named_scope('sc_q'):
            _loop(0, ND, q_step)

        def kv_step(i):
            issue(i, kv_plan)
            t, j = 1 + i // (ND // 2), i % (ND // 2)
            for tt in (1, 2):
                pl.when(t == tt)(functools.partial(_wait, [w_copy(tt, 2 * j), w_copy(tt, 2 * j + 1)]))
            absorb(t, j, 2, jnp.concatenate([_unpacked(hq_s[2 * j + u]) for u in range(2)], axis=1))
        with jax.named_scope('sc_kv'):
            _loop(0, ND, kv_step)

        with jax.named_scope('sc_wo'):
            _wait(cp_wo + [cp_x] + cp_mb)
            for r in range(2):
                mod_s[r] = jnp.concatenate([moda_s[r, j] for j in range(ND)], axis=1)
            for r in range(2, 6):
                w = jnp.concatenate([wmod_v[r * ND + j] for j in range(ND)], axis=1)
                y = _dot(silu_c, w)
                mod_s[r] = 1.0 + y if r == 4 else y

    def residual(x, a):
        return x.astype(_F32) + mod(2) * a

    def recurrence(wqkv, wo_s, pre_s, hb_s, n0_s, mem_s, seg_s, o_s, prev_s):
        def seg_input(s, buf, r):
            h = _layernorm(x_v[s, r:r + 8, :].astype(_F32)) * mod(1) + mod(0)
            seg_s[buf, r:r + 8, :] = h
            return [h]

        def mixer_input(s, r):
            hb = _layernorm(residual(x_v[s, r:r + 16, :], prev_s[r:r + 16, :])) * mod(4) + mod(3)
            hb_s[_aligned(s * seg_len + r, 16), :] = hb
            n0 = _pack(_layernorm(hb))
            n0_s[_aligned((s * seg_len + r) // 2, 8), :] = n0
            return [n0]

        def seg_jobs(s, buf):
            return [functools.partial(seg_input, s, buf, r) for r in range(0, seg_len - _PRE, 8)]

        def mixer_jobs(s):
            return [functools.partial(mixer_input, s, r) for r in range(0, seg_len, 16)]

        mem_s[...] = mem0_ref[...].astype(_F32)
        for job in seg_jobs(0, 0):
            job()
        prev_s[...] = jnp.zeros(prev_s.shape, _F32)

        row = lax.broadcasted_iota(jnp.int32, (L, L), 0)
        col = lax.broadcasted_iota(jnp.int32, (L, L), 1)
        mask = (row < M) | (row >= col)
        half = D // 2

        def seg_step(s, buf, mem):
            jobs = mixer_jobs(jnp.maximum(s - 1, 0)) + seg_jobs(jnp.minimum(s + 1, n_seg - 1), buf)
            lhs = [jnp.concatenate([mem[i], seg_s[buf, :, _cols(i, half)]], axis=0).astype(_BF16)
                   for i in range(2)]
            pre = pre_s.at[:, _aligned(s * _PRE, _PRE), :]

            def proj_part(first, parts):
                rows = slice(parts[0] * half // 2, (parts[-1] + 1) * half // 2)
                due = [jobs.pop(0)] if jobs and first > 2 * H else []
                w = jnp.concatenate([paced(wqkv[first + i, rows, :], due if i == 0 else [])
                                     for i in range(_G)], axis=1)
                return _dot(jnp.concatenate([lhs[i] for i in parts], axis=1), w)

            def heads(first, y):
                return [jnp.concatenate([y[:, _cols(i)], pre[first + i]], axis=0)
                        for i in range(_G)]

            def proj(first):
                return heads(first, proj_part(first, (0, 1)))

            def weights(q, k):
                sc = jnp.where(mask, _dot_nt(q, k.astype(_BF16)) * scale, -1000000000.0)
                e = jnp.exp(sc - jnp.max(sc, axis=-1, keepdims=True))
                return e, jnp.sum(e, axis=-1, keepdims=True)

            def mix(h0, ws, vs):
                for i, ((e, den), v) in enumerate(zip(ws, vs)):
                    o_s[:, _cols(h0 + i)] = _dot(e, v.astype(_BF16)) / den

            def out_proj(h0, h1, part):
                ks = slice(h0 * _LANE, h1 * _LANE)
                cols = range(part * ND // 2, (part + 1) * ND // 2)
                return _dot(o_s[:, ks], jnp.concatenate([wo_s[n, ks, :] for n in cols], axis=1))

            pend = None
            for h in range(0, H, _G):
                if pend is None:
                    q0, k0 = proj_part(h, (0,)), proj_part(H + h, (0,))
                    qs = heads(h, proj_part(h, (1,)) + q0)
                    ks = heads(H + h, proj_part(H + h, (1,)) + k0)
                else:
                    qs, ks = proj(h), proj(H + h)
                    mix(*pend)
                vs = proj(2 * H + h)
                pend = (h, [weights(q, k) for q, k in zip(qs, ks)], vs)
            y0 = out_proj(0, H - _G, 0)
            mix(*pend)
            y1 = out_proj(0, 2 * _G, 1)
            y0 = out_proj(H - _G, H, 0) + y0
            y1 = out_proj(2 * _G, H, 1) + y1
            assert not jobs
            for i, y in enumerate((y0, y1)):
                a_s[_aligned(s * seg_len, seg_len), _cols(i, half)] = y[M:L]
                prev_s[:, _cols(i, half)] = y[M:L]
            return y0[0:M], y1[0:M]

        def seg_steps(i):
            mem = (mem_s[:, 0:half], mem_s[:, half:D])
            for u in range(_UNROLL):
                mem = seg_step(i * _UNROLL + u, 0, mem)
            mem_s[:, 0:half] = mem[0]
            mem_s[:, half:D] = mem[1]

        with jax.named_scope('sc_attn'):
            _loop(0, n_seg // _UNROLL, seg_steps)
        for job in mixer_jobs(n_seg - 1):
            job()

    def mixer(w1_v, w2_v, w3_v, w4_v, hb_s, n0_s, t3_s, t4_s, a1_s, a2_s, n1_s, last_s, out_s, out_sems,
              *g_s):
        n_blk = S // _TM
        shifts = [(-1, 1, -2, 2)[j * _LANE * 4 // D] for j in range(ND)]
        last_s[1] = jnp.zeros(last_s.shape[1:], _F32)
        for g in g_s:
            g[_HALO:2 * _HALO, :] = jnp.zeros((_HALO, _LANE), _F32)
            g[S:S + _HALO, :] = jnp.zeros((_HALO, _LANE), _F32)

        def block(ref, i, n=_TM):
            return ref.at[_aligned(i * n, n), :]

        def weight_terms(src, dst, i, r, col):
            nr, nc = src.shape[0] // P, src.shape[1] // P
            n = nr // n_blk
            dst = dst.at[:, pl.ds(pl.multiple_of(i * (n // 2), 8), n // 2), :]
            w = [[pltpu.bitcast(src[_aligned(a * nr + i * n + r, 16),
                                    b * nc + col:b * nc + col + _LANE], _U32)
                  for b in range(P)] for a in range(P)]
            lo = _rhs_terms([[_low_half(v) for v in row] for row in w])
            hi = _rhs_terms([[_high_half(v) for v in row] for row in w])
            out = [pltpu.pack_elementwise(list(pair), packed_dtype=_BF16) for pair in zip(lo, hi)]
            for t, v in enumerate(out):
                dst[t, r // 2:r // 2 + 8, col:col + _LANE] = v
            return out

        def weight_jobs(src, dst, i):
            return [functools.partial(weight_terms, src, dst, i, r, col)
                    for r in range(0, src.shape[0] // P // n_blk, 16)
                    for col in range(0, src.shape[1] // P, _LANE)]

        def spread(jobs):
            per = -(-len(jobs) // (ND - 1))
            return [[]] + [jobs[j * per:(j + 1) * per] for j in range(ND - 1)]

        def gate(i):
            n0 = _unpacked(block(n0_s, i, _TM // 2)[...])
            for j, (g, off, jobs) in enumerate(zip(g_s, shifts, spread(weight_jobs(w3_v, t3_s, i)))):
                win = g.at[pl.ds(pl.multiple_of(i * _TM, _TM), _TM + 2 * _HALO), :]
                w = paced(pltpu.bitcast(w1_v[:, _cols(j)], _U32), jobs)
                win[_HALO - off:_HALO - off + _TM, :] = _gelu(_dot(n0, w))

        th = _TM // 2

        def mlp_norm(k, buf, r):
            n1 = _layernorm(last_s[buf, r:r + 16, :])
            block(n1_s, k, th)[r:r + 16, :] = n1
            return [n1]

        def norm_jobs(k, buf):
            return [functools.partial(mlp_norm, k, buf, r) for r in range(0, th, 16)]

        def mix(i):
            jobs = weight_jobs(w4_v, t4_s, i)
            for u in range(2):
                x1 = block(hb_s, i).at[u * th:(u + 1) * th, :]
                rows = pl.ds(pl.multiple_of(i * _TM + u * th + _HALO, _HALO), th)
                shifted = jnp.concatenate([g[rows, :] for g in g_s], axis=1).astype(_BF16)
                due = zip(spread(norm_jobs(jnp.maximum(2 * i + u - 1, 0), 1 - u)),
                          spread(jobs[u::2]))
                for j, (norms, terms) in enumerate(due):
                    w = paced(pltpu.bitcast(w2_v[:, _cols(j)], _U32), norms + terms)
                    y = _dot(shifted, w) + x1[:, _cols(j)]
                    x1[:, _cols(j)] = y
                    last_s[u, :, _cols(j)] = y

        def mlp_terms(i, r, col):
            n1 = block(n1_s, i)
            g = [[n1[a * mq + r:a * mq + r + 16, b * dq + col:b * dq + col + _LANE]
                  for b in range(P)] for a in range(P)]
            out = [_pack(v) for v in _lhs_terms(g)]
            for t, v in enumerate(out):
                a1_s[t, r // 2:r // 2 + 8, col:col + _LANE] = v
            return out

        def term_jobs(i):
            return [functools.partial(mlp_terms, i, r, col)
                    for r in range(0, mq, 16) for col in range(0, dq, _LANE)]

        def products(a_ref, w_ref, jobs, every):
            count = [0]

            def product(p, t):
                count[0] += 1
                due = [jobs.pop(0)] if jobs and count[0] % every == 0 else []
                return _dot(_unpacked(a_ref[t]), paced(w_ref[t, :, _cols(p)], due))
            return product

        def out_copy(i, slot):
            return copy(out_s.at[slot], block(out_hbm, i), out_sems.at[slot])

        def mlp(i):
            slot = i % 2

            @pl.when(i >= 2)
            def _():
                out_copy(jnp.maximum(i - 2, 0), slot).wait()

            terms = term_jobs(jnp.minimum(i + 1, n_blk - 1))
            up, down = products(a1_s, t3_s, [], 1), products(a2_s, t4_s, terms, 10)
            for p in range(fq // _LANE):
                g = _combine(_LEVEL, functools.partial(up, p), emit=lambda a, b, y: _gelu(y))
                for t, v in enumerate(_lhs_terms(g)):
                    a2_s[t, :, _cols(p)] = _pack(v)

            dst, att, x1 = out_s.at[slot], block(a_s, i), block(hb_s, i)
            x = x_v.at[pl.ds(i * (_TM // seg_len), _TM // seg_len)]
            for p in range(dq // _LANE):
                def emit(a, b, y):
                    rows, cols = slice(a * mq, (a + 1) * mq), _cols(b * (dq // _LANE) + p)
                    xs = x[a * mq // seg_len:(a + 1) * mq // seg_len, :, cols]
                    res = (xs.astype(_F32).reshape(mq, _LANE) + mod(2, cols) * att[rows, cols]
                           + mod(5, cols) * (x1[rows, cols] + y))
                    dst[rows, cols] = res.astype(dst.dtype)

                _combine(_LEVEL, functools.partial(down, p), emit=emit)
            assert not terms
            out_copy(i, slot).start()

        with jax.named_scope('sc_s1'):
            _loop(0, n_blk, gate)
        with jax.named_scope('sc_s2'):
            _loop(0, n_blk, mix)
        for job in norm_jobs(2 * n_blk - 1, 1) + term_jobs(0):
            job()
        with jax.named_scope('sc_s3'):
            _loop(0, n_blk, mlp)
        for i in (n_blk - 2, n_blk - 1):
            out_copy(i, i % 2).wait()

    def after_weights(wqkv, wo_s, pre_s, w1_v, w2_v, w3_v, w4_v, hb_s, n0_s):
        cps = [copy(src, dst, sems.at[i]) for i, (src, dst) in enumerate(
            ((w1_hbm, w1_v), (w2_hbm, w2_v), (w3_hbm, w3_v), (w4_hbm, w4_v)))]
        _start(cps)
        pl.run_scoped(
            functools.partial(recurrence, wqkv, wo_s, pre_s, hb_s, n0_s),
            pltpu.VMEM((M, D), _F32),
            pltpu.VMEM((2, seg_len - _PRE, D), _F32),
            pltpu.VMEM((L, H * _LANE), _F32),
            pltpu.VMEM((seg_len, D), _F32),
        )
        _wait(cps)

    def whole(w1_v, w2_v, w3_v, w4_v, hb_s, n0_s):
        def attention(wqkv, wo_s, pre_s):
            pl.run_scoped(
                functools.partial(load_weights, wqkv, wo_s, pre_s),
                pltpu.VMEM((D * H, _LANE), _BF16),
                pltpu.VMEM((n_seg, _PRE, D), _BF16),
                pltpu.VMEM((ND, n_seg * _PRE, _LANE), _F32),
                pltpu.VMEM((ND, n_seg * _PRE // 2, _LANE), _U32),
                pltpu.VMEM((6 * ND, D, _LANE), _BF16),
                pltpu.VMEM((2, ND, 8, _LANE), _F32),
                pltpu.SemaphoreType.DMA((ND,)),
                pltpu.SemaphoreType.DMA((6 * ND,)),
                pltpu.SemaphoreType.DMA((ND + 2,)),
            )
            after_weights(wqkv, wo_s, pre_s, w1_v, w2_v, w3_v, w4_v, hb_s, n0_s)

        pl.run_scoped(
            attention,
            pltpu.VMEM((3 * H, D // 2, _LANE), _U32),
            pltpu.VMEM((ND, H * _LANE, _LANE), _BF16),
            pltpu.VMEM((3 * H, n_seg * _PRE, _LANE), _F32),
        )
        pl.run_scoped(
            functools.partial(mixer, w1_v, w2_v, w3_v, w4_v, hb_s, n0_s),
            pltpu.VMEM((T, dq // 2, fq), _U32),
            pltpu.VMEM((T, fq // 2, dq), _U32),
            pltpu.VMEM((T, mq // 2, dq), _U32),
            pltpu.VMEM((T, mq // 2, fq), _U32),
            pltpu.VMEM((S, D), _F32),
            pltpu.VMEM((2, _TM // 2, D), _F32),
            pltpu.VMEM((2, _TM, D), _BF16),
            pltpu.SemaphoreType.DMA((2,)),
            *[pltpu.VMEM((S + 2 * _HALO, _LANE), _F32) for _ in range(ND)],
        )

    pl.run_scoped(
        whole,
        pltpu.VMEM((D, D), _BF16),
        pltpu.VMEM((D, D), _BF16),
        pltpu.VMEM((D, F), _BF16),
        pltpu.VMEM((F, D), _BF16),
        pltpu.VMEM((S, D), _F32),
        pltpu.VMEM((S // 2, D), _U32),
    )


@functools.partial(jax.jit, static_argnames=("A_seg_len",))
def pallas_adaLN_cond__memory_aug_recurrent_mem_tr__mixer_s_mlp__prompt_kernel(
    A_x: jax.Array,
    A_mem0: jax.Array,
    A_Wq: jax.Array,
    A_Wk: jax.Array,
    A_Wv: jax.Array,
    A_Wo: jax.Array,
    A_seg_len: int,
    B_x: jax.Array,
    B_w1: jax.Array,
    B_w2: jax.Array,
    B_w3: jax.Array,
    B_w4: jax.Array,
    c: jax.Array,
    w_mod: jax.Array,
):
    del B_x
    batch, S, D = A_x.shape
    _, H, Dh = A_Wq.shape
    M = A_mem0.shape[1]
    seg_len = int(A_seg_len)
    assert batch == 1 and Dh == _LANE and S % _TM == 0 and _TM % seg_len == 0
    n_seg = S // seg_len

    vmem = pl.BlockSpec(memory_space=pltpu.VMEM)
    hbm = pl.BlockSpec(memory_space=pl.ANY)
    out = pl.pallas_call(
        _kernel,
        out_shape=jax.ShapeDtypeStruct((S, D), A_x.dtype),
        in_specs=[vmem, vmem] + [hbm] * 10,
        out_specs=hbm,
        scratch_shapes=[
            pltpu.VMEM((n_seg, seg_len, D), _BF16),
            pltpu.VMEM((S, D), _F32),
            pltpu.VMEM((6, 8, D), _F32),
            pltpu.VMEM((8, _LANE), _U32),
            pltpu.SemaphoreType.DMA((4,)),
        ],
        compiler_params=pltpu.CompilerParams(vmem_limit_bytes=126 * 1024 * 1024),
        name="adaln_rmt_mixer",
    )(
        A_mem0.reshape(M, D), c, A_x.reshape(n_seg, seg_len, D),
        A_Wq.reshape(D * H, Dh), A_Wk.reshape(D * H, Dh), A_Wv.reshape(D * H, Dh),
        A_Wo.reshape(H * Dh, D), B_w1, B_w2, B_w3, B_w4, w_mod,
    )
    return out.reshape(batch, S, D)
```

```python
import functools
import math

import jax
import jax.numpy as jnp
from jax import lax
import jax.experimental.pallas as pl
import jax.experimental.pallas.tpu as pltpu

_F32 = jnp.float32
_BF16 = jnp.bfloat16
_U32 = jnp.uint32
_LANE = 128
_EPS = 1e-05
_TM = 256
_LEVEL = 2
_UNROLL = 2
_HALO = 8
_PRE = 8
_G = 4


def _dot(a, b):
    return lax.dot_general(a, b, (((1,), (0,)), ((), ())), preferred_element_type=_F32)


def _dot_nt(a, b):
    return lax.dot_general(a, b, (((1,), (1,)), ((), ())), preferred_element_type=_F32)


def _layernorm(x):
    m = jnp.mean(x, axis=-1, keepdims=True)
    d = x - m
    v = jnp.mean(d * d, axis=-1, keepdims=True)
    return d * lax.rsqrt(v + _EPS)


def _gelu(x):
    c = math.sqrt(2.0 / math.pi)
    inner = x * (c + (c * 0.044715) * (x * x))
    hx = 0.5 * x
    return hx + hx * jnp.tanh(inner)


def _pack(x):
    return pltpu.bitcast(x.astype(_BF16), _U32)


def _unpacked(x):
    return pltpu.bitcast(x, _BF16)


def _low_half(w):
    return pltpu.bitcast(w << 16, _F32)


def _high_half(w):
    return pltpu.bitcast(w & jnp.uint32(0xFFFF0000), _F32)


def _quads(g):
    n = len(g) // 2
    return [[row[j * n:(j + 1) * n] for row in g[i * n:(i + 1) * n]]
            for i in range(2) for j in range(2)]


def _add(a, b):
    return [[x + y for x, y in zip(r, t)] for r, t in zip(a, b)]


def _sub(a, b):
    return [[x - y for x, y in zip(r, t)] for r, t in zip(a, b)]


def _lhs_terms(g):
    if len(g) == 1:
        return [g[0][0]]
    a11, a12, a21, a22 = _quads(g)
    terms = (_sub(a11, a22), _sub(a21, a22), a22, _sub(a21, a11), _sub(a22, a12), a11,
             _sub(a11, a12))
    return [v for t in terms for v in _lhs_terms(t)]


def _rhs_terms(g):
    if len(g) == 1:
        return [g[0][0]]
    b11, b12, b21, b22 = _quads(g)
    terms = (_sub(b11, b22), b11, _add(b21, b11), _add(b11, b12), _add(b21, b22), _add(b12, b22),
             b22)
    return [v for t in terms for v in _rhs_terms(t)]


def _combine(level, product, base=0, emit=None):
    if level == 0:
        return [[product(base)]]

    def m(i):
        return _combine(level - 1, product, base + i * 7 ** (level - 1))

    def done(qi, qj, g):
        if emit is None:
            return g
        n = len(g)
        return [[emit(qi * n + a, qj * n + b, g[a][b]) for b in range(n)] for a in range(n)]

    m0, m1 = m(0), m(1)
    c22 = _sub(m0, m1)
    m2 = m(2)
    c11 = _add(m0, m2)
    c21 = done(1, 0, _add(m1, m2))
    m5 = m(5)
    c22 = _add(c22, m5)
    m6 = m(6)
    c11 = _add(c11, m6)
    c12 = done(0, 1, _sub(m5, m6))
    c22 = done(1, 1, _add(m(3), c22))
    c11 = done(0, 0, _sub(c11, m(4)))
    return [x + y for x, y in zip(c11, c12)] + [x + y for x, y in zip(c21, c22)]


def _aligned(start, size):
    return pl.ds(pl.multiple_of(start, size), size)


def _cols(j, n=_LANE):
    return slice(j * n, (j + 1) * n)


def _loop(lo, hi, fn):
    def body(i, carry):
        fn(i)
        return carry
    lax.fori_loop(lo, hi, body, 0)


def _start(cps):
    for cp in cps:
        cp.start()


def _wait(cps):
    for cp in cps:
        cp.wait()


def _kernel(mem0_ref, c_ref, x_hbm, wq_hbm, wk_hbm, wv_hbm, wo_hbm, w1_hbm, w2_hbm, w3_hbm,
            w4_hbm, wmod_hbm, out_hbm, x_v, a_s, mod_s, zero_s, sems):
    n_seg, seg_len, D = x_v.shape
    S = n_seg * seg_len
    M = mem0_ref.shape[0]
    H = wo_hbm.shape[0] // _LANE
    F = w3_hbm.shape[1]
    L = M + seg_len
    ND = D // _LANE
    P = 2 ** _LEVEL
    T = 7 ** _LEVEL
    mq, dq, fq = _TM // P, D // P, F // P
    scale = float(_LANE) ** -0.5
    copy = pltpu.make_async_copy

    def mod(r, cols=slice(None)):
        return mod_s[r, 0:1, cols]

    cf = c_ref[...].astype(_F32)
    silu_c = jnp.broadcast_to(cf * jax.nn.sigmoid(cf), (8, D))
    x_head = 8
    cp_x_tail = copy(x_hbm.at[pl.ds(x_head, n_seg - x_head)],
                     x_v.at[pl.ds(x_head, n_seg - x_head)], sems.at[4])
    zero_s[...] = jnp.zeros(zero_s.shape, _U32)

    def paced(w, jobs):
        step = w.shape[0] // (_LANE // 2) // max(len(jobs), 1) * (_LANE // 2)
        parts = []
        for n, job in enumerate(jobs):
            tiles = [pltpu.bitcast(v, _U32)[r:r + 8, c:c + _LANE] for v in job()
                     for r in range(0, v.shape[0], 8) for c in range(0, v.shape[1], _LANE)]
            done = functools.reduce(jnp.bitwise_or, tiles) & zero_s[...]
            parts += [w[n * step:n * step + 8] | done, w[n * step + 8:(n + 1) * step]]
        if len(jobs) * step < w.shape[0]:
            parts.append(w[len(jobs) * step:])
        return _unpacked(jnp.concatenate(parts, axis=0))

    def load_weights(wqkv, wo_s, pre_s, stage, xq_v, nq_s, hq_s, wmod_v, moda_s, w_sems, m_sems,
                     o_sems):
        rows_c = _LANE * H
        words = stage.bitcast(_U32)
        w_hbm = (wq_hbm, wk_hbm, wv_hbm)

        def w_copy(t, j):
            return copy(w_hbm[t].at[_aligned(j * rows_c, rows_c), :],
                        stage.at[_aligned(j * rows_c, rows_c), :], w_sems.at[j])

        def m_copy(r, j):
            n = r * ND + j
            return copy(wmod_hbm.at[:, _aligned(n * _LANE, _LANE)], wmod_v.at[n], m_sems.at[n])

        def modulate(j):
            hs = []
            for u in (2 * j, 2 * j + 1):
                shift = _dot(silu_c, wmod_v[u])
                gain = 1.0 + _dot(silu_c, wmod_v[ND + u])
                moda_s[0, u] = shift
                moda_s[1, u] = gain
                hs.append(nq_s[u] * gain[0:1] + shift[0:1])
            mh = hs[0].shape[0] // 2
            for n, v in enumerate(_lhs_terms([[h[_cols(a, mh)] for h in hs] for a in range(2)])):
                hq_s[j, n] = _pack(v)

        def absorb(t, j):
            src = words.at[_aligned(j * rows_c, rows_c), :]
            dst = wqkv.at[pl.ds(t * H, H), _aligned(j * _LANE, _LANE), :]
            acc = pre_s.at[pl.ds(t * H, H)]
            lhs = hq_s.at[j]
            mh = lhs.shape[1] * 2
            for hp in range(H // 2):
                w = src[pl.ds(hp, 2 * _LANE, stride=H // 2), :]
                pair = (_low_half(w), _high_half(w))
                for i in range(2):
                    dst[2 * hp + i] = _pack(pair[i])
                rhs = _rhs_terms([[v[_cols(u)] for v in pair] for u in range(2)])

                def emit(a, b, y):
                    old = acc[2 * hp + b, _cols(a, mh), :]
                    acc[2 * hp + b, _cols(a, mh), :] = y + jnp.where(j == 0, 0.0, old)

                _combine(1, lambda n: _dot(_unpacked(lhs[n]), rhs[n].astype(_BF16)), emit=emit)

        cp_xq = copy(x_hbm.at[:, pl.ds(seg_len - _PRE, _PRE), :], xq_v, o_sems.at[ND])
        cp_x_head = copy(x_hbm.at[pl.ds(0, x_head)], x_v.at[pl.ds(0, x_head)], o_sems.at[ND + 1])
        cp_wo = [copy(wo_hbm.at[:, pl.ds(n * _LANE, _LANE)], wo_s.at[n], o_sems.at[n])
                 for n in range(ND)]
        cp_mb = [m_copy(r, j) for r in range(2, 5) for j in range(ND)]

        mu = [[m_copy(0, j), m_copy(1, j)] for j in range(ND)]
        qu, ku, vu = ([[w_copy(t, j)] for j in range(ND)] for t in range(3))
        m2, q2, k2, v2 = ([u[2 * j] + u[2 * j + 1] for j in range(ND // 2)] for u in (mu, qu, ku, vu))
        plan = [q2[1] + m2[2] + cp_wo[0:1], q2[2] + m2[3] + cp_wo[1:2], q2[3] + k2[0],
                k2[1] + k2[2], k2[3] + cp_wo[2:4], v2[0] + cp_wo[4:6], v2[1] + cp_wo[6:],
                v2[2] + cp_mb[:ND], v2[3] + cp_mb[ND:2 * ND], cp_mb[2 * ND:] + [cp_x_head]]

        with jax.named_scope('sc_first'):
            _start([cp_xq] + m2[0] + q2[0])
            cp_xq.wait()
            _start(m2[1])
            nq = _layernorm(xq_v[...].astype(_F32).reshape(n_seg * _PRE, D))
            for j in range(ND):
                nq_s[j] = nq[:, _cols(j)]

        def step(i):
            t, j = i // (ND // 2), i % (ND // 2)

            @pl.when(t == 0)
            def _():
                _wait([m_copy(r, 2 * j + u) for r in range(2) for u in range(2)])
                modulate(j)

            for tt in range(3):
                pl.when(t == tt)(functools.partial(_wait, [w_copy(tt, 2 * j), w_copy(tt, 2 * j + 1)]))
            for n, cps in enumerate(plan):
                pl.when(i == n)(functools.partial(_start, cps))
            absorb(t, j)
        with jax.named_scope('sc_kv'):
            _loop(0, 3 * ND // 2, step)

        with jax.named_scope('sc_wo'):
            _wait(cp_wo + [cp_x_head] + cp_mb)
            for r in range(2):
                mod_s[r] = jnp.concatenate([moda_s[r, j] for j in range(ND)], axis=1)
            for r in range(2, 5):
                w = jnp.concatenate([wmod_v[r * ND + j] for j in range(ND)], axis=1)
                y = _dot(silu_c, w)
                mod_s[r] = 1.0 + y if r == 4 else y

    def residual(x, a):
        return x.astype(_F32) + mod(2) * a

    def recurrence(wqkv, wo_s, pre_s, hb_s, n0_s, mem_s, seg_s, o_s, prev_s):
        def seg_input(s, buf, r):
            h = _layernorm(x_v[s, r:r + 8, :].astype(_F32)) * mod(1) + mod(0)
            seg_s[buf, r:r + 8, :] = h
            return [h]

        def mixer_input(s, r):
            hb = _layernorm(residual(x_v[s, r:r + 16, :], prev_s[r:r + 16, :])) * mod(4) + mod(3)
            hb_s[_aligned(s * seg_len + r, 16), :] = hb
            n0 = _pack(_layernorm(hb))
            n0_s[_aligned((s * seg_len + r) // 2, 8), :] = n0
            return [n0]

        def seg_jobs(s, buf):
            return [functools.partial(seg_input, s, buf, r) for r in range(0, seg_len - _PRE, 8)]

        def mixer_jobs(s):
            return [functools.partial(mixer_input, s, r) for r in range(0, seg_len, 16)]

        mem_s[...] = mem0_ref[...].astype(_F32)
        for job in seg_jobs(0, 0):
            job()
        prev_s[...] = jnp.zeros(prev_s.shape, _F32)

        row = lax.broadcasted_iota(jnp.int32, (L, L), 0)
        col = lax.broadcasted_iota(jnp.int32, (L, L), 1)
        mask = (row < M) | (row >= col)
        half = D // 2

        def seg_step(s, buf, mem):
            jobs = mixer_jobs(jnp.maximum(s - 1, 0)) + seg_jobs(jnp.minimum(s + 1, n_seg - 1), buf)
            lhs = [jnp.concatenate([mem[i], seg_s[buf, :, _cols(i, half)]], axis=0).astype(_BF16)
                   for i in range(2)]
            pre = pre_s.at[:, _aligned(s * _PRE, _PRE), :]

            def proj_part(ids, parts):
                rows = slice(parts[0] * half // 2, (parts[-1] + 1) * half // 2)
                due = {ids[-1]: [jobs.pop(0)]} if jobs and ids[-1] >= 2 * H + _G else {}
                w = jnp.concatenate([paced(wqkv[n, rows, :], due.get(n, [])) for n in ids], axis=1)
                return _dot(jnp.concatenate([lhs[i] for i in parts], axis=1), w)

            def proj(ids, y=None):
                y = proj_part(ids, (0, 1)) if y is None else proj_part(ids, (1,)) + y
                return [jnp.concatenate([y[:, _cols(i)], pre[n]], axis=0) for i, n in enumerate(ids)]

            def weights(q, k):
                sc = jnp.where(mask, _dot_nt(q, k.astype(_BF16)) * scale, -1000000000.0)
                e = jnp.exp(sc - jnp.max(sc, axis=-1, keepdims=True))
                return e, jnp.sum(e, axis=-1, keepdims=True)

            def mix(h0, ws, vs):
                for i, ((e, den), v) in enumerate(zip(ws, vs)):
                    o_s[:, _cols(h0 + i)] = _dot(e, v.astype(_BF16)) / den

            def out_proj(h0, h1, part):
                ks = slice(h0 * _LANE, h1 * _LANE)
                cols = range(part * ND // 2, (part + 1) * ND // 2)
                return _dot(o_s[:, ks], jnp.concatenate([wo_s[n, ks, :] for n in cols], axis=1))

            pend = None
            for h in range(0, H, _G):
                ids = [t * H + h + i for t in range(3) for i in range(_G)]
                if pend is None:
                    qkv = proj(ids[:2 * _G], proj_part(ids[:2 * _G], (0,))) + proj(ids[2 * _G:])
                else:
                    qkv = proj(ids)
                    mix(*pend)
                pend = (h, [weights(q, k) for q, k in zip(qkv[:_G], qkv[_G:2 * _G])], qkv[2 * _G:])
            y0 = out_proj(0, H - _G, 0)
            mix(*pend)
            y1 = out_proj(0, 2 * _G, 1)
            y0 = out_proj(H - _G, H, 0) + y0
            y1 = out_proj(2 * _G, H, 1) + y1
            assert not jobs
            for i, y in enumerate((y0, y1)):
                a_s[_aligned(s * seg_len, seg_len), _cols(i, half)] = y[M:L]
                prev_s[:, _cols(i, half)] = y[M:L]
            return y0[0:M], y1[0:M]

        def seg_steps(i):
            pl.when(i == x_head // _UNROLL - 1)(cp_x_tail.wait)
            mem = (mem_s[:, 0:half], mem_s[:, half:D])
            for u in range(_UNROLL):
                mem = seg_step(i * _UNROLL + u, 0, mem)
            mem_s[:, 0:half] = mem[0]
            mem_s[:, half:D] = mem[1]

        with jax.named_scope('sc_attn'):
            _loop(0, n_seg // _UNROLL, seg_steps)
        for job in mixer_jobs(n_seg - 1):
            job()

    def mixer(w1_v, w2_v, w3_v, w4_v, hb_s, n0_s, t3_s, t4_s, a1_s, a2_s, n1_s, last_s, wg_v, out_s, out_sems,
              *g_s):
        n_blk = S // _TM
        shifts = [(-1, 1, -2, 2)[j * _LANE * 4 // D] for j in range(ND)]
        cp_gate = copy(wmod_hbm.at[:, pl.ds(5 * D, D)], wg_v, sems.at[5])
        cp_gate.start()
        last_s[1] = jnp.zeros(last_s.shape[1:], _F32)
        for g in g_s:
            g[_HALO:2 * _HALO, :] = jnp.zeros((_HALO, _LANE), _F32)
            g[S:S + _HALO, :] = jnp.zeros((_HALO, _LANE), _F32)

        def block(ref, i, n=_TM):
            return ref.at[_aligned(i * n, n), :]

        def weight_terms(src, dst, i, r, col):
            nr, nc = src.shape[0] // P, src.shape[1] // P
            n = nr // n_blk
            dst = dst.at[:, pl.ds(pl.multiple_of(i * (n // 2), 8), n // 2), :]
            w = [[pltpu.bitcast(src[_aligned(a * nr + i * n + r, 16),
                                    b * nc + col:b * nc + col + _LANE], _U32)
                  for b in range(P)] for a in range(P)]
            lo = _rhs_terms([[_low_half(v) for v in row] for row in w])
            hi = _rhs_terms([[_high_half(v) for v in row] for row in w])
            out = [pltpu.pack_elementwise(list(pair), packed_dtype=_BF16) for pair in zip(lo, hi)]
            for t, v in enumerate(out):
                dst[t, r // 2:r // 2 + 8, col:col + _LANE] = v
            return out

        def weight_jobs(src, dst, i):
            return [functools.partial(weight_terms, src, dst, i, r, col)
                    for r in range(0, src.shape[0] // P // n_blk, 16)
                    for col in range(0, src.shape[1] // P, _LANE)]

        def spread(jobs):
            per = -(-len(jobs) // (ND - 1))
            return [[]] + [jobs[j * per:(j + 1) * per] for j in range(ND - 1)]

        def gate(i):
            n0 = _unpacked(block(n0_s, i, _TM // 2)[...])
            for j, (g, off, jobs) in enumerate(zip(g_s, shifts, spread(weight_jobs(w3_v, t3_s, i)))):
                win = g.at[pl.ds(pl.multiple_of(i * _TM, _TM), _TM + 2 * _HALO), :]
                w = paced(pltpu.bitcast(w1_v[:, _cols(j)], _U32), jobs)
                win[_HALO - off:_HALO - off + _TM, :] = _gelu(_dot(n0, w))

        th = _TM // 2

        def mlp_norm(k, buf, r):
            n1 = _layernorm(last_s[buf, r:r + 16, :])
            block(n1_s, k, th)[r:r + 16, :] = n1
            return [n1]

        def norm_jobs(k, buf):
            return [functools.partial(mlp_norm, k, buf, r) for r in range(0, th, 16)]

        def mix(i):
            jobs = weight_jobs(w4_v, t4_s, i)
            for u in range(2):
                x1 = block(hb_s, i).at[u * th:(u + 1) * th, :]
                rows = pl.ds(pl.multiple_of(i * _TM + u * th + _HALO, _HALO), th)
                shifted = jnp.concatenate([g[rows, :] for g in g_s], axis=1).astype(_BF16)
                due = zip(spread(norm_jobs(jnp.maximum(2 * i + u - 1, 0), 1 - u)),
                          spread(jobs[u::2]))
                for j, (norms, terms) in enumerate(due):
                    w = paced(pltpu.bitcast(w2_v[:, _cols(j)], _U32), norms + terms)
                    y = _dot(shifted, w) + x1[:, _cols(j)]
                    x1[:, _cols(j)] = y
                    last_s[u, :, _cols(j)] = y

        def mlp_terms(i, r, col):
            n1 = block(n1_s, i)
            g = [[n1[a * mq + r:a * mq + r + 16, b * dq + col:b * dq + col + _LANE]
                  for b in range(P)] for a in range(P)]
            out = [_pack(v) for v in _lhs_terms(g)]
            for t, v in enumerate(out):
                a1_s[t, r // 2:r // 2 + 8, col:col + _LANE] = v
            return out

        def term_jobs(i):
            return [functools.partial(mlp_terms, i, r, col)
                    for r in range(0, mq, 16) for col in range(0, dq, _LANE)]

        def products(a_ref, w_ref, jobs, every):
            count = [0]

            def product(p, t):
                count[0] += 1
                due = [jobs.pop(0)] if jobs and count[0] % every == 0 else []
                return _dot(_unpacked(a_ref[t]), paced(w_ref[t, :, _cols(p)], due))
            return product

        def out_copy(i, slot):
            return copy(out_s.at[slot], block(out_hbm, i), out_sems.at[slot])

        def mlp(i):
            slot = i % 2

            @pl.when(i >= 2)
            def _():
                out_copy(jnp.maximum(i - 2, 0), slot).wait()

            terms = term_jobs(jnp.minimum(i + 1, n_blk - 1))
            up, down = products(a1_s, t3_s, [], 1), products(a2_s, t4_s, terms, 10)
            for p in range(fq // _LANE):
                g = _combine(_LEVEL, functools.partial(up, p), emit=lambda a, b, y: _gelu(y))
                for t, v in enumerate(_lhs_terms(g)):
                    a2_s[t, :, _cols(p)] = _pack(v)

            dst, att, x1 = out_s.at[slot], block(a_s, i), block(hb_s, i)
            x = x_v.at[pl.ds(i * (_TM // seg_len), _TM // seg_len)]
            for p in range(dq // _LANE):
                def emit(a, b, y):
                    rows, cols = slice(a * mq, (a + 1) * mq), _cols(b * (dq // _LANE) + p)
                    xs = x[a * mq // seg_len:(a + 1) * mq // seg_len, :, cols]
                    res = (xs.astype(_F32).reshape(mq, _LANE) + mod(2, cols) * att[rows, cols]
                           + mod(5, cols) * (x1[rows, cols] + y))
                    dst[rows, cols] = res.astype(dst.dtype)

                _combine(_LEVEL, functools.partial(down, p), emit=emit)
            assert not terms
            out_copy(i, slot).start()

        with jax.named_scope('sc_s1'):
            _loop(0, n_blk, gate)
        with jax.named_scope('sc_s2'):
            _loop(0, n_blk, mix)
        cp_gate.wait()
        mod_s[5] = jnp.concatenate(
            [_dot(silu_c, paced(pltpu.bitcast(wg_v[:, _cols(j)], _U32), list(jobs)))
             for j, jobs in enumerate(zip(norm_jobs(2 * n_blk - 1, 1), term_jobs(0), strict=True))],
            axis=1)
        with jax.named_scope('sc_s3'):
            _loop(0, n_blk, mlp)
        for i in (n_blk - 2, n_blk - 1):
            out_copy(i, i % 2).wait()

    def after_weights(wqkv, wo_s, pre_s, w1_v, w2_v, w3_v, w4_v, hb_s, n0_s):
        cps = [copy(src, dst, sems.at[i]) for i, (src, dst) in enumerate(
            ((w1_hbm, w1_v), (w2_hbm, w2_v), (w3_hbm, w3_v), (w4_hbm, w4_v)))]
        _start([cp_x_tail] + cps)
        pl.run_scoped(
            functools.partial(recurrence, wqkv, wo_s, pre_s, hb_s, n0_s),
            pltpu.VMEM((M, D), _F32),
            pltpu.VMEM((2, seg_len - _PRE, D), _F32),
            pltpu.VMEM((L, H * _LANE), _F32),
            pltpu.VMEM((seg_len, D), _F32),
        )
        _wait(cps)

    def whole(w1_v, w2_v, w3_v, w4_v, hb_s, n0_s):
        def attention(wqkv, wo_s, pre_s):
            pl.run_scoped(
                functools.partial(load_weights, wqkv, wo_s, pre_s),
                pltpu.VMEM((D * H, _LANE), _BF16),
                pltpu.VMEM((n_seg, _PRE, D), _BF16),
                pltpu.VMEM((ND, n_seg * _PRE, _LANE), _F32),
                pltpu.VMEM((ND // 2, 7, n_seg * _PRE // 4, _LANE), _U32),
                pltpu.VMEM((5 * ND, D, _LANE), _BF16),
                pltpu.VMEM((2, ND, 8, _LANE), _F32),
                pltpu.SemaphoreType.DMA((ND,)),
                pltpu.SemaphoreType.DMA((5 * ND,)),
                pltpu.SemaphoreType.DMA((ND + 2,)),
            )
            after_weights(wqkv, wo_s, pre_s, w1_v, w2_v, w3_v, w4_v, hb_s, n0_s)

        pl.run_scoped(
            attention,
            pltpu.VMEM((3 * H, D // 2, _LANE), _U32),
            pltpu.VMEM((ND, H * _LANE, _LANE), _BF16),
            pltpu.VMEM((3 * H, n_seg * _PRE, _LANE), _F32),
        )
        pl.run_scoped(
            functools.partial(mixer, w1_v, w2_v, w3_v, w4_v, hb_s, n0_s),
            pltpu.VMEM((T, dq // 2, fq), _U32),
            pltpu.VMEM((T, fq // 2, dq), _U32),
            pltpu.VMEM((T, mq // 2, dq), _U32),
            pltpu.VMEM((T, mq // 2, fq), _U32),
            pltpu.VMEM((S, D), _F32),
            pltpu.VMEM((2, _TM // 2, D), _F32),
            pltpu.VMEM((D, D), _BF16),
            pltpu.VMEM((2, _TM, D), _BF16),
            pltpu.SemaphoreType.DMA((2,)),
            *[pltpu.VMEM((S + 2 * _HALO, _LANE), _F32) for _ in range(ND)],
        )

    pl.run_scoped(
        whole,
        pltpu.VMEM((D, D), _BF16),
        pltpu.VMEM((D, D), _BF16),
        pltpu.VMEM((D, F), _BF16),
        pltpu.VMEM((F, D), _BF16),
        pltpu.VMEM((S, D), _F32),
        pltpu.VMEM((S // 2, D), _U32),
    )


@functools.partial(jax.jit, static_argnames=("A_seg_len",))
def pallas_adaLN_cond__memory_aug_recurrent_mem_tr__mixer_s_mlp__prompt_kernel(
    A_x: jax.Array,
    A_mem0: jax.Array,
    A_Wq: jax.Array,
    A_Wk: jax.Array,
    A_Wv: jax.Array,
    A_Wo: jax.Array,
    A_seg_len: int,
    B_x: jax.Array,
    B_w1: jax.Array,
    B_w2: jax.Array,
    B_w3: jax.Array,
    B_w4: jax.Array,
    c: jax.Array,
    w_mod: jax.Array,
):
    del B_x
    batch, S, D = A_x.shape
    _, H, Dh = A_Wq.shape
    M = A_mem0.shape[1]
    seg_len = int(A_seg_len)
    assert batch == 1 and Dh == _LANE and S % _TM == 0 and _TM % seg_len == 0
    n_seg = S // seg_len

    vmem = pl.BlockSpec(memory_space=pltpu.VMEM)
    hbm = pl.BlockSpec(memory_space=pl.ANY)
    out = pl.pallas_call(
        _kernel,
        out_shape=jax.ShapeDtypeStruct((S, D), A_x.dtype),
        in_specs=[vmem, vmem] + [hbm] * 10,
        out_specs=hbm,
        scratch_shapes=[
            pltpu.VMEM((n_seg, seg_len, D), _BF16),
            pltpu.VMEM((S, D), _F32),
            pltpu.VMEM((6, 8, D), _F32),
            pltpu.VMEM((8, _LANE), _U32),
            pltpu.SemaphoreType.DMA((6,)),
        ],
        compiler_params=pltpu.CompilerParams(vmem_limit_bytes=126 * 1024 * 1024),
        name="adaln_rmt_mixer",
    )(
        A_mem0.reshape(M, D), c, A_x.reshape(n_seg, seg_len, D),
        A_Wq.reshape(D * H, Dh), A_Wk.reshape(D * H, Dh), A_Wv.reshape(D * H, Dh),
        A_Wo.reshape(H * Dh, D), B_w1, B_w2, B_w3, B_w4, w_mod,
    )
    return out.reshape(batch, S, D)
```

```python
import functools
import math

import jax
import jax.numpy as jnp
from jax import lax
import jax.experimental.pallas as pl
import jax.experimental.pallas.tpu as pltpu

_F32 = jnp.float32
_BF16 = jnp.bfloat16
_U32 = jnp.uint32
_LANE = 128
_EPS = 1e-05
_TM = 256
_LEVEL = 2
_UNROLL = 2
_HALO = 8
_PRE = 8
_G = 4


def _dot(a, b):
    return lax.dot_general(a, b, (((1,), (0,)), ((), ())), preferred_element_type=_F32)


def _dot_nt(a, b):
    return lax.dot_general(a, b, (((1,), (1,)), ((), ())), preferred_element_type=_F32)


def _layernorm(x):
    m = jnp.mean(x, axis=-1, keepdims=True)
    d = x - m
    v = jnp.mean(d * d, axis=-1, keepdims=True)
    return d * lax.rsqrt(v + _EPS)


def _gelu(x):
    c = math.sqrt(2.0 / math.pi)
    inner = x * (c + (c * 0.044715) * (x * x))
    hx = 0.5 * x
    return hx + hx * jnp.tanh(inner)


def _pack(x):
    return pltpu.bitcast(x.astype(_BF16), _U32)


def _unpacked(x):
    return pltpu.bitcast(x, _BF16)


def _low_half(w):
    return pltpu.bitcast(w << 16, _F32)


def _high_half(w):
    return pltpu.bitcast(w & jnp.uint32(0xFFFF0000), _F32)


def _quads(g):
    n = len(g) // 2
    return [[row[j * n:(j + 1) * n] for row in g[i * n:(i + 1) * n]]
            for i in range(2) for j in range(2)]


def _add(a, b):
    return [[x + y for x, y in zip(r, t)] for r, t in zip(a, b)]


def _sub(a, b):
    return [[x - y for x, y in zip(r, t)] for r, t in zip(a, b)]


def _lhs_terms(g):
    if len(g) == 1:
        return [g[0][0]]
    a11, a12, a21, a22 = _quads(g)
    terms = (_sub(a11, a22), _sub(a21, a22), a22, _sub(a21, a11), _sub(a22, a12), a11,
             _sub(a11, a12))
    return [v for t in terms for v in _lhs_terms(t)]


def _rhs_terms(g):
    if len(g) == 1:
        return [g[0][0]]
    b11, b12, b21, b22 = _quads(g)
    terms = (_sub(b11, b22), b11, _add(b21, b11), _add(b11, b12), _add(b21, b22), _add(b12, b22),
             b22)
    return [v for t in terms for v in _rhs_terms(t)]


def _combine(level, product, base=0, emit=None):
    if level == 0:
        return [[product(base)]]

    def m(i):
        return _combine(level - 1, product, base + i * 7 ** (level - 1))

    def done(qi, qj, g):
        if emit is None:
            return g
        n = len(g)
        return [[emit(qi * n + a, qj * n + b, g[a][b]) for b in range(n)] for a in range(n)]

    m0, m1 = m(0), m(1)
    c22 = _sub(m0, m1)
    m2 = m(2)
    c11 = _add(m0, m2)
    c21 = done(1, 0, _add(m1, m2))
    m5 = m(5)
    c22 = _add(c22, m5)
    m6 = m(6)
    c11 = _add(c11, m6)
    c12 = done(0, 1, _sub(m5, m6))
    c22 = done(1, 1, _add(m(3), c22))
    c11 = done(0, 0, _sub(c11, m(4)))
    return [x + y for x, y in zip(c11, c12)] + [x + y for x, y in zip(c21, c22)]


def _aligned(start, size):
    return pl.ds(pl.multiple_of(start, size), size)


def _cols(j, n=_LANE):
    return slice(j * n, (j + 1) * n)


def _loop(lo, hi, fn):
    def body(i, carry):
        fn(i)
        return carry
    lax.fori_loop(lo, hi, body, 0)


def _start(cps):
    for cp in cps:
        cp.start()


def _wait(cps):
    for cp in cps:
        cp.wait()


def _kernel(mem0_ref, c_ref, x_hbm, wq_hbm, wk_hbm, wv_hbm, wo_hbm, w1_hbm, w2_hbm, w3_hbm,
            w4_hbm, wmod_hbm, out_hbm, x_v, a_s, mod_s, zero_s, sems):
    n_seg, seg_len, D = x_v.shape
    S = n_seg * seg_len
    M = mem0_ref.shape[0]
    H = wo_hbm.shape[0] // _LANE
    F = w3_hbm.shape[1]
    L = M + seg_len
    ND = D // _LANE
    P = 2 ** _LEVEL
    T = 7 ** _LEVEL
    mq, dq, fq = _TM // P, D // P, F // P
    scale = float(_LANE) ** -0.5
    copy = pltpu.make_async_copy

    def mod(r, cols=slice(None)):
        return mod_s[r, 0:1, cols]

    cf = c_ref[...].astype(_F32)
    silu_c = jnp.broadcast_to(cf * jax.nn.sigmoid(cf), (8, D))
    x_head = 8
    cp_x_tail = copy(x_hbm.at[pl.ds(x_head, n_seg - x_head)],
                     x_v.at[pl.ds(x_head, n_seg - x_head)], sems.at[2])
    zero_s[...] = jnp.zeros(zero_s.shape, _U32)

    def paced(w, jobs):
        step = w.shape[0] // (_LANE // 2) // max(len(jobs), 1) * (_LANE // 2)
        parts = []
        for n, job in enumerate(jobs):
            tiles = [pltpu.bitcast(v, _U32)[r:r + 8, c:c + _LANE] for v in job()
                     for r in range(0, v.shape[0], 8) for c in range(0, v.shape[1], _LANE)]
            done = functools.reduce(jnp.bitwise_or, tiles) & zero_s[...]
            parts += [w[n * step:n * step + 8] | done, w[n * step + 8:(n + 1) * step]]
        if len(jobs) * step < w.shape[0]:
            parts.append(w[len(jobs) * step:])
        return _unpacked(jnp.concatenate(parts, axis=0))

    def load_weights(wqkv, wo_s, pre_s, stage, xq_v, nq_s, hq_s, wmod_v, moda_s, w_sems, m_sems,
                     o_sems):
        rows_c = _LANE * H
        words = stage.bitcast(_U32)
        w_hbm = (wq_hbm, wk_hbm, wv_hbm)

        def w_copy(t, j):
            return copy(w_hbm[t].at[_aligned(j * rows_c, rows_c), :],
                        stage.at[_aligned(j * rows_c, rows_c), :], w_sems.at[j])

        def m_copy(r, j):
            n = r % 3 * ND + j
            return copy(wmod_hbm.at[:, _aligned((r * ND + j) * _LANE, _LANE)], wmod_v.at[n],
                        m_sems.at[n])

        def modulate(j):
            hs = []
            for u in (2 * j, 2 * j + 1):
                shift = _dot(silu_c, wmod_v[u])
                gain = 1.0 + _dot(silu_c, wmod_v[ND + u])
                moda_s[0, u] = shift
                moda_s[1, u] = gain
                hs.append(nq_s[u] * gain[0:1] + shift[0:1])
            mh = hs[0].shape[0] // 2
            for n, v in enumerate(_lhs_terms([[h[_cols(a, mh)] for h in hs] for a in range(2)])):
                hq_s[j, n] = _pack(v)

        def absorb(t, j):
            src = words.at[_aligned(j * rows_c, rows_c), :]
            dst = wqkv.at[pl.ds(t * H, H), _aligned(j * _LANE, _LANE), :]
            acc = pre_s.at[pl.ds(t * H, H)]
            lhs = hq_s.at[j]
            mh = lhs.shape[1] * 2
            for hp in range(H // 2):
                w = src[pl.ds(hp, 2 * _LANE, stride=H // 2), :]
                pair = (_low_half(w), _high_half(w))
                for i in range(2):
                    dst[2 * hp + i] = _pack(pair[i])
                rhs = _rhs_terms([[v[_cols(u)] for v in pair] for u in range(2)])

                def emit(a, b, y):
                    old = acc[2 * hp + b, _cols(a, mh), :]
                    acc[2 * hp + b, _cols(a, mh), :] = y + jnp.where(j == 0, 0.0, old)

                _combine(1, lambda n: _dot(_unpacked(lhs[n]), rhs[n].astype(_BF16)), emit=emit)

        cp_xq = copy(x_hbm.at[:, pl.ds(seg_len - _PRE, _PRE), :], xq_v, o_sems.at[ND])
        cp_x_head = copy(x_hbm.at[pl.ds(0, x_head)], x_v.at[pl.ds(0, x_head)], o_sems.at[ND + 1])
        cp_wo = [copy(wo_hbm.bitcast(_U32).at[:, pl.ds(n * _LANE, _LANE)], wo_s.at[n], o_sems.at[n])
                 for n in range(ND)]
        cp_mb = [m_copy(r, j) for r in range(2, 5) for j in range(ND)]

        mu = [[m_copy(0, j), m_copy(1, j)] for j in range(ND)]
        qu, ku, vu = ([[w_copy(t, j)] for j in range(ND)] for t in range(3))
        m2, q2, k2, v2 = ([u[2 * j] + u[2 * j + 1] for j in range(ND // 2)] for u in (mu, qu, ku, vu))
        plan = [q2[1] + m2[2], q2[2] + m2[3] + cp_wo[0:1], q2[3] + k2[0],
                k2[1] + k2[2], k2[3] + cp_wo[1:4], v2[0] + cp_wo[4:6], v2[1] + cp_wo[6:],
                v2[2] + cp_mb[:ND], v2[3] + cp_mb[ND:2 * ND], cp_mb[2 * ND:] + [cp_x_head]]

        with jax.named_scope('sc_first'):
            _start([cp_xq] + m2[0] + q2[0])
            cp_xq.wait()
            nq = _layernorm(xq_v[...].astype(_F32).reshape(n_seg * _PRE, D))
            for j in range(ND):
                nq_s[j] = nq[:, _cols(j)]
            _wait(m2[0])
            _start(m2[1])

        def step(i):
            t, j = i // (ND // 2), i % (ND // 2)

            @pl.when(t == 0)
            def _():
                pl.when(j > 0)(functools.partial(
                    _wait, [m_copy(r, 2 * j + u) for r in range(2) for u in range(2)]))
                modulate(j)

            for tt in range(3):
                pl.when(t == tt)(functools.partial(_wait, [w_copy(tt, 2 * j), w_copy(tt, 2 * j + 1)]))
            for n, cps in enumerate(plan):
                pl.when(i == n)(functools.partial(_start, cps))
            absorb(t, j)
        with jax.named_scope('sc_kv'):
            _loop(0, 3 * ND // 2, step)

        with jax.named_scope('sc_wo'):
            _wait(cp_wo + [cp_x_head] + cp_mb)
            for r in range(2):
                mod_s[r] = jnp.concatenate([moda_s[r, j] for j in range(ND)], axis=1)
            for r in range(2, 5):
                w = jnp.concatenate([wmod_v[r % 3 * ND + j] for j in range(ND)], axis=1)
                y = _dot(silu_c, w)
                mod_s[r] = 1.0 + y if r == 4 else y

    def residual(x, a):
        return x.astype(_F32) + mod(2) * a

    def recurrence(wqkv, wo_s, pre_s, hb_s, n0_s, mem_s, seg_s, o_s, prev_s):
        def seg_input(s, buf, r):
            h = _layernorm(x_v[s, r:r + 8, :].astype(_F32)) * mod(1) + mod(0)
            seg_s[buf, r:r + 8, :] = h
            return [h]

        def mixer_input(s, r):
            hb = _layernorm(residual(x_v[s, r:r + 16, :], prev_s[r:r + 16, :])) * mod(4) + mod(3)
            hb_s[_aligned(s * seg_len + r, 16), :] = hb
            n0 = _pack(_layernorm(hb))
            n0_s[_aligned((s * seg_len + r) // 2, 8), :] = n0
            return [n0]

        def seg_jobs(s, buf):
            return [functools.partial(seg_input, s, buf, r) for r in range(0, seg_len - _PRE, 8)]

        def mixer_jobs(s):
            return [functools.partial(mixer_input, s, r) for r in range(0, seg_len, 16)]

        mem_s[...] = mem0_ref[...].astype(_F32)
        for job in seg_jobs(0, 0):
            job()
        prev_s[...] = jnp.zeros(prev_s.shape, _F32)

        row = lax.broadcasted_iota(jnp.int32, (L, L), 0)
        col = lax.broadcasted_iota(jnp.int32, (L, L), 1)
        mask = (row < M) | (row >= col)
        half = D // 2

        def seg_step(s, buf, mem):
            jobs = mixer_jobs(jnp.maximum(s - 1, 0)) + seg_jobs(jnp.minimum(s + 1, n_seg - 1), buf)
            lhs = [jnp.concatenate([mem[i], seg_s[buf, :, _cols(i, half)]], axis=0).astype(_BF16)
                   for i in range(2)]
            pre = pre_s.at[:, _aligned(s * _PRE, _PRE), :]

            def proj_part(ids, parts):
                rows = slice(parts[0] * half // 2, (parts[-1] + 1) * half // 2)
                due = {ids[-1]: [jobs.pop(0)]} if jobs and ids[-1] >= 2 * H + _G else {}
                w = jnp.concatenate([paced(wqkv[n, rows, :], due.get(n, [])) for n in ids], axis=1)
                return _dot(jnp.concatenate([lhs[i] for i in parts], axis=1), w)

            def proj(ids, y=None):
                y = proj_part(ids, (0, 1)) if y is None else proj_part(ids, (1,)) + y
                return [jnp.concatenate([y[:, _cols(i)], pre[n]], axis=0) for i, n in enumerate(ids)]

            def weights(q, k):
                sc = jnp.where(mask, _dot_nt(q, k.astype(_BF16)) * scale, -1000000000.0)
                e = jnp.exp(sc - jnp.max(sc, axis=-1, keepdims=True))
                return e, jnp.sum(e, axis=-1, keepdims=True)

            def mix(h0, ws, vs):
                for i, ((e, den), v) in enumerate(zip(ws, vs)):
                    o_s[:, _cols(h0 + i)] = _dot(e, v.astype(_BF16)) / den

            def out_proj(h0, h1, part):
                ks = slice(h0 * _LANE, h1 * _LANE)
                cols = range(part * ND // 2, (part + 1) * ND // 2)
                w = [_unpacked(wo_s[n, h0 * _LANE // 2:h1 * _LANE // 2, :]) for n in cols]
                return _dot(o_s[:, ks], jnp.concatenate(w, axis=1))

            pend = None
            for h in range(0, H, _G):
                ids = [t * H + h + i for t in range(3) for i in range(_G)]
                if pend is None:
                    qkv = proj(ids[:2 * _G], proj_part(ids[:2 * _G], (0,))) + proj(ids[2 * _G:])
                else:
                    qkv = proj(ids)
                    mix(*pend)
                pend = (h, [weights(q, k) for q, k in zip(qkv[:_G], qkv[_G:2 * _G])], qkv[2 * _G:])
            y0 = out_proj(0, H - _G, 0)
            mix(*pend)
            y1 = out_proj(0, 2 * _G, 1)
            y0 = out_proj(H - _G, H, 0) + y0
            y1 = out_proj(2 * _G, H, 1) + y1
            assert not jobs
            for i, y in enumerate((y0, y1)):
                a_s[_aligned(s * seg_len, seg_len), _cols(i, half)] = y[M:L]
                prev_s[:, _cols(i, half)] = y[M:L]
            return y0[0:M], y1[0:M]

        def seg_steps(i):
            pl.when(i == x_head // _UNROLL - 1)(cp_x_tail.wait)
            mem = (mem_s[:, 0:half], mem_s[:, half:D])
            for u in range(_UNROLL):
                mem = seg_step(i * _UNROLL + u, 0, mem)
            mem_s[:, 0:half] = mem[0]
            mem_s[:, half:D] = mem[1]

        with jax.named_scope('sc_attn'):
            _loop(0, n_seg // _UNROLL, seg_steps)
        for job in mixer_jobs(n_seg - 1):
            job()

    def mixer(w1_v, w2_v, w3_v, w4_v, hb_s, n0_s, t3_s, t4_s, a1_s, a2_s, n1_s, last_s, wg_v, out_s, out_sems,
              *g_s):
        n_blk = S // _TM
        shifts = [(-1, 1, -2, 2)[j * _LANE * 4 // D] for j in range(ND)]
        cp_gate = copy(wmod_hbm.at[:, pl.ds(5 * D, D)], wg_v, sems.at[3])
        cp_gate.start()
        last_s[1] = jnp.zeros(last_s.shape[1:], _F32)
        for g in g_s:
            g[_HALO:2 * _HALO, :] = jnp.zeros((_HALO, _LANE), _F32)
            g[S:S + _HALO, :] = jnp.zeros((_HALO, _LANE), _F32)

        def block(ref, i, n=_TM):
            return ref.at[_aligned(i * n, n), :]

        def weight_terms(src, dst, i, r, col):
            nr, nc = src.shape[0] // P, src.shape[1] // P
            n = nr // n_blk
            dst = dst.at[:, pl.ds(pl.multiple_of(i * (n // 2), 8), n // 2), :]
            w = [[pltpu.bitcast(src[_aligned(a * nr + i * n + r, 16),
                                    b * nc + col:b * nc + col + _LANE], _U32)
                  for b in range(P)] for a in range(P)]
            lo = _rhs_terms([[_low_half(v) for v in row] for row in w])
            hi = _rhs_terms([[_high_half(v) for v in row] for row in w])
            out = [pltpu.pack_elementwise(list(pair), packed_dtype=_BF16) for pair in zip(lo, hi)]
            for t, v in enumerate(out):
                dst[t, r // 2:r // 2 + 8, col:col + _LANE] = v
            return out

        def weight_jobs(src, dst, i):
            return [functools.partial(weight_terms, src, dst, i, r, col)
                    for r in range(0, src.shape[0] // P // n_blk, 16)
                    for col in range(0, src.shape[1] // P, _LANE)]

        def spread(jobs):
            cut = [j * len(jobs) // (ND - 1) for j in range(ND)]
            return [[]] + [jobs[cut[j]:cut[j + 1]] for j in range(ND - 1)]

        def gate(i):
            n0 = _unpacked(block(n0_s, i, _TM // 2)[...])
            for j, (g, off, jobs) in enumerate(zip(g_s, shifts, spread(weight_jobs(w3_v, t3_s, i)))):
                win = g.at[pl.ds(pl.multiple_of(i * _TM, _TM), _TM + 2 * _HALO), :]
                w = paced(w1_v[j], jobs)
                win[_HALO - off:_HALO - off + _TM, :] = _gelu(_dot(n0, w))

        th = 128
        nh = _TM // th

        def mlp_norm(k, buf, r):
            n1 = _layernorm(last_s[buf, r:r + 16, :])
            block(n1_s, k, th)[r:r + 16, :] = n1
            return [n1]

        def norm_jobs(k, buf):
            return [functools.partial(mlp_norm, k, buf, r) for r in range(0, th, 16)]

        def mix(i):
            terms = weight_jobs(w4_v, t4_s, i)
            for u in range(nh):
                x1 = block(hb_s, i).at[u * th:(u + 1) * th, :]
                rows = pl.ds(pl.multiple_of(i * _TM + u * th + _HALO, _HALO), th)
                shifted = jnp.concatenate([g[rows, :] for g in g_s], axis=1).astype(_BF16)
                due = zip(spread(norm_jobs(jnp.maximum(nh * i + u - 1, 0), 1 - u % 2)),
                          spread(terms[u::nh]))
                for j, (norms, jobs) in enumerate(due):
                    w = paced(w2_v[j], jobs + norms)
                    y = _dot(shifted, w) + x1[:, _cols(j)]
                    x1[:, _cols(j)] = y
                    last_s[u % 2, :, _cols(j)] = y

        def mlp_terms(i, r, col):
            n1 = block(n1_s, i)
            g = [[n1[a * mq + r:a * mq + r + 16, b * dq + col:b * dq + col + _LANE]
                  for b in range(P)] for a in range(P)]
            out = [_pack(v) for v in _lhs_terms(g)]
            for t, v in enumerate(out):
                a1_s[t, r // 2:r // 2 + 8, col:col + _LANE] = v
            return out

        def term_jobs(i):
            return [functools.partial(mlp_terms, i, r, col)
                    for r in range(0, mq, 16) for col in range(0, dq, _LANE)]

        def products(a_ref, w_ref, jobs, every):
            count = [0]

            def product(p, t):
                count[0] += 1
                due = [jobs.pop(0)] if jobs and count[0] % every == 0 else []
                return _dot(_unpacked(a_ref[t]), paced(w_ref[t, :, _cols(p)], due))
            return product

        def out_copy(i, slot):
            return copy(out_s.at[slot], block(out_hbm, i), out_sems.at[slot])

        def mlp(i):
            slot = i % 2

            @pl.when(i >= 2)
            def _():
                out_copy(jnp.maximum(i - 2, 0), slot).wait()

            terms = term_jobs(jnp.minimum(i + 1, n_blk - 1))
            up, down = products(a1_s, t3_s, [], 1), products(a2_s, t4_s, terms, 10)
            for p in range(fq // _LANE):
                g = _combine(_LEVEL, functools.partial(up, p), emit=lambda a, b, y: _gelu(y))
                for t, v in enumerate(_lhs_terms(g)):
                    a2_s[t, :, _cols(p)] = _pack(v)

            dst, att, x1 = out_s.at[slot], block(a_s, i), block(hb_s, i)
            x = x_v.at[pl.ds(i * (_TM // seg_len), _TM // seg_len)]
            for p in range(dq // _LANE):
                def emit(a, b, y):
                    rows, cols = slice(a * mq, (a + 1) * mq), _cols(b * (dq // _LANE) + p)
                    xs = x[a * mq // seg_len:(a + 1) * mq // seg_len, :, cols]
                    res = (xs.astype(_F32).reshape(mq, _LANE) + mod(2, cols) * att[rows, cols]
                           + mod(5, cols) * (x1[rows, cols] + y))
                    dst[rows, cols] = res.astype(dst.dtype)

                _combine(_LEVEL, functools.partial(down, p), emit=emit)
            assert not terms
            out_copy(i, slot).start()

        with jax.named_scope('sc_s1'):
            _loop(0, n_blk, gate)
        with jax.named_scope('sc_s2'):
            _loop(0, n_blk, mix)
        cp_gate.wait()
        norms, terms = norm_jobs(nh * n_blk - 1, 1), term_jobs(0)
        mod_s[5] = jnp.concatenate(
            [_dot(silu_c, paced(pltpu.bitcast(wg_v[:, _cols(j)], _U32), norms[j::ND] + terms[j::ND]))
             for j in range(ND)], axis=1)
        with jax.named_scope('sc_s3'):
            _loop(0, n_blk, mlp)
        for i in (n_blk - 2, n_blk - 1):
            out_copy(i, i % 2).wait()

    def after_weights(wqkv, wo_s, pre_s, w1_v, w2_v, w3_v, w4_v, hb_s, n0_s):
        cps = [copy(w3_hbm, w3_v, sems.at[0]), copy(w4_hbm, w4_v, sems.at[1])]
        cps += [copy(src.bitcast(_U32).at[:, pl.ds(j * _LANE, _LANE)], dst.at[j],
                     sems.at[4 + n * ND + j])
                for n, (src, dst) in enumerate(((w1_hbm, w1_v), (w2_hbm, w2_v))) for j in range(ND)]
        _start([cp_x_tail] + cps)
        pl.run_scoped(
            functools.partial(recurrence, wqkv, wo_s, pre_s, hb_s, n0_s),
            pltpu.VMEM((M, D), _F32),
            pltpu.VMEM((2, seg_len - _PRE, D), _F32),
            pltpu.VMEM((L, H * _LANE), _F32),
            pltpu.VMEM((seg_len, D), _F32),
        )
        _wait(cps)

    def whole(w1_v, w2_v, w3_v, w4_v, hb_s, n0_s):
        def attention(wqkv, wo_s, pre_s):
            pl.run_scoped(
                functools.partial(load_weights, wqkv, wo_s, pre_s),
                pltpu.VMEM((D * H, _LANE), _BF16),
                pltpu.VMEM((n_seg, _PRE, D), _BF16),
                pltpu.VMEM((ND, n_seg * _PRE, _LANE), _F32),
                pltpu.VMEM((ND // 2, 7, n_seg * _PRE // 4, _LANE), _U32),
                pltpu.VMEM((3 * ND, D, _LANE), _BF16),
                pltpu.VMEM((2, ND, 8, _LANE), _F32),
                pltpu.SemaphoreType.DMA((ND,)),
                pltpu.SemaphoreType.DMA((3 * ND,)),
                pltpu.SemaphoreType.DMA((ND + 2,)),
            )
            after_weights(wqkv, wo_s, pre_s, w1_v, w2_v, w3_v, w4_v, hb_s, n0_s)

        pl.run_scoped(
            attention,
            pltpu.VMEM((3 * H, D // 2, _LANE), _U32),
            pltpu.VMEM((ND, H * _LANE // 2, _LANE), _U32),
            pltpu.VMEM((3 * H, n_seg * _PRE, _LANE), _F32),
        )
        pl.run_scoped(
            functools.partial(mixer, w1_v, w2_v, w3_v, w4_v, hb_s, n0_s),
            pltpu.VMEM((T, dq // 2, fq), _U32),
            pltpu.VMEM((T, fq // 2, dq), _U32),
            pltpu.VMEM((T, mq // 2, dq), _U32),
            pltpu.VMEM((T, mq // 2, fq), _U32),
            pltpu.VMEM((S, D), _F32),
            pltpu.VMEM((2, 128, D), _F32),
            pltpu.VMEM((D, D), _BF16),
            pltpu.VMEM((2, _TM, D), _BF16),
            pltpu.SemaphoreType.DMA((2,)),
            *[pltpu.VMEM((S + 2 * _HALO, _LANE), _F32) for _ in range(ND)],
        )

    pl.run_scoped(
        whole,
        pltpu.VMEM((ND, D // 2, _LANE), _U32),
        pltpu.VMEM((ND, D // 2, _LANE), _U32),
        pltpu.VMEM((D, F), _BF16),
        pltpu.VMEM((F, D), _BF16),
        pltpu.VMEM((S, D), _F32),
        pltpu.VMEM((S // 2, D), _U32),
    )


@functools.partial(jax.jit, static_argnames=("A_seg_len",))
def pallas_adaLN_cond__memory_aug_recurrent_mem_tr__mixer_s_mlp__prompt_kernel(
    A_x: jax.Array,
    A_mem0: jax.Array,
    A_Wq: jax.Array,
    A_Wk: jax.Array,
    A_Wv: jax.Array,
    A_Wo: jax.Array,
    A_seg_len: int,
    B_x: jax.Array,
    B_w1: jax.Array,
    B_w2: jax.Array,
    B_w3: jax.Array,
    B_w4: jax.Array,
    c: jax.Array,
    w_mod: jax.Array,
):
    del B_x
    batch, S, D = A_x.shape
    _, H, Dh = A_Wq.shape
    M = A_mem0.shape[1]
    seg_len = int(A_seg_len)
    assert batch == 1 and Dh == _LANE and S % _TM == 0 and _TM % seg_len == 0
    n_seg = S // seg_len

    vmem = pl.BlockSpec(memory_space=pltpu.VMEM)
    hbm = pl.BlockSpec(memory_space=pl.ANY)
    out = pl.pallas_call(
        _kernel,
        out_shape=jax.ShapeDtypeStruct((S, D), A_x.dtype),
        in_specs=[vmem, vmem] + [hbm] * 10,
        out_specs=hbm,
        scratch_shapes=[
            pltpu.VMEM((n_seg, seg_len, D), _BF16),
            pltpu.VMEM((S, D), _F32),
            pltpu.VMEM((6, 8, D), _F32),
            pltpu.VMEM((8, _LANE), _U32),
            pltpu.SemaphoreType.DMA((4 + 2 * D // _LANE,)),
        ],
        compiler_params=pltpu.CompilerParams(vmem_limit_bytes=126 * 1024 * 1024),
        name="adaln_rmt_mixer",
    )(
        A_mem0.reshape(M, D), c, A_x.reshape(n_seg, seg_len, D),
        A_Wq.reshape(D * H, Dh), A_Wk.reshape(D * H, Dh), A_Wv.reshape(D * H, Dh),
        A_Wo.reshape(H * Dh, D), B_w1, B_w2, B_w3, B_w4, w_mod,
    )
    return out.reshape(batch, S, D)
```

```python
import functools
import math

import jax
import jax.numpy as jnp
from jax import lax
import jax.experimental.pallas as pl
import jax.experimental.pallas.tpu as pltpu

_F32 = jnp.float32
_BF16 = jnp.bfloat16
_U32 = jnp.uint32
_LANE = 128
_EPS = 1e-05
_TM = 256
_LEVEL = 2
_UNROLL = 2
_HALO = 8
_PRE = 8
_G = 4


def _dot(a, b):
    return lax.dot_general(a, b, (((1,), (0,)), ((), ())), preferred_element_type=_F32)


def _dot_nt(a, b):
    return lax.dot_general(a, b, (((1,), (1,)), ((), ())), preferred_element_type=_F32)


def _layernorm(x):
    m = jnp.mean(x, axis=-1, keepdims=True)
    d = x - m
    v = jnp.mean(d * d, axis=-1, keepdims=True)
    return d * lax.rsqrt(v + _EPS)


def _gelu(x):
    c = math.sqrt(2.0 / math.pi)
    inner = x * (c + (c * 0.044715) * (x * x))
    hx = 0.5 * x
    return hx + hx * jnp.tanh(inner)


def _pack(x):
    return pltpu.bitcast(x.astype(_BF16), _U32)


def _unpacked(x):
    return pltpu.bitcast(x, _BF16)


def _low_half(w):
    return pltpu.bitcast(w << 16, _F32)


def _high_half(w):
    return pltpu.bitcast(w & jnp.uint32(0xFFFF0000), _F32)


def _quads(g):
    n = len(g) // 2
    return [[row[j * n:(j + 1) * n] for row in g[i * n:(i + 1) * n]]
            for i in range(2) for j in range(2)]


def _add(a, b):
    return [[x + y for x, y in zip(r, t)] for r, t in zip(a, b)]


def _sub(a, b):
    return [[x - y for x, y in zip(r, t)] for r, t in zip(a, b)]


def _lhs_terms(g):
    if len(g) == 1:
        return [g[0][0]]
    a11, a12, a21, a22 = _quads(g)
    terms = (_sub(a11, a22), _sub(a21, a22), a22, _sub(a21, a11), _sub(a22, a12), a11,
             _sub(a11, a12))
    return [v for t in terms for v in _lhs_terms(t)]


def _rhs_terms(g):
    if len(g) == 1:
        return [g[0][0]]
    b11, b12, b21, b22 = _quads(g)
    terms = (_sub(b11, b22), b11, _add(b21, b11), _add(b11, b12), _add(b21, b22), _add(b12, b22),
             b22)
    return [v for t in terms for v in _rhs_terms(t)]


def _combine(level, product, base=0, emit=None):
    if level == 0:
        return [[product(base)]]

    def m(i):
        return _combine(level - 1, product, base + i * 7 ** (level - 1))

    def done(qi, qj, g):
        if emit is None:
            return g
        n = len(g)
        return [[emit(qi * n + a, qj * n + b, g[a][b]) for b in range(n)] for a in range(n)]

    m0, m1 = m(0), m(1)
    c22 = _sub(m0, m1)
    m2 = m(2)
    c11 = _add(m0, m2)
    c21 = done(1, 0, _add(m1, m2))
    m5 = m(5)
    c22 = _add(c22, m5)
    m6 = m(6)
    c11 = _add(c11, m6)
    c12 = done(0, 1, _sub(m5, m6))
    c22 = done(1, 1, _add(m(3), c22))
    c11 = done(0, 0, _sub(c11, m(4)))
    return [x + y for x, y in zip(c11, c12)] + [x + y for x, y in zip(c21, c22)]


def _aligned(start, size):
    return pl.ds(pl.multiple_of(start, size), size)


def _cols(j, n=_LANE):
    return slice(j * n, (j + 1) * n)


def _loop(lo, hi, fn):
    def body(i, carry):
        fn(i)
        return carry
    lax.fori_loop(lo, hi, body, 0)


def _start(cps):
    for cp in cps:
        cp.start()


def _wait(cps):
    for cp in cps:
        cp.wait()


def _kernel(mem0_ref, c_ref, x_hbm, wq_hbm, wk_hbm, wv_hbm, wo_hbm, w1_hbm, w2_hbm, w3_hbm,
            w4_hbm, wmod_hbm, out_hbm, x_v, a_s, mod_s, zero_s, sems):
    n_seg, seg_len, D = x_v.shape
    S = n_seg * seg_len
    M = mem0_ref.shape[0]
    H = wo_hbm.shape[0] // _LANE
    F = w3_hbm.shape[1]
    L = M + seg_len
    ND = D // _LANE
    P = 2 ** _LEVEL
    T = 7 ** _LEVEL
    mq, dq, fq = _TM // P, D // P, F // P
    scale = float(_LANE) ** -0.5
    copy = pltpu.make_async_copy

    def mod(r, cols=slice(None)):
        return mod_s[r, 0:1, cols]

    cf = c_ref[...].astype(_F32)
    silu_c = jnp.broadcast_to(cf * jax.nn.sigmoid(cf), (8, D))
    x_head = 8
    cp_x_tail = copy(x_hbm.at[pl.ds(x_head, n_seg - x_head)],
                     x_v.at[pl.ds(x_head, n_seg - x_head)], sems.at[2])
    zero_s[...] = jnp.zeros(zero_s.shape, _U32)

    def paced(w, jobs):
        step = w.shape[0] // (_LANE // 2) // max(len(jobs), 1) * (_LANE // 2)
        parts = []
        for n, job in enumerate(jobs):
            tiles = [pltpu.bitcast(v, _U32)[r:r + 8, c:c + _LANE] for v in job()
                     for r in range(0, v.shape[0], 8) for c in range(0, v.shape[1], _LANE)]
            done = functools.reduce(jnp.bitwise_or, tiles) & zero_s[...]
            parts += [w[n * step:n * step + 8] | done, w[n * step + 8:(n + 1) * step]]
        if len(jobs) * step < w.shape[0]:
            parts.append(w[len(jobs) * step:])
        return _unpacked(jnp.concatenate(parts, axis=0))

    def load_weights(wqkv, wo_s, pre_s, stage, xq_v, nq_s, hq_s, wmod_v, moda_s, w_sems, m_sems,
                     o_sems):
        rows_c = _LANE * H
        words = stage.bitcast(_U32)
        w_hbm = (wq_hbm, wk_hbm, wv_hbm)

        def w_copy(t, j):
            return copy(w_hbm[t].at[_aligned(j * rows_c, rows_c), :],
                        stage.at[_aligned(j * rows_c, rows_c), :], w_sems.at[j])

        def m_copy(r, j):
            n = r % 3 * ND + j
            return copy(wmod_hbm.at[:, _aligned((r * ND + j) * _LANE, _LANE)], wmod_v.at[n],
                        m_sems.at[n])

        def modulate(j):
            hs = []
            for u in (2 * j, 2 * j + 1):
                shift = _dot(silu_c, wmod_v[u])
                gain = 1.0 + _dot(silu_c, wmod_v[ND + u])
                moda_s[0, u] = shift
                moda_s[1, u] = gain
                hs.append(nq_s[u] * gain[0:1] + shift[0:1])
            mh = hs[0].shape[0] // 2
            for n, v in enumerate(_lhs_terms([[h[_cols(a, mh)] for h in hs] for a in range(2)])):
                hq_s[j, n] = _pack(v)

        def absorb(t, j):
            src = words.at[_aligned(j * rows_c, rows_c), :]
            dst = wqkv.at[pl.ds(t * H, H), _aligned(j * _LANE, _LANE), :]
            acc = pre_s.at[pl.ds(t * H, H)]
            lhs = hq_s.at[j]
            mh = lhs.shape[1] * 2
            for hp in range(H // 2):
                w = src[pl.ds(hp, 2 * _LANE, stride=H // 2), :]
                pair = (_low_half(w), _high_half(w))
                for i in range(2):
                    dst[2 * hp + i] = _pack(pair[i])
                rhs = _rhs_terms([[v[_cols(u)] for v in pair] for u in range(2)])

                def emit(a, b, y):
                    old = acc[2 * hp + b, _cols(a, mh), :]
                    acc[2 * hp + b, _cols(a, mh), :] = y + jnp.where(j == 0, 0.0, old)

                _combine(1, lambda n: _dot(_unpacked(lhs[n]), rhs[n].astype(_BF16)), emit=emit)

        cp_xq = copy(x_hbm.at[:, pl.ds(seg_len - _PRE, _PRE), :], xq_v, o_sems.at[ND])
        cp_x_head = copy(x_hbm.at[pl.ds(0, x_head)], x_v.at[pl.ds(0, x_head)], o_sems.at[ND + 1])
        cp_wo = [copy(wo_hbm.bitcast(_U32).at[:, pl.ds(n * _LANE, _LANE)], wo_s.at[n], o_sems.at[n])
                 for n in range(ND)]
        cp_mb = [m_copy(r, j) for r in range(2, 5) for j in range(ND)]

        mu = [[m_copy(0, j), m_copy(1, j)] for j in range(ND)]
        qu, ku, vu = ([[w_copy(t, j)] for j in range(ND)] for t in range(3))
        m2, q2, k2, v2 = ([u[2 * j] + u[2 * j + 1] for j in range(ND // 2)] for u in (mu, qu, ku, vu))
        plan = [q2[1] + m2[2], q2[2] + m2[3] + cp_wo[0:1], q2[3] + k2[0],
                k2[1] + k2[2], k2[3] + cp_wo[1:4], v2[0] + cp_wo[4:6], v2[1] + cp_wo[6:],
                v2[2] + cp_mb[:ND], v2[3] + cp_mb[ND:2 * ND], cp_mb[2 * ND:] + [cp_x_head]]

        with jax.named_scope('sc_first'):
            _start([cp_xq] + m2[0] + q2[0])
            cp_xq.wait()
            nq = _layernorm(xq_v[...].astype(_F32).reshape(n_seg * _PRE, D))
            for j in range(ND):
                nq_s[j] = nq[:, _cols(j)]
            _wait(m2[0])
            _start(m2[1])

        def step(i):
            t, j = i // (ND // 2), i % (ND // 2)

            @pl.when(t == 0)
            def _():
                pl.when(j > 0)(functools.partial(
                    _wait, [m_copy(r, 2 * j + u) for r in range(2) for u in range(2)]))
                modulate(j)

            for tt in range(3):
                pl.when(t == tt)(functools.partial(_wait, [w_copy(tt, 2 * j), w_copy(tt, 2 * j + 1)]))
            for n, cps in enumerate(plan):
                pl.when(i == n)(functools.partial(_start, cps))
            absorb(t, j)
        with jax.named_scope('sc_kv'):
            _loop(0, 3 * ND // 2, step)

        with jax.named_scope('sc_wo'):
            _wait(cp_wo + [cp_x_head] + cp_mb)
            for r in range(2):
                mod_s[r] = jnp.concatenate([moda_s[r, j] for j in range(ND)], axis=1)
            for r in range(2, 5):
                w = jnp.concatenate([wmod_v[r % 3 * ND + j] for j in range(ND)], axis=1)
                y = _dot(silu_c, w)
                mod_s[r] = 1.0 + y if r == 4 else y

    def residual(x, a):
        return x.astype(_F32) + mod(2) * a

    def recurrence(wqkv, wo_s, pre_s, hb_s, n0_s, mem_s, seg_s, o_s, prev_s):
        def seg_input(s, buf, r):
            h = _layernorm(x_v[s, r:r + 8, :].astype(_F32)) * mod(1) + mod(0)
            seg_s[buf, r:r + 8, :] = h
            return [h]

        def mixer_input(s, r):
            hb = _layernorm(residual(x_v[s, r:r + 16, :], prev_s[r:r + 16, :])) * mod(4) + mod(3)
            hb_s[_aligned(s * seg_len + r, 16), :] = hb
            n0 = _pack(_layernorm(hb))
            n0_s[_aligned((s * seg_len + r) // 2, 8), :] = n0
            return [n0]

        def seg_jobs(s, buf):
            return [functools.partial(seg_input, s, buf, r) for r in range(0, seg_len - _PRE, 8)]

        def mixer_jobs(s):
            return [functools.partial(mixer_input, s, r) for r in range(0, seg_len, 16)]

        mem_s[...] = mem0_ref[...].astype(_F32)
        for job in seg_jobs(0, 0):
            job()
        prev_s[...] = jnp.zeros(prev_s.shape, _F32)

        row = lax.broadcasted_iota(jnp.int32, (L, L), 0)
        col = lax.broadcasted_iota(jnp.int32, (L, L), 1)
        mask = (row < M) | (row >= col)
        half = D // 2

        def seg_step(s, buf, mem):
            jobs = mixer_jobs(jnp.maximum(s - 1, 0)) + seg_jobs(jnp.minimum(s + 1, n_seg - 1), buf)
            lhs = [jnp.concatenate([mem[i], seg_s[buf, :, _cols(i, half)]], axis=0).astype(_BF16)
                   for i in range(2)]
            pre = pre_s.at[:, _aligned(s * _PRE, _PRE), :]

            def proj_part(ids, parts):
                rows = slice(parts[0] * half // 2, (parts[-1] + 1) * half // 2)
                due = {ids[-1]: [jobs.pop(0)]} if jobs and ids[-1] >= 2 * H + _G else {}
                w = jnp.concatenate([paced(wqkv[n, rows, :], due.get(n, [])) for n in ids], axis=1)
                return _dot(jnp.concatenate([lhs[i] for i in parts], axis=1), w)

            def proj(ids, y=None):
                y = proj_part(ids, (0, 1)) if y is None else proj_part(ids, (1,)) + y
                return [jnp.concatenate([y[:, _cols(i)], pre[n]], axis=0) for i, n in enumerate(ids)]

            def weights(q, k):
                sc = jnp.where(mask, _dot_nt(q, k.astype(_BF16)) * scale, -1000000000.0)
                e = jnp.exp(sc - jnp.max(sc, axis=-1, keepdims=True))
                return e / jnp.sum(e, axis=-1, keepdims=True)

            def mix(h0, ws, vs):
                for i, (p, v) in enumerate(zip(ws, vs)):
                    o_s[:, _cols(h0 + i)] = _dot(p, v.astype(_BF16))

            def out_proj(h0, h1, part):
                ks = slice(h0 * _LANE, h1 * _LANE)
                cols = range(part * ND // 2, (part + 1) * ND // 2)
                w = [_unpacked(wo_s[n, h0 * _LANE // 2:h1 * _LANE // 2, :]) for n in cols]
                return _dot(o_s[:, ks], jnp.concatenate(w, axis=1))

            pend = None
            for h in range(0, H, _G):
                ids = [t * H + h + i for t in range(3) for i in range(_G)]
                if pend is None:
                    qkv = proj(ids[:2 * _G], proj_part(ids[:2 * _G], (0,))) + proj(ids[2 * _G:])
                else:
                    qkv = proj(ids)
                    mix(*pend)
                pend = (h, [weights(q, k) for q, k in zip(qkv[:_G], qkv[_G:2 * _G])], qkv[2 * _G:])
            y0 = out_proj(0, H - _G, 0)
            mix(*pend)
            y1 = out_proj(0, 2 * _G, 1)
            y0 = out_proj(H - _G, H, 0) + y0
            y1 = out_proj(2 * _G, H, 1) + y1
            assert not jobs
            for i, y in enumerate((y0, y1)):
                a_s[_aligned(s * seg_len, seg_len), _cols(i, half)] = y[M:L]
                prev_s[:, _cols(i, half)] = y[M:L]
            return y0[0:M], y1[0:M]

        def seg_steps(i):
            pl.when(i == x_head // _UNROLL - 1)(cp_x_tail.wait)
            mem = (mem_s[:, 0:half], mem_s[:, half:D])
            for u in range(_UNROLL):
                mem = seg_step(i * _UNROLL + u, 0, mem)
            mem_s[:, 0:half] = mem[0]
            mem_s[:, half:D] = mem[1]

        with jax.named_scope('sc_attn'):
            _loop(0, n_seg // _UNROLL, seg_steps)
        for job in mixer_jobs(n_seg - 1):
            job()

    def mixer(w1_v, w2_v, w3_v, w4_v, hb_s, n0_s, t3_s, t4_s, a1_s, a2_s, n1_s, last_s, wg_v, out_s, out_sems,
              *g_s):
        n_blk = S // _TM
        shifts = [(-1, 1, -2, 2)[j * _LANE * 4 // D] for j in range(ND)]
        cp_gate = copy(wmod_hbm.at[:, pl.ds(5 * D, D)], wg_v, sems.at[3])
        cp_gate.start()
        last_s[1] = jnp.zeros(last_s.shape[1:], _F32)
        for g in g_s:
            g[_HALO:2 * _HALO, :] = jnp.zeros((_HALO, _LANE), _F32)
            g[S:S + _HALO, :] = jnp.zeros((_HALO, _LANE), _F32)

        def block(ref, i, n=_TM):
            return ref.at[_aligned(i * n, n), :]

        def weight_terms(src, dst, i, r, col):
            nr, nc = src.shape[0] // P, src.shape[1] // P
            n = nr // n_blk
            dst = dst.at[:, pl.ds(pl.multiple_of(i * (n // 2), 8), n // 2), :]
            w = [[pltpu.bitcast(src[_aligned(a * nr + i * n + r, 16),
                                    b * nc + col:b * nc + col + _LANE], _U32)
                  for b in range(P)] for a in range(P)]
            lo = _rhs_terms([[_low_half(v) for v in row] for row in w])
            hi = _rhs_terms([[_high_half(v) for v in row] for row in w])
            out = [pltpu.pack_elementwise(list(pair), packed_dtype=_BF16) for pair in zip(lo, hi)]
            for t, v in enumerate(out):
                dst[t, r // 2:r // 2 + 8, col:col + _LANE] = v
            return out

        def weight_jobs(src, dst, i):
            return [functools.partial(weight_terms, src, dst, i, r, col)
                    for r in range(0, src.shape[0] // P // n_blk, 16)
                    for col in range(0, src.shape[1] // P, _LANE)]

        def spread(jobs):
            cut = [j * len(jobs) // (ND - 1) for j in range(ND)]
            return [[]] + [jobs[cut[j]:cut[j + 1]] for j in range(ND - 1)]

        def gate(i):
            n0 = _unpacked(block(n0_s, i, _TM // 2)[...])
            for j, (g, off, jobs) in enumerate(zip(g_s, shifts, spread(weight_jobs(w3_v, t3_s, i)))):
                win = g.at[pl.ds(pl.multiple_of(i * _TM, _TM), _TM + 2 * _HALO), :]
                w = paced(w1_v[j], jobs)
                win[_HALO - off:_HALO - off + _TM, :] = _gelu(_dot(n0, w))

        th = 128
        nh = _TM // th

        def mlp_norm(k, buf, r):
            n1 = _layernorm(last_s[buf, r:r + 16, :])
            dst = n1_s.at[:, _aligned(k * th, th), :]
            for j in range(ND):
                dst[j, r:r + 16, :] = n1[:, _cols(j)]
            return [n1]

        def norm_jobs(k, buf):
            return [functools.partial(mlp_norm, k, buf, r) for r in range(0, th, 16)]

        def mix(i):
            terms = weight_jobs(w4_v, t4_s, i)
            for u in range(nh):
                x1 = block(hb_s, i).at[u * th:(u + 1) * th, :]
                rows = pl.ds(pl.multiple_of(i * _TM + u * th + _HALO, _HALO), th)
                shifted = jnp.concatenate([g[rows, :] for g in g_s], axis=1).astype(_BF16)
                due = zip(spread(norm_jobs(jnp.maximum(nh * i + u - 1, 0), 1 - u % 2)),
                          spread(terms[u::nh]))
                for j, (norms, jobs) in enumerate(due):
                    w = paced(w2_v[j], jobs + norms)
                    y = _dot(shifted, w) + x1[:, _cols(j)]
                    x1[:, _cols(j)] = y
                    last_s[u % 2, :, _cols(j)] = y

        def mlp_terms(i, r, col):
            n1 = n1_s.at[:, _aligned(i * _TM, _TM), :]
            even, odd = (_lhs_terms(
                [[n1[(b * dq + col) // _LANE, pl.ds(a * mq + r + u, 8, stride=2), :]
                  for b in range(P)] for a in range(P)]) for u in range(2))
            out = [pltpu.pack_elementwise(list(pair), packed_dtype=_BF16) for pair in zip(even, odd)]
            for t, v in enumerate(out):
                a1_s[t, r // 2:r // 2 + 8, col:col + _LANE] = v
            return out

        def term_jobs(i):
            return [functools.partial(mlp_terms, i, r, col)
                    for r in range(0, mq, 16) for col in range(0, dq, _LANE)]

        def products(a_ref, w_ref, jobs, every):
            count = [0]

            def product(p, t):
                count[0] += 1
                due = [jobs.pop(0)] if jobs and count[0] % every == 0 else []
                return _dot(_unpacked(a_ref[t]), paced(w_ref[t, :, _cols(p)], due))
            return product

        def out_copy(i, slot):
            return copy(out_s.at[slot], block(out_hbm, i), out_sems.at[slot])

        def mlp(i):
            slot = i % 2

            @pl.when(i >= 2)
            def _():
                out_copy(jnp.maximum(i - 2, 0), slot).wait()

            terms = term_jobs(jnp.minimum(i + 1, n_blk - 1))
            up, down = products(a1_s, t3_s, [], 1), products(a2_s, t4_s, terms, 10)
            for p in range(fq // _LANE):
                g = _combine(_LEVEL, functools.partial(up, p), emit=lambda a, b, y: _gelu(y))
                for t, v in enumerate(_lhs_terms(g)):
                    a2_s[t, :, _cols(p)] = _pack(v)

            dst, att, x1 = out_s.at[slot], block(a_s, i), block(hb_s, i)
            x = x_v.at[pl.ds(i * (_TM // seg_len), _TM // seg_len)]
            for p in range(dq // _LANE):
                def emit(a, b, y):
                    rows, cols = slice(a * mq, (a + 1) * mq), _cols(b * (dq // _LANE) + p)
                    xs = x[a * mq // seg_len:(a + 1) * mq // seg_len, :, cols]
                    res = (xs.astype(_F32).reshape(mq, _LANE) + mod(2, cols) * att[rows, cols]
                           + mod(5, cols) * (x1[rows, cols] + y))
                    dst[rows, cols] = res.astype(dst.dtype)

                _combine(_LEVEL, functools.partial(down, p), emit=emit)
            assert not terms
            out_copy(i, slot).start()

        with jax.named_scope('sc_s1'):
            _loop(0, n_blk, gate)
        with jax.named_scope('sc_s2'):
            _loop(0, n_blk, mix)
        cp_gate.wait()
        norms, terms = norm_jobs(nh * n_blk - 1, 1), term_jobs(0)
        mod_s[5] = jnp.concatenate(
            [_dot(silu_c, paced(pltpu.bitcast(wg_v[:, _cols(j)], _U32), norms[j::ND] + terms[j::ND]))
             for j in range(ND)], axis=1)
        with jax.named_scope('sc_s3'):
            _loop(0, n_blk, mlp)
        for i in (n_blk - 2, n_blk - 1):
            out_copy(i, i % 2).wait()

    def after_weights(wqkv, wo_s, pre_s, w1_v, w2_v, w3_v, w4_v, hb_s, n0_s):
        cps = [copy(w3_hbm, w3_v, sems.at[0]), copy(w4_hbm, w4_v, sems.at[1])]
        cps += [copy(src.bitcast(_U32).at[:, pl.ds(j * _LANE, _LANE)], dst.at[j],
                     sems.at[4 + n * ND + j])
                for n, (src, dst) in enumerate(((w1_hbm, w1_v), (w2_hbm, w2_v))) for j in range(ND)]
        _start([cp_x_tail] + cps)
        pl.run_scoped(
            functools.partial(recurrence, wqkv, wo_s, pre_s, hb_s, n0_s),
            pltpu.VMEM((M, D), _F32),
            pltpu.VMEM((2, seg_len - _PRE, D), _F32),
            pltpu.VMEM((L, H * _LANE), _F32),
            pltpu.VMEM((seg_len, D), _F32),
        )
        _wait(cps)

    def whole(w1_v, w2_v, w3_v, w4_v, hb_s, n0_s):
        def attention(wqkv, wo_s, pre_s):
            pl.run_scoped(
                functools.partial(load_weights, wqkv, wo_s, pre_s),
                pltpu.VMEM((D * H, _LANE), _BF16),
                pltpu.VMEM((n_seg, _PRE, D), _BF16),
                pltpu.VMEM((ND, n_seg * _PRE, _LANE), _F32),
                pltpu.VMEM((ND // 2, 7, n_seg * _PRE // 4, _LANE), _U32),
                pltpu.VMEM((3 * ND, D, _LANE), _BF16),
                pltpu.VMEM((2, ND, 8, _LANE), _F32),
                pltpu.SemaphoreType.DMA((ND,)),
                pltpu.SemaphoreType.DMA((3 * ND,)),
                pltpu.SemaphoreType.DMA((ND + 2,)),
            )
            after_weights(wqkv, wo_s, pre_s, w1_v, w2_v, w3_v, w4_v, hb_s, n0_s)

        pl.run_scoped(
            attention,
            pltpu.VMEM((3 * H, D // 2, _LANE), _U32),
            pltpu.VMEM((ND, H * _LANE // 2, _LANE), _U32),
            pltpu.VMEM((3 * H, n_seg * _PRE, _LANE), _F32),
        )
        pl.run_scoped(
            functools.partial(mixer, w1_v, w2_v, w3_v, w4_v, hb_s, n0_s),
            pltpu.VMEM((T, dq // 2, fq), _U32),
            pltpu.VMEM((T, fq // 2, dq), _U32),
            pltpu.VMEM((T, mq // 2, dq), _U32),
            pltpu.VMEM((T, mq // 2, fq), _U32),
            pltpu.VMEM((ND, S, _LANE), _F32),
            pltpu.VMEM((2, _TM // 2, D), _F32),
            pltpu.VMEM((D, D), _BF16),
            pltpu.VMEM((2, _TM, D), _BF16),
            pltpu.SemaphoreType.DMA((2,)),
            *[pltpu.VMEM((S + 2 * _HALO, _LANE), _F32) for _ in range(ND)],
        )

    pl.run_scoped(
        whole,
        pltpu.VMEM((ND, D // 2, _LANE), _U32),
        pltpu.VMEM((ND, D // 2, _LANE), _U32),
        pltpu.VMEM((D, F), _BF16),
        pltpu.VMEM((F, D), _BF16),
        pltpu.VMEM((S, D), _F32),
        pltpu.VMEM((S // 2, D), _U32),
    )


@functools.partial(jax.jit, static_argnames=("A_seg_len",))
def pallas_adaLN_cond__memory_aug_recurrent_mem_tr__mixer_s_mlp__prompt_kernel(
    A_x: jax.Array,
    A_mem0: jax.Array,
    A_Wq: jax.Array,
    A_Wk: jax.Array,
    A_Wv: jax.Array,
    A_Wo: jax.Array,
    A_seg_len: int,
    B_x: jax.Array,
    B_w1: jax.Array,
    B_w2: jax.Array,
    B_w3: jax.Array,
    B_w4: jax.Array,
    c: jax.Array,
    w_mod: jax.Array,
):
    del B_x
    batch, S, D = A_x.shape
    _, H, Dh = A_Wq.shape
    M = A_mem0.shape[1]
    seg_len = int(A_seg_len)
    assert batch == 1 and Dh == _LANE and S % _TM == 0 and _TM % seg_len == 0
    n_seg = S // seg_len

    vmem = pl.BlockSpec(memory_space=pltpu.VMEM)
    hbm = pl.BlockSpec(memory_space=pl.ANY)
    out = pl.pallas_call(
        _kernel,
        out_shape=jax.ShapeDtypeStruct((S, D), A_x.dtype),
        in_specs=[vmem, vmem] + [hbm] * 10,
        out_specs=hbm,
        scratch_shapes=[
            pltpu.VMEM((n_seg, seg_len, D), _BF16),
            pltpu.VMEM((S, D), _F32),
            pltpu.VMEM((6, 8, D), _F32),
            pltpu.VMEM((8, _LANE), _U32),
            pltpu.SemaphoreType.DMA((4 + 2 * D // _LANE,)),
        ],
        compiler_params=pltpu.CompilerParams(vmem_limit_bytes=126 * 1024 * 1024),
        name="adaln_rmt_mixer",
    )(
        A_mem0.reshape(M, D), c, A_x.reshape(n_seg, seg_len, D),
        A_Wq.reshape(D * H, Dh), A_Wk.reshape(D * H, Dh), A_Wv.reshape(D * H, Dh),
        A_Wo.reshape(H * Dh, D), B_w1, B_w2, B_w3, B_w4, w_mod,
    )
    return out.reshape(batch, S, D)
```

```python
import functools
import math

import jax
import jax.numpy as jnp
from jax import lax
import jax.experimental.pallas as pl
import jax.experimental.pallas.tpu as pltpu

_F32 = jnp.float32
_BF16 = jnp.bfloat16
_U32 = jnp.uint32
_LANE = 128
_EPS = 1e-05
_TM = 256
_LEVEL = 2
_UNROLL = 2
_HALO = 8
_PRE = 8
_G = 4


def _dot(a, b):
    return lax.dot_general(a, b, (((1,), (0,)), ((), ())), preferred_element_type=_F32)


def _dot_nt(a, b):
    return lax.dot_general(a, b, (((1,), (1,)), ((), ())), preferred_element_type=_F32)


def _layernorm(x):
    m = jnp.mean(x, axis=-1, keepdims=True)
    d = x - m
    v = jnp.mean(d * d, axis=-1, keepdims=True)
    return d * lax.rsqrt(v + _EPS)


def _gelu(x):
    c = math.sqrt(2.0 / math.pi)
    inner = x * (c + (c * 0.044715) * (x * x))
    hx = 0.5 * x
    return hx + hx * jnp.tanh(inner)


def _pack(x):
    return pltpu.bitcast(x.astype(_BF16), _U32)


def _unpacked(x):
    return pltpu.bitcast(x, _BF16)


def _low_half(w):
    return pltpu.bitcast(w << 16, _F32)


def _high_half(w):
    return pltpu.bitcast(w & jnp.uint32(0xFFFF0000), _F32)


def _quads(g):
    n = len(g) // 2
    return [[row[j * n:(j + 1) * n] for row in g[i * n:(i + 1) * n]]
            for i in range(2) for j in range(2)]


def _add(a, b):
    return [[x + y for x, y in zip(r, t)] for r, t in zip(a, b)]


def _sub(a, b):
    return [[x - y for x, y in zip(r, t)] for r, t in zip(a, b)]


def _lhs_terms(g):
    if len(g) == 1:
        return [g[0][0]]
    a11, a12, a21, a22 = _quads(g)
    terms = (_sub(a11, a22), _sub(a21, a22), a22, _sub(a21, a11), _sub(a22, a12), a11,
             _sub(a11, a12))
    return [v for t in terms for v in _lhs_terms(t)]


def _rhs_terms(g):
    if len(g) == 1:
        return [g[0][0]]
    b11, b12, b21, b22 = _quads(g)
    terms = (_sub(b11, b22), b11, _add(b21, b11), _add(b11, b12), _add(b21, b22), _add(b12, b22),
             b22)
    return [v for t in terms for v in _rhs_terms(t)]


def _combine(level, product, base=0, emit=None):
    if level == 0:
        return [[product(base)]]

    def m(i):
        return _combine(level - 1, product, base + i * 7 ** (level - 1))

    def done(qi, qj, g):
        if emit is None:
            return g
        n = len(g)
        return [[emit(qi * n + a, qj * n + b, g[a][b]) for b in range(n)] for a in range(n)]

    m1, m2 = m(1), m(2)
    c21 = done(1, 0, _add(m1, m2))
    m5 = m(5)
    c22 = _sub(m5, m1)
    m6 = m(6)
    c11 = _add(m2, m6)
    c12 = done(0, 1, _sub(m5, m6))
    m0 = m(0)
    c11, c22 = _add(c11, m0), _add(c22, m0)
    c22 = done(1, 1, _add(m(3), c22))
    c11 = done(0, 0, _sub(c11, m(4)))
    return [x + y for x, y in zip(c11, c12)] + [x + y for x, y in zip(c21, c22)]


def _aligned(start, size):
    return pl.ds(pl.multiple_of(start, size), size)


def _cols(j, n=_LANE):
    return slice(j * n, (j + 1) * n)


def _loop(lo, hi, fn):
    def body(i, carry):
        fn(i)
        return carry
    lax.fori_loop(lo, hi, body, 0)


def _start(cps):
    for cp in cps:
        cp.start()


def _wait(cps):
    for cp in cps:
        cp.wait()


def _kernel(mem0_hbm, c_hbm, x_hbm, wq_hbm, wk_hbm, wv_hbm, wo_hbm, w1_hbm, w2_hbm, w3_hbm,
            w4_hbm, wmod_hbm, out_hbm, c_ref, zero_s, mem0_ref, x_v, xm_s, mod_s, sems):
    n_seg, seg_len, D = x_v.shape
    S = n_seg * seg_len
    M = mem0_ref.shape[0]
    H = wo_hbm.shape[0] // _LANE
    F = w3_hbm.shape[1]
    L = M + seg_len
    ND = D // _LANE
    P = 2 ** _LEVEL
    T = 7 ** _LEVEL
    mq, dq, fq = _TM // P, D // P, F // P
    scale = float(_LANE) ** -0.5
    copy = pltpu.make_async_copy

    def mod(r, cols=slice(None)):
        return mod_s[r, 0:1, cols]

    x_head = 8
    cp_x_tail = copy(x_hbm.at[pl.ds(x_head, n_seg - x_head)],
                     x_v.at[pl.ds(x_head, n_seg - x_head)], sems.at[2])
    zero_s[...] = jnp.zeros(zero_s.shape, _U32)

    def paced(w, jobs):
        step = w.shape[0] // (_LANE // 2) // max(len(jobs), 1) * (_LANE // 2)
        parts = []
        for n, job in enumerate(jobs):
            tiles = [pltpu.bitcast(v, _U32)[r:r + 8, c:c + _LANE] for v in job()
                     for r in range(0, v.shape[0], 8) for c in range(0, v.shape[1], _LANE)]
            done = functools.reduce(jnp.bitwise_or, tiles) & zero_s[0:8, :]
            parts += [w[n * step:n * step + 8] | done, w[n * step + 8:(n + 1) * step]]
        if len(jobs) * step < w.shape[0]:
            parts.append(w[len(jobs) * step:])
        return _unpacked(jnp.concatenate(parts, axis=0))

    def load_weights(wqkv, wo_s, pre_s, stage, xq_v, nq_s, hq_s, wmod_v, moda_s, w_sems, m_sems,
                     o_sems):
        rows_c = _LANE * H
        words = stage.bitcast(_U32)
        w_hbm = (wq_hbm, wk_hbm, wv_hbm)

        def w_copy(t, j):
            return copy(w_hbm[t].at[_aligned(j * rows_c, rows_c), :],
                        stage.at[_aligned(j * rows_c, rows_c), :], w_sems.at[j])

        def m_copy(r, j):
            n = r % 3 * ND + j
            return copy(wmod_hbm.at[:, _aligned((r * ND + j) * _LANE, _LANE)], wmod_v.at[n],
                        m_sems.at[n])

        def modulate(j):
            hs = []
            for u in (2 * j, 2 * j + 1):
                shift = _dot(mod_s[6], wmod_v[u])
                gain = 1.0 + _dot(mod_s[6], wmod_v[ND + u])
                moda_s[0, u] = shift
                moda_s[1, u] = gain
                hs.append(nq_s[u] * gain[0:1] + shift[0:1])
            mh = hs[0].shape[0] // 2
            for n, v in enumerate(_lhs_terms([[h[_cols(a, mh)] for h in hs] for a in range(2)])):
                hq_s[j, n] = _pack(v)

        def absorb(t, j):
            src = words.at[_aligned(j * rows_c, rows_c), :]
            dst = wqkv.at[pl.ds(t * H, H), _aligned(j * _LANE, _LANE), :]
            acc = pre_s.at[pl.ds(t * H, H)]
            lhs = hq_s.at[j]
            mh = lhs.shape[1] * 2
            for hp in range(H // 2):
                w = src[pl.ds(hp, 2 * _LANE, stride=H // 2), :]
                pair = (_low_half(w), _high_half(w))
                for i in range(2):
                    dst[2 * hp + i] = _pack(pair[i])
                rhs = _rhs_terms([[v[_cols(u)] for v in pair] for u in range(2)])

                def emit(a, b, y):
                    old = acc[2 * hp + b, _cols(a, mh), :]
                    acc[2 * hp + b, _cols(a, mh), :] = y + jnp.where(j == 0, 0.0, old)

                _combine(1, lambda n: _dot(_unpacked(lhs[n]), rhs[n].astype(_BF16)), emit=emit)

        cp_xq = copy(x_hbm.at[:, pl.ds(seg_len - _PRE, _PRE), :], xq_v, o_sems.at[ND])
        cp_x_head = copy(x_hbm.at[pl.ds(0, x_head)], x_v.at[pl.ds(0, x_head)], o_sems.at[ND + 1])
        cp_wo = [copy(wo_hbm.bitcast(_U32).at[:, pl.ds(n * _LANE, _LANE)], wo_s.at[n], o_sems.at[n])
                 for n in range(ND)]
        cp_mb = [m_copy(r, j) for r in range(2, 5) for j in range(ND)]

        mu = [[m_copy(0, j), m_copy(1, j)] for j in range(ND)]
        qu, ku, vu = ([[w_copy(t, j)] for j in range(ND)] for t in range(3))
        m2, q2, k2, v2 = ([u[2 * j] + u[2 * j + 1] for j in range(ND // 2)] for u in (mu, qu, ku, vu))
        plan = [q2[1] + m2[2], q2[2] + m2[3] + cp_wo[0:1], q2[3] + k2[0],
                k2[1] + k2[2], k2[3] + cp_wo[1:4], v2[0] + cp_wo[4:6], v2[1] + cp_wo[6:],
                v2[2] + cp_mb[:ND], v2[3] + cp_mb[ND:2 * ND], cp_mb[2 * ND:] + [cp_x_head]]

        small = [copy(c_hbm, c_ref, sems.at[0]), copy(mem0_hbm, mem0_ref, sems.at[1])]
        _start(small + [cp_xq] + m2[0] + q2[0])
        _wait(small)
        cf = c_ref[...].astype(_F32)
        mod_s[6] = jnp.broadcast_to(cf * jax.nn.sigmoid(cf), (8, D))
        cp_xq.wait()
        nq = _layernorm(xq_v[...].astype(_F32).reshape(n_seg * _PRE, D))
        for j in range(ND):
            nq_s[j] = nq[:, _cols(j)]
        _wait(m2[0])
        _start(m2[1])

        def step(i):
            t, j = i // (ND // 2), i % (ND // 2)

            @pl.when(t == 0)
            def _():
                pl.when(j > 0)(functools.partial(
                    _wait, [m_copy(r, 2 * j + u) for r in range(2) for u in range(2)]))
                modulate(j)

            for tt in range(3):
                pl.when(t == tt)(functools.partial(_wait, [w_copy(tt, 2 * j), w_copy(tt, 2 * j + 1)]))
            for n, cps in enumerate(plan):
                pl.when(i == n)(functools.partial(_start, cps))
            absorb(t, j)
        _loop(0, 3 * ND // 2, step)

        _wait(cp_wo + [cp_x_head] + cp_mb)
        for r in range(2):
            mod_s[r] = jnp.concatenate([moda_s[r, j] for j in range(ND)], axis=1)
        for r in range(2, 5):
            w = jnp.concatenate([wmod_v[r % 3 * ND + j] for j in range(ND)], axis=1)
            y = _dot(mod_s[6], w)
            mod_s[r] = 1.0 + y if r == 4 else y

    def recurrence(wqkv, wo_s, pre_s, hb_s, n0_s, mem_s, seg_s, o_s, prev_s):
        def seg_input(s, r):
            h = _layernorm(x_v[s, r:r + 8, :].astype(_F32)) * mod(1) + mod(0)
            seg_s[r:r + 8, :] = h
            return [h]

        def mixer_input(s, r):
            xm = x_v[s, r:r + 16, :].astype(_F32) + mod(2) * prev_s[r:r + 16, :]
            xm_s[_aligned(s * seg_len + r, 16), :] = xm
            hb = _layernorm(xm) * mod(4) + mod(3)
            hb_s[_aligned(s * seg_len + r, 16), :] = hb
            n0 = _pack(_layernorm(hb))
            n0_s[_aligned((s * seg_len + r) // 2, 8), :] = n0
            return [n0]

        def seg_jobs(s):
            return [functools.partial(seg_input, s, r) for r in range(0, seg_len - _PRE, 8)]

        def mixer_jobs(s):
            return [functools.partial(mixer_input, s, r) for r in range(0, seg_len, 16)]

        mem_s[...] = mem0_ref[...].astype(_F32)
        for job in seg_jobs(0):
            job()
        prev_s[...] = jnp.zeros(prev_s.shape, _F32)

        row = lax.broadcasted_iota(jnp.int32, (L, L), 0)
        col = lax.broadcasted_iota(jnp.int32, (L, L), 1)
        mask = (row < M) | (row >= col)
        half = D // 2

        def seg_step(s, mem):
            jobs = mixer_jobs(jnp.maximum(s - 1, 0)) + seg_jobs(jnp.minimum(s + 1, n_seg - 1))
            lhs = [jnp.concatenate([mem[i], seg_s[:, _cols(i, half)]], axis=0).astype(_BF16)
                   for i in range(2)]
            pre = pre_s.at[:, _aligned(s * _PRE, _PRE), :]

            def proj_part(ids, parts):
                rows = slice(parts[0] * half // 2, (parts[-1] + 1) * half // 2)
                due = {ids[-1]: [jobs.pop(0)]} if jobs and ids[-1] >= 2 * H + _G else {}
                w = jnp.concatenate([paced(wqkv[n, rows, :], due.get(n, [])) for n in ids], axis=1)
                return _dot(jnp.concatenate([lhs[i] for i in parts], axis=1), w)

            def proj(ids, y=None):
                y = proj_part(ids, (0, 1)) if y is None else proj_part(ids, (1,)) + y
                return [jnp.concatenate([y[:, _cols(i)], pre[n]], axis=0) for i, n in enumerate(ids)]

            def weights(q, k):
                sc = jnp.where(mask, _dot_nt(q, k.astype(_BF16)) * scale, -1000000000.0)
                e = jnp.exp(sc - jnp.max(sc, axis=-1, keepdims=True))
                return e / jnp.sum(e, axis=-1, keepdims=True)

            def mix(h0, ws, vs):
                for i, (p, v) in enumerate(zip(ws, vs)):
                    o_s[:, _cols(h0 + i)] = _dot(p, v.astype(_BF16))

            def out_proj(h0, h1, part):
                ks = slice(h0 * _LANE, h1 * _LANE)
                cols = range(part * ND // 2, (part + 1) * ND // 2)
                w = [_unpacked(wo_s[n, h0 * _LANE // 2:h1 * _LANE // 2, :]) for n in cols]
                return _dot(o_s[:, ks], jnp.concatenate(w, axis=1))

            pend = None
            for h in range(0, H, _G):
                ids = [t * H + h + i for t in range(3) for i in range(_G)]
                if pend is None:
                    qkv = proj(ids[:2 * _G], proj_part(ids[:2 * _G], (0,))) + proj(ids[2 * _G:])
                else:
                    qkv = proj(ids)
                    mix(*pend)
                pend = (h, [weights(q, k) for q, k in zip(qkv[:_G], qkv[_G:2 * _G])], qkv[2 * _G:])
            y0 = out_proj(0, H - _G, 0)
            mix(*pend)
            y1 = out_proj(0, 2 * _G, 1)
            y0 = out_proj(H - _G, H, 0) + y0
            y1 = out_proj(2 * _G, H, 1) + y1
            assert not jobs
            for i, y in enumerate((y0, y1)):
                prev_s[:, _cols(i, half)] = y[M:L]
            return y0[0:M], y1[0:M]

        def seg_steps(i):
            pl.when(i == x_head // _UNROLL - 1)(cp_x_tail.wait)
            mem = (mem_s[:, 0:half], mem_s[:, half:D])
            for u in range(_UNROLL):
                mem = seg_step(i * _UNROLL + u, mem)
            mem_s[:, 0:half] = mem[0]
            mem_s[:, half:D] = mem[1]

        _loop(0, n_seg // _UNROLL, seg_steps)
        for job in mixer_jobs(n_seg - 1):
            job()

    def mixer(w1_v, w2_v, w3_v, w4_v, hb_s, n0_s, t3_s, t4_s, a1_s, a2_s, n1_s, last_s, wg_v,
              out_s, out_sems, *g_s):
        n_blk = S // _TM
        shifts = [(-1, 1, -2, 2)[j * _LANE * 4 // D] for j in range(ND)]
        cp_gate = copy(wmod_hbm.at[:, pl.ds(5 * D, D)], wg_v, sems.at[3])
        cp_gate.start()
        last_s[1] = jnp.zeros(last_s.shape[1:], _F32)
        for g in g_s:
            g[_HALO:2 * _HALO, :] = jnp.zeros((_HALO, _LANE), _F32)
            g[S:S + _HALO, :] = jnp.zeros((_HALO, _LANE), _F32)

        def block(ref, i, n=_TM):
            return ref.at[_aligned(i * n, n), :]

        def weight_terms(src, dst, i, r, j):
            nr, nc = src.shape[1] // P, src.shape[0] // P
            n = nr // n_blk
            dst = dst.at[:, pl.ds(pl.multiple_of(i * n, 8), n), :]
            w = [[src[b * nc + j, _aligned(a * nr + i * n + r, 8), :] for b in range(P)]
                 for a in range(P)]
            lo = _rhs_terms([[_low_half(v) for v in row] for row in w])
            hi = _rhs_terms([[_high_half(v) for v in row] for row in w])
            out = [pltpu.pack_elementwise(list(pair), packed_dtype=_BF16) for pair in zip(lo, hi)]
            for t, v in enumerate(out):
                dst[t, r:r + 8, _cols(j)] = v
            return out

        def weight_jobs(src, dst, i):
            return [functools.partial(weight_terms, src, dst, i, r, j)
                    for r in range(0, src.shape[1] // P // n_blk, 8)
                    for j in range(src.shape[0] // P)]

        def spread(jobs):
            cut = [j * len(jobs) // (ND - 1) for j in range(ND)]
            return [[]] + [jobs[cut[j]:cut[j + 1]] for j in range(ND - 1)]

        def gate(i):
            n0 = _unpacked(block(n0_s, i, _TM // 2)[...])
            for j, (g, off, jobs) in enumerate(zip(g_s, shifts, spread(weight_jobs(w3_v, t3_s, i)))):
                win = g.at[pl.ds(pl.multiple_of(i * _TM, _TM), _TM + 2 * _HALO), :]
                w = paced(w1_v[j], jobs)
                win[_HALO - off:_HALO - off + _TM, :] = _gelu(_dot(n0, w))

        nh = 2
        th = _TM // nh

        def mlp_norm(k, buf, r):
            n1 = _layernorm(last_s[buf, r:r + 16, :])
            dst = n1_s.at[:, _aligned(k * th, th), :]
            for j in range(ND):
                dst[j, r:r + 16, :] = n1[:, _cols(j)]
            return [n1]

        def norm_jobs(k, buf):
            return [functools.partial(mlp_norm, k, buf, r) for r in range(0, th, 16)]

        def mix(i):
            terms = weight_jobs(w4_v, t4_s, i)
            for u in range(nh):
                x1 = block(hb_s, i).at[u * th:(u + 1) * th, :]
                rows = pl.ds(pl.multiple_of(i * _TM + u * th + _HALO, _HALO), th)
                shifted = jnp.concatenate([g[rows, :] for g in g_s], axis=1).astype(_BF16)
                due = zip(spread(norm_jobs(jnp.maximum(nh * i + u - 1, 0), 1 - u % 2)),
                          spread(terms[u::nh]))
                for j, (norms, jobs) in enumerate(due):
                    w = paced(w2_v[j], jobs + norms)
                    y = _dot(shifted, w) + x1[:, _cols(j)]
                    x1[:, _cols(j)] = y
                    last_s[u % 2, :, _cols(j)] = y

        def mlp_terms(i, r, col):
            n1 = n1_s.at[:, _aligned(i * _TM, _TM), :]
            even, odd = (_lhs_terms(
                [[n1[(b * dq + col) // _LANE, pl.ds(a * mq + r + u, 8, stride=2), :]
                  for b in range(P)] for a in range(P)]) for u in range(2))
            out = [pltpu.pack_elementwise(list(pair), packed_dtype=_BF16) for pair in zip(even, odd)]
            for t, v in enumerate(out):
                a1_s[t, r // 2:r // 2 + 8, col:col + _LANE] = v
            return out

        def term_jobs(i):
            return [functools.partial(mlp_terms, i, r, col)
                    for r in range(0, mq, 16) for col in range(0, dq, _LANE)]

        def products(a_ref, w_ref, jobs, every):
            count = [0]

            def product(p, t):
                count[0] += 1
                due = [jobs.pop(0)] if jobs and count[0] % every == 0 else []
                return _dot(_unpacked(a_ref[t]), paced(w_ref[t, :, _cols(p)], due))
            return product

        def out_copy(i, slot):
            return copy(out_s.at[slot], block(out_hbm, i), out_sems.at[slot])

        def mlp(i):
            slot = i % 2

            @pl.when(i >= 2)
            def _():
                out_copy(jnp.maximum(i - 2, 0), slot).wait()

            terms = term_jobs(jnp.minimum(i + 1, n_blk - 1))
            up, down = products(a1_s, t3_s, [], 1), products(a2_s, t4_s, terms, 10)
            for p in range(fq // _LANE):
                g = _combine(_LEVEL, functools.partial(up, p), emit=lambda a, b, y: _gelu(y))
                for t, v in enumerate(_lhs_terms(g)):
                    a2_s[t, :, _cols(p)] = _pack(v)

            dst, xm, x1 = out_s.at[slot], block(xm_s, i), block(hb_s, i)
            for p in range(dq // _LANE):
                def emit(a, b, y):
                    rows, cols = slice(a * mq, (a + 1) * mq), _cols(b * (dq // _LANE) + p)
                    res = xm[rows, cols] + mod(5, cols) * (x1[rows, cols] + y)
                    dst[rows, cols] = res.astype(dst.dtype)

                _combine(_LEVEL, functools.partial(down, p), emit=emit)
            assert not terms
            out_copy(i, slot).start()

        _loop(0, n_blk, gate)
        _loop(0, n_blk, mix)
        cp_gate.wait()
        norms, terms = norm_jobs(nh * n_blk - 1, 1), term_jobs(0)
        mod_s[5] = jnp.concatenate(
            [_dot(mod_s[6], paced(pltpu.bitcast(wg_v[:, _cols(j)], _U32), norms[j::ND] + terms[j::ND]))
             for j in range(ND)], axis=1)
        _loop(0, n_blk, mlp)
        for i in (n_blk - 2, n_blk - 1):
            out_copy(i, i % 2).wait()

    def after_weights(wqkv, wo_s, pre_s, w1_v, w2_v, w3_v, w4_v, hb_s, n0_s):
        slabs = [(src, dst, j) for src, dst in ((w1_hbm, w1_v), (w2_hbm, w2_v), (w3_hbm, w3_v),
                                               (w4_hbm, w4_v)) for j in range(dst.shape[0])]
        cps = [copy(src.bitcast(_U32).at[:, pl.ds(j * _LANE, _LANE)], dst.at[j], sems.at[4 + n])
               for n, (src, dst, j) in enumerate(slabs)]
        _start([cp_x_tail] + cps)
        pl.run_scoped(
            functools.partial(recurrence, wqkv, wo_s, pre_s, hb_s, n0_s),
            pltpu.VMEM((M, D), _F32),
            pltpu.VMEM((seg_len - _PRE, D), _F32),
            pltpu.VMEM((L, H * _LANE), _F32),
            pltpu.VMEM((seg_len, D), _F32),
        )
        _wait(cps)

    def whole(w1_v, w2_v, w3_v, w4_v, hb_s, n0_s):
        def attention(wqkv, wo_s, pre_s):
            pl.run_scoped(
                functools.partial(load_weights, wqkv, wo_s, pre_s),
                pltpu.VMEM((D * H, _LANE), _BF16),
                pltpu.VMEM((n_seg, _PRE, D), _BF16),
                pltpu.VMEM((ND, n_seg * _PRE, _LANE), _F32),
                pltpu.VMEM((ND // 2, 7, n_seg * _PRE // 4, _LANE), _U32),
                pltpu.VMEM((3 * ND, D, _LANE), _BF16),
                pltpu.VMEM((2, ND, 8, _LANE), _F32),
                pltpu.SemaphoreType.DMA((ND,)),
                pltpu.SemaphoreType.DMA((3 * ND,)),
                pltpu.SemaphoreType.DMA((ND + 2,)),
            )
            after_weights(wqkv, wo_s, pre_s, w1_v, w2_v, w3_v, w4_v, hb_s, n0_s)

        pl.run_scoped(
            attention,
            pltpu.VMEM((3 * H, D // 2, _LANE), _U32),
            pltpu.VMEM((ND, H * _LANE // 2, _LANE), _U32),
            pltpu.VMEM((3 * H, n_seg * _PRE, _LANE), _F32),
        )
        pl.run_scoped(
            functools.partial(mixer, w1_v, w2_v, w3_v, w4_v, hb_s, n0_s),
            pltpu.VMEM((T, dq // 2, fq), _U32),
            pltpu.VMEM((T, fq // 2, dq), _U32),
            pltpu.VMEM((T, mq // 2, dq), _U32),
            pltpu.VMEM((T, mq // 2, fq), _U32),
            pltpu.VMEM((ND, S, _LANE), _F32),
            pltpu.VMEM((2, _TM // 2, D), _F32),
            pltpu.VMEM((D, D), _BF16),
            pltpu.VMEM((2, _TM, D), _BF16),
            pltpu.SemaphoreType.DMA((2,)),
            *[pltpu.VMEM((S + 4 * _HALO, _LANE), _F32) for _ in range(ND)],
        )

    pl.run_scoped(
        whole,
        pltpu.VMEM((ND, D // 2, _LANE), _U32),
        pltpu.VMEM((ND, D // 2, _LANE), _U32),
        pltpu.VMEM((F // _LANE, D // 2, _LANE), _U32),
        pltpu.VMEM((ND, F // 2, _LANE), _U32),
        pltpu.VMEM((S, D), _F32),
        pltpu.VMEM((S // 2, D), _U32),
    )


@functools.partial(jax.jit, static_argnames=("A_seg_len",))
def pallas_adaLN_cond__memory_aug_recurrent_mem_tr__mixer_s_mlp__prompt_kernel(
    A_x: jax.Array,
    A_mem0: jax.Array,
    A_Wq: jax.Array,
    A_Wk: jax.Array,
    A_Wv: jax.Array,
    A_Wo: jax.Array,
    A_seg_len: int,
    B_x: jax.Array,
    B_w1: jax.Array,
    B_w2: jax.Array,
    B_w3: jax.Array,
    B_w4: jax.Array,
    c: jax.Array,
    w_mod: jax.Array,
):
    del B_x
    batch, S, D = A_x.shape
    _, H, Dh = A_Wq.shape
    M = A_mem0.shape[1]
    seg_len = int(A_seg_len)
    assert (batch, S, D, Dh, M, seg_len, B_w3.shape[1]) == (1, 2048, 1024, _LANE, 8, 32, 3584)
    n_seg = S // seg_len

    hbm = pl.BlockSpec(memory_space=pl.ANY)
    out = pl.pallas_call(
        _kernel,
        out_shape=jax.ShapeDtypeStruct((S, D), A_x.dtype),
        in_specs=[hbm] * 12,
        out_specs=hbm,
        scratch_shapes=[
            pltpu.VMEM(c.shape, _BF16),
            pltpu.VMEM((16, _LANE), _U32),
            pltpu.VMEM((M, D), _BF16),
            pltpu.VMEM((n_seg, seg_len, D), _BF16),
            pltpu.VMEM((S, D), _F32),
            pltpu.VMEM((7, 8, D), _F32),
            pltpu.SemaphoreType.DMA((4 + (3 * D + B_w3.shape[1]) // _LANE,)),
        ],
        compiler_params=pltpu.CompilerParams(vmem_limit_bytes=126 * 1024 * 1024),
        name="adaln_rmt_mixer",
    )(
        A_mem0.reshape(M, D), c, A_x.reshape(n_seg, seg_len, D),
        A_Wq.reshape(D * H, Dh), A_Wk.reshape(D * H, Dh), A_Wv.reshape(D * H, Dh),
        A_Wo.reshape(H * Dh, D), B_w1, B_w2, B_w3, B_w4, w_mod,
    )
    return out.reshape(batch, S, D)
```

```python
import functools
import math

import jax
import jax.numpy as jnp
from jax import lax
import jax.experimental.pallas as pl
import jax.experimental.pallas.tpu as pltpu

_F32 = jnp.float32
_BF16 = jnp.bfloat16
_U32 = jnp.uint32
_LANE = 128
_EPS = 1e-05
_TM = 256
_LEVEL = 2
_UNROLL = 2
_HALO = 8
_PRE = 8
_G = 4


def _dot(a, b):
    return lax.dot_general(a, b, (((1,), (0,)), ((), ())), preferred_element_type=_F32)


def _dot_nt(a, b):
    return lax.dot_general(a, b, (((1,), (1,)), ((), ())), preferred_element_type=_F32)


def _layernorm(x):
    m = jnp.mean(x, axis=-1, keepdims=True)
    d = x - m
    v = jnp.mean(d * d, axis=-1, keepdims=True)
    return d * lax.rsqrt(v + _EPS)


def _gelu(x):
    c = math.sqrt(2.0 / math.pi)
    inner = x * (c + (c * 0.044715) * (x * x))
    hx = 0.5 * x
    return hx + hx * jnp.tanh(inner)


def _pack(x):
    return pltpu.bitcast(x.astype(_BF16), _U32)


def _unpacked(x):
    return pltpu.bitcast(x, _BF16)


def _low_half(w):
    return pltpu.bitcast(w << 16, _F32)


def _high_half(w):
    return pltpu.bitcast(w & jnp.uint32(0xFFFF0000), _F32)


def _quads(g):
    n = len(g) // 2
    return [[row[j * n:(j + 1) * n] for row in g[i * n:(i + 1) * n]]
            for i in range(2) for j in range(2)]


def _add(a, b):
    return [[x + y for x, y in zip(r, t)] for r, t in zip(a, b)]


def _sub(a, b):
    return [[x - y for x, y in zip(r, t)] for r, t in zip(a, b)]


def _lhs_terms(g):
    if len(g) == 1:
        return [g[0][0]]
    a11, a12, a21, a22 = _quads(g)
    terms = (_sub(a11, a22), _sub(a21, a22), a22, _sub(a21, a11), _sub(a22, a12), a11,
             _sub(a11, a12))
    return [v for t in terms for v in _lhs_terms(t)]


def _rhs_terms(g):
    if len(g) == 1:
        return [g[0][0]]
    b11, b12, b21, b22 = _quads(g)
    terms = (_sub(b11, b22), b11, _add(b21, b11), _add(b11, b12), _add(b21, b22), _add(b12, b22),
             b22)
    return [v for t in terms for v in _rhs_terms(t)]


def _combine(level, product, base=0, emit=None):
    if level == 0:
        return [[product(base)]]

    def m(i):
        return _combine(level - 1, product, base + i * 7 ** (level - 1))

    def done(qi, qj, g):
        if emit is None:
            return g
        n = len(g)
        return [[emit(qi * n + a, qj * n + b, g[a][b]) for b in range(n)] for a in range(n)]

    m1, m2 = m(1), m(2)
    c21 = done(1, 0, _add(m1, m2))
    m5 = m(5)
    c22 = _sub(m5, m1)
    m6 = m(6)
    c11 = _add(m2, m6)
    c12 = done(0, 1, _sub(m5, m6))
    m0 = m(0)
    c11, c22 = _add(c11, m0), _add(c22, m0)
    c22 = done(1, 1, _add(m(3), c22))
    c11 = done(0, 0, _sub(c11, m(4)))
    return [x + y for x, y in zip(c11, c12)] + [x + y for x, y in zip(c21, c22)]


def _aligned(start, size):
    return pl.ds(pl.multiple_of(start, size), size)


def _cols(j, n=_LANE):
    return slice(j * n, (j + 1) * n)


def _loop(lo, hi, fn):
    def body(i, carry):
        fn(i)
        return carry
    lax.fori_loop(lo, hi, body, 0)


def _start(cps):
    for cp in cps:
        cp.start()


def _wait(cps):
    for cp in cps:
        cp.wait()


def _kernel(mem0_hbm, c_hbm, x_hbm, wq_hbm, wk_hbm, wv_hbm, wo_hbm, w1_hbm, w2_hbm, w3_hbm,
            w4_hbm, wmod_hbm, out_hbm, c_ref, zero_s, mem0_ref, x_v, xm_s, mod_s, sems):
    n_seg, seg_len, D = x_v.shape
    S = n_seg * seg_len
    M = mem0_ref.shape[0]
    H = wo_hbm.shape[0] // _LANE
    F = w3_hbm.shape[1]
    L = M + seg_len
    ND = D // _LANE
    P = 2 ** _LEVEL
    T = 7 ** _LEVEL
    mq, dq, fq = _TM // P, D // P, F // P
    scale = float(_LANE) ** -0.5
    copy = pltpu.make_async_copy

    def mod(r, cols=slice(None)):
        return mod_s[r, 0:1, cols]

    x_head = 8
    cp_x_tail = copy(x_hbm.at[pl.ds(x_head, n_seg - x_head)],
                     x_v.at[pl.ds(x_head, n_seg - x_head)], sems.at[2])
    zero_s[...] = jnp.zeros(zero_s.shape, _U32)

    def paced(w, jobs):
        step = w.shape[0] // (_LANE // 2) // max(len(jobs), 1) * (_LANE // 2)
        parts = []
        for n, job in enumerate(jobs):
            tiles = [pltpu.bitcast(v, _U32)[r:r + 8, c:c + _LANE] for v in job()
                     for r in range(0, v.shape[0], 8) for c in range(0, v.shape[1], _LANE)]
            done = functools.reduce(jnp.bitwise_or, tiles) & zero_s[0:8, :]
            parts += [w[n * step:n * step + 8] | done, w[n * step + 8:(n + 1) * step]]
        if len(jobs) * step < w.shape[0]:
            parts.append(w[len(jobs) * step:])
        return _unpacked(jnp.concatenate(parts, axis=0))

    def load_weights(wqkv, wo_s, pre_s, stage, xq_v, nq_s, hq_s, wmod_v, moda_s, w_sems, m_sems,
                     o_sems):
        rows_c = _LANE * H
        words = stage.bitcast(_U32)
        w_hbm = (wq_hbm, wk_hbm, wv_hbm)

        def w_copy(t, j):
            return copy(w_hbm[t].at[_aligned(j * rows_c, rows_c), :],
                        stage.at[_aligned(j * rows_c, rows_c), :], w_sems.at[j])

        def m_copy(r, j):
            n = r % 3 * ND + j
            return copy(wmod_hbm.at[:, _aligned((r * ND + j) * _LANE, _LANE)], wmod_v.at[n],
                        m_sems.at[n])

        def modulate(j):
            hs = []
            for u in (2 * j, 2 * j + 1):
                shift = _dot(mod_s[6], wmod_v[u])
                gain = 1.0 + _dot(mod_s[6], wmod_v[ND + u])
                moda_s[0, u] = shift
                moda_s[1, u] = gain
                hs.append(nq_s[u] * gain[0:1] + shift[0:1])
            mh = hs[0].shape[0] // 2
            for n, v in enumerate(_lhs_terms([[h[_cols(a, mh)] for h in hs] for a in range(2)])):
                hq_s[j, n] = _pack(v)

        def absorb(t, j):
            src = words.at[_aligned(j * rows_c, rows_c), :]
            dst = wqkv.at[pl.ds(t * H, H), _aligned(j * _LANE, _LANE), :]
            acc = pre_s.at[pl.ds(t * H, H)]
            lhs = hq_s.at[j]
            mh = lhs.shape[1] * 2
            for hp in range(H // 2):
                w = src[pl.ds(hp, 2 * _LANE, stride=H // 2), :]
                pair = (_low_half(w), _high_half(w))
                for i in range(2):
                    dst[2 * hp + i] = _pack(pair[i])
                rhs = _rhs_terms([[v[_cols(u)] for v in pair] for u in range(2)])

                def emit(a, b, y):
                    old = acc[2 * hp + b, _cols(a, mh), :]
                    acc[2 * hp + b, _cols(a, mh), :] = y + jnp.where(j == 0, 0.0, old)

                _combine(1, lambda n: _dot(_unpacked(lhs[n]), rhs[n].astype(_BF16)), emit=emit)

        cp_xq = copy(x_hbm.at[:, pl.ds(seg_len - _PRE, _PRE), :], xq_v, o_sems.at[ND])
        cp_x_head = copy(x_hbm.at[pl.ds(0, x_head)], x_v.at[pl.ds(0, x_head)], o_sems.at[ND + 1])
        cp_wo = [copy(wo_hbm.bitcast(_U32).at[:, pl.ds(n * _LANE, _LANE)], wo_s.at[n], o_sems.at[n])
                 for n in range(ND)]
        cp_mb = [m_copy(r, j) for r in range(2, 5) for j in range(ND)]

        mu = [[m_copy(0, j), m_copy(1, j)] for j in range(ND)]
        qu, ku, vu = ([[w_copy(t, j)] for j in range(ND)] for t in range(3))
        m2, q2, k2, v2 = ([u[2 * j] + u[2 * j + 1] for j in range(ND // 2)] for u in (mu, qu, ku, vu))
        plan = [q2[1] + m2[2], q2[2] + m2[3] + cp_wo[0:1], q2[3] + k2[0],
                k2[1] + k2[2], k2[3] + cp_wo[1:4], v2[0] + cp_wo[4:6], v2[1] + cp_wo[6:],
                v2[2] + cp_mb[:ND], v2[3] + cp_mb[ND:2 * ND], cp_mb[2 * ND:] + [cp_x_head]]

        small = [copy(c_hbm, c_ref, sems.at[0]), copy(mem0_hbm, mem0_ref, sems.at[1])]
        _start(small + [cp_xq] + m2[0] + q2[0])
        _wait(small)
        cf = c_ref[...].astype(_F32)
        mod_s[6] = jnp.broadcast_to(cf * jax.nn.sigmoid(cf), (8, D))
        cp_xq.wait()
        nq = _layernorm(xq_v[...].astype(_F32).reshape(n_seg * _PRE, D))
        for j in range(ND):
            nq_s[j] = nq[:, _cols(j)]
        _wait(m2[0])
        _start(m2[1])

        def step(i):
            t, j = i // (ND // 2), i % (ND // 2)

            @pl.when(t == 0)
            def _():
                pl.when(j > 0)(functools.partial(
                    _wait, [m_copy(r, 2 * j + u) for r in range(2) for u in range(2)]))
                modulate(j)

            for tt in range(3):
                pl.when(t == tt)(functools.partial(_wait, [w_copy(tt, 2 * j), w_copy(tt, 2 * j + 1)]))
            for n, cps in enumerate(plan):
                pl.when(i == n)(functools.partial(_start, cps))
            absorb(t, j)
        _loop(0, 3 * ND // 2, step)

        _wait(cp_wo + [cp_x_head] + cp_mb)
        for r in range(2):
            mod_s[r] = jnp.concatenate([moda_s[r, j] for j in range(ND)], axis=1)
        for r in range(2, 5):
            w = jnp.concatenate([wmod_v[r % 3 * ND + j] for j in range(ND)], axis=1)
            y = _dot(mod_s[6], w)
            mod_s[r] = 1.0 + y if r == 4 else y

    def recurrence(wqkv, wo_s, pre_s, hb_s, n0_s, mem_s, seg_s, o_s, prev_s):
        def seg_input(s, r):
            h = _layernorm(x_v[s, r:r + 8, :].astype(_F32)) * mod(1) + mod(0)
            seg_s[r:r + 8, :] = h
            return [h]

        def mixer_input(s, r):
            hb = _layernorm(prev_s[r:r + 16, :]) * mod(4) + mod(3)
            hb_s[_aligned(s * seg_len + r, 16), :] = hb
            n0 = _pack(_layernorm(hb))
            n0_s[_aligned((s * seg_len + r) // 2, 8), :] = n0
            return [n0]

        def seg_jobs(s):
            return [functools.partial(seg_input, s, r) for r in range(0, seg_len - _PRE, 8)]

        def mixer_jobs(s):
            return [functools.partial(mixer_input, s, r) for r in range(0, seg_len, 16)]

        mem_s[...] = mem0_ref[...].astype(_F32)
        for job in seg_jobs(0):
            job()
        prev_s[...] = jnp.zeros(prev_s.shape, _F32)

        row = lax.broadcasted_iota(jnp.int32, (L, L), 0)
        col = lax.broadcasted_iota(jnp.int32, (L, L), 1)
        mask = (row < M) | (row >= col)
        half = D // 2

        def seg_step(s, mem):
            jobs = mixer_jobs(jnp.maximum(s - 1, 0)) + seg_jobs(jnp.minimum(s + 1, n_seg - 1))
            lhs = [jnp.concatenate([mem[i], seg_s[:, _cols(i, half)]], axis=0).astype(_BF16)
                   for i in range(2)]
            pre = pre_s.at[:, _aligned(s * _PRE, _PRE), :]

            def proj_part(ids, parts):
                rows = slice(parts[0] * half // 2, (parts[-1] + 1) * half // 2)
                due = {ids[-1]: [jobs.pop(0)]} if jobs and ids[-1] >= 2 * H + _G else {}
                w = jnp.concatenate([paced(wqkv[n, rows, :], due.get(n, [])) for n in ids], axis=1)
                return _dot(jnp.concatenate([lhs[i] for i in parts], axis=1), w)

            def proj(ids, y=None):
                y = proj_part(ids, (0, 1)) if y is None else proj_part(ids, (1,)) + y
                return [jnp.concatenate([y[:, _cols(i)], pre[n]], axis=0) for i, n in enumerate(ids)]

            def weights(q, k):
                sc = jnp.where(mask, _dot_nt(q, k.astype(_BF16)) * scale, -1000000000.0)
                e = jnp.exp(sc - jnp.max(sc, axis=-1, keepdims=True))
                return e / jnp.sum(e, axis=-1, keepdims=True)

            def mix(h0, ws, vs):
                for i, (p, v) in enumerate(zip(ws, vs)):
                    o_s[:, _cols(h0 + i)] = _dot(p, v.astype(_BF16))

            def out_proj(h0, h1, part):
                ks = slice(h0 * _LANE, h1 * _LANE)
                cols = range(part * ND // 2, (part + 1) * ND // 2)
                w = [_unpacked(wo_s[n, h0 * _LANE // 2:h1 * _LANE // 2, :]) for n in cols]
                return _dot(o_s[:, ks], jnp.concatenate(w, axis=1))

            pend = None
            for h in range(0, H, _G):
                ids = [t * H + h + i for t in range(3) for i in range(_G)]
                if pend is None:
                    qkv = proj(ids[:2 * _G], proj_part(ids[:2 * _G], (0,))) + proj(ids[2 * _G:])
                else:
                    qkv = proj(ids)
                    mix(*pend)
                pend = (h, [weights(q, k) for q, k in zip(qkv[:_G], qkv[_G:2 * _G])], qkv[2 * _G:])
            y0 = out_proj(0, H - _G, 0)
            mix(*pend)
            y1 = out_proj(0, 2 * _G, 1)
            y0 = out_proj(H - _G, H, 0) + y0
            y1 = out_proj(2 * _G, H, 1) + y1
            assert not jobs
            for i, y in enumerate((y0, y1)):
                cols = _cols(i, half)
                xm = x_v[s, :, cols].astype(_F32) + mod(2, cols) * y[M:L]
                xm_s[_aligned(s * seg_len, seg_len), cols] = xm
                prev_s[:, cols] = xm
            return y0[0:M], y1[0:M]

        def seg_steps(i):
            pl.when(i == x_head // _UNROLL - 1)(cp_x_tail.wait)
            mem = (mem_s[:, 0:half], mem_s[:, half:D])
            for u in range(_UNROLL):
                mem = seg_step(i * _UNROLL + u, mem)
            mem_s[:, 0:half] = mem[0]
            mem_s[:, half:D] = mem[1]

        _loop(0, n_seg // _UNROLL, seg_steps)
        for job in mixer_jobs(n_seg - 1):
            job()

    def mixer(w1_v, w2_v, w3_v, w4_v, hb_s, n0_s, t3_s, t4_s, a1_s, a2_s, n1_s, last_s, wg_v,
              out_s, out_sems, *g_s):
        n_blk = S // _TM
        shifts = [(-1, 1, -2, 2)[j * _LANE * 4 // D] for j in range(ND)]
        cp_gate = copy(wmod_hbm.at[:, pl.ds(5 * D, D)], wg_v, sems.at[3])
        cp_gate.start()
        last_s[1] = jnp.zeros(last_s.shape[1:], _F32)
        for g in g_s:
            g[_HALO:2 * _HALO, :] = jnp.zeros((_HALO, _LANE), _F32)
            g[S:S + _HALO, :] = jnp.zeros((_HALO, _LANE), _F32)

        def block(ref, i, n=_TM):
            return ref.at[_aligned(i * n, n), :]

        def weight_terms(src, dst, i, r, j):
            nr, nc = src.shape[1] // P, src.shape[0] // P
            n = nr // n_blk
            dst = dst.at[:, pl.ds(pl.multiple_of(i * n, 8), n), :]
            w = [[src[b * nc + j, _aligned(a * nr + i * n + r, 8), :] for b in range(P)]
                 for a in range(P)]
            lo = _rhs_terms([[_low_half(v) for v in row] for row in w])
            hi = _rhs_terms([[_high_half(v) for v in row] for row in w])
            out = [pltpu.pack_elementwise(list(pair), packed_dtype=_BF16) for pair in zip(lo, hi)]
            for t, v in enumerate(out):
                dst[t, r:r + 8, _cols(j)] = v
            return out

        def weight_jobs(src, dst, i):
            return [functools.partial(weight_terms, src, dst, i, r, j)
                    for r in range(0, src.shape[1] // P // n_blk, 8)
                    for j in range(src.shape[0] // P)]

        def spread(jobs):
            cut = [j * len(jobs) // (ND - 1) for j in range(ND)]
            return [[]] + [jobs[cut[j]:cut[j + 1]] for j in range(ND - 1)]

        def gate(i):
            n0 = _unpacked(block(n0_s, i, _TM // 2)[...])
            for j, (g, off, jobs) in enumerate(zip(g_s, shifts, spread(weight_jobs(w3_v, t3_s, i)))):
                win = g.at[pl.ds(pl.multiple_of(i * _TM, _TM), _TM + 2 * _HALO), :]
                w = paced(w1_v[j], jobs)
                win[_HALO - off:_HALO - off + _TM, :] = _gelu(_dot(n0, w))

        nh = 2
        th = _TM // nh

        def mlp_norm(k, buf, r):
            n1 = _layernorm(last_s[buf, r:r + 16, :])
            dst = n1_s.at[:, _aligned(k * th, th), :]
            for j in range(ND):
                dst[j, r:r + 16, :] = n1[:, _cols(j)]
            return [n1]

        def norm_jobs(k, buf):
            return [functools.partial(mlp_norm, k, buf, r) for r in range(0, th, 16)]

        def mix(i):
            terms = weight_jobs(w4_v, t4_s, i)
            for u in range(nh):
                x1 = block(hb_s, i).at[u * th:(u + 1) * th, :]
                rows = pl.ds(pl.multiple_of(i * _TM + u * th + _HALO, _HALO), th)
                shifted = jnp.concatenate([g[rows, :] for g in g_s], axis=1).astype(_BF16)
                due = zip(spread(norm_jobs(jnp.maximum(nh * i + u - 1, 0), 1 - u % 2)),
                          spread(terms[u::nh]))
                for j, (norms, jobs) in enumerate(due):
                    w = paced(w2_v[j], jobs + norms)
                    y = _dot(shifted, w) + x1[:, _cols(j)]
                    x1[:, _cols(j)] = y
                    last_s[u % 2, :, _cols(j)] = y

        def mlp_terms(i, r, col):
            n1 = n1_s.at[:, _aligned(i * _TM, _TM), :]
            even, odd = (_lhs_terms(
                [[n1[(b * dq + col) // _LANE, pl.ds(a * mq + r + u, 8, stride=2), :]
                  for b in range(P)] for a in range(P)]) for u in range(2))
            out = [pltpu.pack_elementwise(list(pair), packed_dtype=_BF16) for pair in zip(even, odd)]
            for t, v in enumerate(out):
                a1_s[t, r // 2:r // 2 + 8, col:col + _LANE] = v
            return out

        def term_jobs(i):
            return [functools.partial(mlp_terms, i, r, col)
                    for r in range(0, mq, 16) for col in range(0, dq, _LANE)]

        def products(a_ref, w_ref, jobs, every):
            count = [0]

            def product(p, t):
                count[0] += 1
                due = [jobs.pop(0)] if jobs and count[0] % every == 0 else []
                return _dot(_unpacked(a_ref[t]), paced(w_ref[t, :, _cols(p)], due))
            return product

        def out_copy(i, slot):
            return copy(out_s.at[slot], block(out_hbm, i), out_sems.at[slot])

        def mlp(i):
            slot = i % 2

            @pl.when(i >= 2)
            def _():
                out_copy(jnp.maximum(i - 2, 0), slot).wait()

            terms = term_jobs(jnp.minimum(i + 1, n_blk - 1))
            up, down = products(a1_s, t3_s, [], 1), products(a2_s, t4_s, terms, 7)
            for p in range(fq // _LANE):
                g = _combine(_LEVEL, functools.partial(up, p), emit=lambda a, b, y: _gelu(y))
                for t, v in enumerate(_lhs_terms(g)):
                    a2_s[t, :, _cols(p)] = _pack(v)

            dst, xm, x1 = out_s.at[slot], block(xm_s, i), block(hb_s, i)
            for p in range(dq // _LANE):
                def emit(a, b, y):
                    rows, cols = slice(a * mq, (a + 1) * mq), _cols(b * (dq // _LANE) + p)
                    res = xm[rows, cols] + mod(5, cols) * (x1[rows, cols] + y)
                    dst[rows, cols] = res.astype(dst.dtype)

                _combine(_LEVEL, functools.partial(down, p), emit=emit)
            assert not terms
            out_copy(i, slot).start()

        _loop(0, n_blk, gate)
        _loop(0, n_blk, mix)
        cp_gate.wait()
        norms, terms = norm_jobs(nh * n_blk - 1, 1), term_jobs(0)
        mod_s[5] = jnp.concatenate(
            [_dot(mod_s[6], paced(pltpu.bitcast(wg_v[:, _cols(j)], _U32), norms[j::ND] + terms[j::ND]))
             for j in range(ND)], axis=1)
        _loop(0, n_blk, mlp)
        for i in (n_blk - 2, n_blk - 1):
            out_copy(i, i % 2).wait()

    def after_weights(wqkv, wo_s, pre_s, w1_v, w2_v, w3_v, w4_v, hb_s, n0_s):
        slabs = [(src, dst, j) for src, dst in ((w1_hbm, w1_v), (w2_hbm, w2_v), (w3_hbm, w3_v),
                                               (w4_hbm, w4_v)) for j in range(dst.shape[0])]
        cps = [copy(src.bitcast(_U32).at[:, pl.ds(j * _LANE, _LANE)], dst.at[j], sems.at[4 + n])
               for n, (src, dst, j) in enumerate(slabs)]
        _start([cp_x_tail] + cps)
        pl.run_scoped(
            functools.partial(recurrence, wqkv, wo_s, pre_s, hb_s, n0_s),
            pltpu.VMEM((M, D), _F32),
            pltpu.VMEM((seg_len - _PRE, D), _F32),
            pltpu.VMEM((L, H * _LANE), _F32),
            pltpu.VMEM((seg_len, D), _F32),
        )
        _wait(cps)

    def whole(w1_v, w2_v, w3_v, w4_v, hb_s, n0_s):
        def attention(wqkv, wo_s, pre_s):
            pl.run_scoped(
                functools.partial(load_weights, wqkv, wo_s, pre_s),
                pltpu.VMEM((D * H, _LANE), _BF16),
                pltpu.VMEM((n_seg, _PRE, D), _BF16),
                pltpu.VMEM((ND, n_seg * _PRE, _LANE), _F32),
                pltpu.VMEM((ND // 2, 7, n_seg * _PRE // 4, _LANE), _U32),
                pltpu.VMEM((3 * ND, D, _LANE), _BF16),
                pltpu.VMEM((2, ND, 8, _LANE), _F32),
                pltpu.SemaphoreType.DMA((ND,)),
                pltpu.SemaphoreType.DMA((3 * ND,)),
                pltpu.SemaphoreType.DMA((ND + 2,)),
            )
            after_weights(wqkv, wo_s, pre_s, w1_v, w2_v, w3_v, w4_v, hb_s, n0_s)

        pl.run_scoped(
            attention,
            pltpu.VMEM((3 * H, D // 2, _LANE), _U32),
            pltpu.VMEM((ND, H * _LANE // 2, _LANE), _U32),
            pltpu.VMEM((3 * H, n_seg * _PRE, _LANE), _F32),
        )
        pl.run_scoped(
            functools.partial(mixer, w1_v, w2_v, w3_v, w4_v, hb_s, n0_s),
            pltpu.VMEM((T, dq // 2, fq), _U32),
            pltpu.VMEM((T, fq // 2, dq), _U32),
            pltpu.VMEM((T, mq // 2, dq), _U32),
            pltpu.VMEM((T, mq // 2, fq), _U32),
            pltpu.VMEM((ND, S, _LANE), _F32),
            pltpu.VMEM((2, _TM // 2, D), _F32),
            pltpu.VMEM((D, D), _BF16),
            pltpu.VMEM((2, _TM, D), _BF16),
            pltpu.SemaphoreType.DMA((2,)),
            *[pltpu.VMEM((S + 4 * _HALO, _LANE), _F32) for _ in range(ND)],
        )

    pl.run_scoped(
        whole,
        pltpu.VMEM((ND, D // 2, _LANE), _U32),
        pltpu.VMEM((ND, D // 2, _LANE), _U32),
        pltpu.VMEM((F // _LANE, D // 2, _LANE), _U32),
        pltpu.VMEM((ND, F // 2, _LANE), _U32),
        pltpu.VMEM((S, D), _F32),
        pltpu.VMEM((S // 2, D), _U32),
    )


@functools.partial(jax.jit, static_argnames=("A_seg_len",))
def pallas_adaLN_cond__memory_aug_recurrent_mem_tr__mixer_s_mlp__prompt_kernel(
    A_x: jax.Array,
    A_mem0: jax.Array,
    A_Wq: jax.Array,
    A_Wk: jax.Array,
    A_Wv: jax.Array,
    A_Wo: jax.Array,
    A_seg_len: int,
    B_x: jax.Array,
    B_w1: jax.Array,
    B_w2: jax.Array,
    B_w3: jax.Array,
    B_w4: jax.Array,
    c: jax.Array,
    w_mod: jax.Array,
):
    del B_x
    batch, S, D = A_x.shape
    _, H, Dh = A_Wq.shape
    M = A_mem0.shape[1]
    seg_len = int(A_seg_len)
    assert (batch, S, D, Dh, M, seg_len, B_w3.shape[1]) == (1, 2048, 1024, _LANE, 8, 32, 3584)
    n_seg = S // seg_len

    hbm = pl.BlockSpec(memory_space=pl.ANY)
    out = pl.pallas_call(
        _kernel,
        out_shape=jax.ShapeDtypeStruct((S, D), A_x.dtype),
        in_specs=[hbm] * 12,
        out_specs=hbm,
        scratch_shapes=[
            pltpu.VMEM(c.shape, _BF16),
            pltpu.VMEM((16, _LANE), _U32),
            pltpu.VMEM((M, D), _BF16),
            pltpu.VMEM((n_seg, seg_len, D), _BF16),
            pltpu.VMEM((S, D), _F32),
            pltpu.VMEM((7, 8, D), _F32),
            pltpu.SemaphoreType.DMA((4 + (3 * D + B_w3.shape[1]) // _LANE,)),
        ],
        compiler_params=pltpu.CompilerParams(vmem_limit_bytes=126 * 1024 * 1024),
        name="adaln_rmt_mixer",
    )(
        A_mem0.reshape(M, D), c, A_x.reshape(n_seg, seg_len, D),
        A_Wq.reshape(D * H, Dh), A_Wk.reshape(D * H, Dh), A_Wv.reshape(D * H, Dh),
        A_Wo.reshape(H * Dh, D), B_w1, B_w2, B_w3, B_w4, w_mod,
    )
    return out.reshape(batch, S, D)
```
